```python
import jax
import jax.numpy as jnp

def _softmax(x, axis=-1):
    return jax.nn.softmax(x, axis=axis)
def _gelu(x):
    return jax.nn.gelu(x, approximate=True)
def _silu(x):
    return jax.nn.silu(x)
def _sigmoid(x):
    return jax.nn.sigmoid(x)
def _layernorm(x, axis=-1, eps=1e-5):
    m = jnp.mean(x, axis=axis, keepdims=True)
    v = jnp.var(x, axis=axis, keepdims=True)
    return (x - m) / jnp.sqrt(v + eps)
def _scatter_add(tgt, idx, src, axis=0):
    return tgt.at[idx].add(src)
def _segment_sum(src, seg, n):
    return jax.ops.segment_sum(src, seg, n)
class _Rng:
    def __init__(self, key):
        self._k = key
    def _next(self):
        self._k, sub = jax.random.split(self._k)
        return sub
    def normal(self, shape):
        return jax.random.normal(self._next(), shape, dtype=jnp.bfloat16)
    def randint(self, lo, hi, shape):
        return jax.random.randint(self._next(), shape, lo, hi, dtype=jnp.int32)
    def uniform(self, shape, lo=0.0, hi=1.0):
        return jax.random.uniform(self._next(), shape, jnp.bfloat16, lo, hi)
    def permutation(self, n):
        return jax.random.permutation(self._next(), n)


kernel_name = 'gated_mix__linear_kernel_hedgehog__moe_arch_mod__prompt'

def setup_inputs():
    _rng = _Rng(jax.random.key(int.from_bytes(__import__("os").urandom(4), "little")))
    _w = (lambda a: (lambda t: t.astype(jnp.bfloat16) if jnp.issubdtype(t.dtype, jnp.floating) else t)(jnp.asarray(a)))
    def _A_setup():
        B, S, D, H = 1, 2048, 1024, 32
        Dh = D // H
        return {
            "x": _w((lambda *s: _rng.normal(s) * 0.05)(B, S, D)),
            "wqkv": _w((lambda *s: _rng.normal(s) * 0.05)(D, 3 * D)),
            "w_phi": _w((lambda *s: _rng.normal(s) * 0.05)(H, Dh, Dh) * (Dh ** -0.5)),
            "wo": _w((lambda *s: _rng.normal(s) * 0.05)(D, D)),
        }
    _A_in = _A_setup()

    def _B_setup():
        B, S, D, F, C = 1, 2048, 1024, 3584, 1
        return {
            "x": _w((lambda *s: _rng.normal(s) * 0.05)(B, S, D)),
            "w_r": _w((lambda *s: _rng.normal(s) * 0.05)(D)),
            "w_gate": _w((lambda *s: _rng.normal(s) * 0.05)(D, F)),
            "w_up": _w((lambda *s: _rng.normal(s) * 0.05)(D, F)),
            "w_down": _w((lambda *s: _rng.normal(s) * 0.05)(F, D)),
        }
    _B_in = _B_setup()

    return {
        "A_x": _A_in["x"],
        "A_wqkv": _A_in["wqkv"],
        "A_w_phi": _A_in["w_phi"],
        "A_wo": _A_in["wo"],
        "B_x": _B_in["x"],
        "B_w_r": _B_in["w_r"],
        "B_w_gate": _B_in["w_gate"],
        "B_w_up": _B_in["w_up"],
        "B_w_down": _B_in["w_down"],
        "gate_w": _w((lambda *s: _rng.normal(s) * 0.05)(1024)),
    }

def reference(A_x, A_wqkv, A_w_phi, A_wo, B_x, B_w_r, B_w_gate, B_w_up, B_w_down, gate_w):
    def _A_ref(x, wqkv, w_phi, wo):
        B, S, D = x.shape
        H = 32; Dh = D // H
        qkv = (lambda x, *d: x.transpose(*d))((x @ wqkv).reshape(B, S, 3, H, Dh), 2, 0, 3, 1, 4)
        q, k, v = qkv[0], qkv[1], qkv[2]
        pq = jnp.einsum("bhsd,hdf->bhsf", q, w_phi)
        pk = jnp.einsum("bhsd,hdf->bhsf", k, w_phi)
        phi_q = jnp.concatenate([_softmax(pq, axis=-1), _softmax(-pq, axis=-1)], axis=-1)
        phi_k = jnp.concatenate([_softmax(pk, axis=-1), _softmax(-pk, axis=-1)], axis=-1)
        kv = jnp.einsum("bhsf,bhsd->bhfd", phi_k, v)
        z  = jnp.einsum("bhsf->bhf", phi_k)
        num = jnp.einsum("bhqf,bhfd->bhqd", phi_q, kv)
        den = jnp.einsum("bhqf,bhf->bhq", phi_q, z)[..., None] + 1e-6
        o = num / den
        return (lambda x, *d: x.transpose(*d))(o, 0, 2, 1, 3).reshape(B, S, D) @ wo

    def _B_ref(x, w_r, w_gate, w_up, w_down):
        B, S, D = x.shape
        C = 1
        r = x @ w_r
        idx = jnp.argsort(-r, axis=-1)[:, :C]
        idx_e = jnp.repeat(idx.reshape(B, C, 1), D, axis=2)
        x_sel = jnp.take_along_axis(x, idx_e, axis=1)
        g = _silu(x_sel @ w_gate)
        u = x_sel @ w_up
        y = (g * u) @ w_down
        r_sel = _sigmoid(jnp.take_along_axis(r, idx, axis=1))
        y = y * r_sel.reshape(B, C, 1)
        b_off = (jnp.arange(B) * S).reshape(B, 1)
        flat_idx = (idx + b_off).reshape(B * C)
        zero = (x * 0.0).reshape(B * S, D)
        upd = _scatter_add(zero, flat_idx, y.reshape(B * C, D), axis=0)
        return x + upd.reshape(B, S, D)

    x = A_x
    g = _sigmoid((x * gate_w).sum(-1, keepdims=True))
    a = _A_ref(x, A_wqkv, A_w_phi, A_wo)
    b = _B_ref(x, B_w_r, B_w_gate, B_w_up, B_w_down)
    return g * a + (1 - g) * b
```

```python
import functools
import jax
import jax.numpy as jnp
import numpy as np
from jax import lax
import jax.experimental.pallas as pl
import jax.experimental.pallas.tpu as pltpu

S, D, H, DH, F = 2048, 1024, 32, 32, 3584
NG = 8
T = 256
NT_ = S // T
NFC = 4
FC = F // NFC
LOG2E = 1.4426950408889634

NT = (((1,), (1,)), ((), ()))
NN = (((1,), (0,)), ((), ()))
TN = (((0,), (0,)), ((), ()))
f32 = jnp.float32
bf16 = jnp.bfloat16


def _dot(a, b, dims):
    return lax.dot_general(a, b, dims, preferred_element_type=f32)


def _dual_softmax(p):
    outs = []
    for h in range(2):
        ph = p[h * DH:(h + 1) * DH]
        mx = jnp.max(ph, axis=0, keepdims=True)
        mn = jnp.min(ph, axis=0, keepdims=True)
        ep = jnp.exp2(ph - mx)
        en = jnp.exp2(mn - ph)
        sp = jnp.sum(ep, axis=0, keepdims=True)
        sn = jnp.sum(en, axis=0, keepdims=True)
        outs.append((ep * (1.0 / sp)).astype(bf16))
        outs.append((en * (1.0 / sn)).astype(bf16))
    return jnp.concatenate(outs, axis=0)


def kernel(xa_hbm, wqkv_hbm, wphi_ref, wo_hbm, wr_ref, wg_hbm, wu_hbm, wd_hbm, gw_ref,
           out_hbm,
           xa, w3, wo, wg, wu, wd, wt, kvs, ot, rs, hs, sems, osems):
    def xa_cp(t):
        return pltpu.make_async_copy(xa_hbm.at[pl.ds(t * T, T)], xa.at[pl.ds(t * T, T)], sems.at[t])

    def w3_cp(j):
        return pltpu.make_async_copy(wqkv_hbm.at[:, pl.ds(j * 128, 128)], w3.at[j], sems.at[8 + j])

    xb = xa
    wo_cp = pltpu.make_async_copy(wo_hbm, wo, sems.at[33])

    def wg_cp(c):
        return pltpu.make_async_copy(wg_hbm.at[:, pl.ds(c * FC, FC)], wg.at[c], sems.at[34 + c])

    def wu_cp(c):
        return pltpu.make_async_copy(wu_hbm.at[:, pl.ds(c * FC, FC)], wu.at[c], sems.at[38 + c])

    def wd_cp(c):
        return pltpu.make_async_copy(wd_hbm.at[pl.ds(c * FC, FC)], wd.at[c], sems.at[42 + c])

    def out_cp(t, slot):
        r0 = pl.multiple_of(t * T, T)
        return pltpu.make_async_copy(xb.at[pl.ds(r0, T)], out_hbm.at[pl.ds(r0, T)], osems.at[slot])

    w3_cp(8).start()
    w3_cp(16).start()
    for t in range(NT_):
        xa_cp(t).start()
    for g in range(1, NG):
        w3_cp(8 + g).start()
        w3_cp(16 + g).start()

    row = lax.broadcasted_iota(jnp.int32, (128, 128), 0)
    col = lax.broadcasted_iota(jnp.int32, (128, 128), 1)
    e_row = lax.broadcasted_iota(jnp.int32, (128, DH), 0)
    e_col = lax.broadcasted_iota(jnp.int32, (128, DH), 1)

    def fold(g, j):
        p = wphi_ref[pl.ds(pl.multiple_of(g * 128, 128), 128), :]
        e = jnp.where((e_row % DH) == e_col, 1.0, 0.0).astype(bf16)
        bdt = _dot(e, p, NT)
        bdt = jnp.where((row // DH) == (col // DH), bdt, 0.0).astype(bf16)
        return (_dot(bdt, w3[j], NT) * LOG2E).astype(bf16)

    def prep_kv(g, slot):
        w3_cp(8 + g).wait()
        w3_cp(16 + g).wait()
        kt = fold(g, 8 + g)
        vt = w3[16 + g].T
        for p in range(2):
            wt[slot, pl.ds(p * 128, 64), :] = kt[p * 64:(p + 1) * 64]
            wt[slot, pl.ds(p * 128 + 64, 64), :] = vt[p * 64:(p + 1) * 64]

    def prep_q(g, slot):
        w3_cp(g).wait()
        wt[slot, pl.ds(0, 128), :] = fold(g, g)

    ones_rows = jnp.ones((16, T), bf16)
    r80 = lax.broadcasted_iota(jnp.int32, (80, 128), 0)
    c80 = lax.broadcasted_iota(jnp.int32, (80, 128), 1)
    kv_mask = jnp.where(r80 < 64, r80 // DH, r80 - 64) == (c80 // 64)

    def kv_group(g, slot, first):
        for p in range(2):
            w = wt[slot, pl.ds(p * 128, 128), :]
            acc = None
            for t in range(NT_):
                if first and p == 0:
                    xa_cp(t).wait()
                r = _dot(w, xa[pl.ds(t * T, T), :], NT)
                phi = _dual_softmax(r[:64])
                vt = jnp.concatenate([r[64:].astype(bf16), ones_rows], axis=0)
                d = _dot(vt, phi, NT)
                acc = d if acc is None else acc + d
            kvs[2 * g + p] = jnp.where(kv_mask, acc, 0.0).astype(bf16)

    prep_kv(0, 0)
    kv_group(0, 0, True)
    prep_kv(1, 1)
    for g in range(NG):
        w3_cp(g).start()

    def p1(g, c):
        slot = g % 2

        @pl.when(g == 2)
        def _():
            wo_cp.start()

        @pl.when(jnp.logical_and(g >= 3, g < 7))
        def _():
            wg_cp(g - 3).start()
            wu_cp(g - 3).start()

        kv_group(g, slot, False)
        prep_kv(g + 1, 1 - slot)
        return c

    lax.fori_loop(1, NG - 1, p1, 0)
    for c in range(NFC):
        wd_cp(c).start()
    kv_group(NG - 1, 1, False)
    prep_q(0, 0)

    wr = wr_ref[...].astype(f32)
    wr_rows = jnp.concatenate(
        [jnp.broadcast_to(wr[j:j + 1, :], (16, 128)) for j in range(8)], axis=1).astype(bf16)

    def q_group(g, slot):
        w = wt[slot, pl.ds(0, 128), :]
        for t in range(NT_):
            r = _dot(w, xa[pl.ds(t * T, T), :], NT)
            for p in range(2):
                phi = _dual_softmax(r[p * 64:(p + 1) * 64])
                nd = _dot(kvs[2 * g + p], phi, NN)
                inv = 1.0 / (nd[64:72] + 1e-6)
                o0 = nd[0:32] * inv[0:1]
                o1 = nd[32:64] * inv[1:2]
                r0 = pl.multiple_of(g * 128 + p * 64, 64)
                ot[t, pl.ds(r0, 64), :] = jnp.concatenate([o0, o1], axis=0).astype(bf16)
        t0 = pl.multiple_of(g * T, T)
        rs[g] = _dot(wr_rows, xb[pl.ds(t0, T), :], NT)[:8]

    def p2(g, c):
        slot = g % 2
        q_group(g, slot)
        prep_q(g + 1, 1 - slot)
        return c

    lax.fori_loop(0, NG - 1, p2, 0)
    q_group(NG - 1, 1)

    r = rs[...].astype(bf16).astype(f32)
    pos = (lax.broadcasted_iota(jnp.int32, r.shape, 0) * T
           + lax.broadcasted_iota(jnp.int32, r.shape, 2))
    m = jnp.max(jnp.where(r == r, r, -jnp.inf))
    idx = jnp.min(jnp.where(r == m, pos, S))
    idx = jnp.where(idx >= S, 0, idx)
    r_sel = jnp.max(jnp.where(pos == idx, r, -jnp.inf))
    blk = pl.multiple_of((idx // 16) * 16, 16)
    t_last = idx // T

    wo_cp.wait()
    gw = gw_ref[...].astype(f32)

    def out_tile(i):
        t = (t_last + 1 + i) % NT_
        r0 = pl.multiple_of(t * T, T)
        a = _dot(ot[t], wo[...], TN)
        xg = None
        for j in range(8):
            pj = xa[pl.ds(r0, T), pl.ds(j * 128, 128)].astype(f32) * gw[j:j + 1, :]
            xg = pj if xg is None else xg + pj
        gate = jax.nn.sigmoid(jnp.sum(xg, axis=1, keepdims=True))
        b = xb[pl.ds(r0, T), :].astype(f32)
        xb[pl.ds(r0, T), :] = (gate * a + (1.0 - gate) * b).astype(bf16)
        out_cp(t, i).start()

    def p3a(i, c):
        wg_cp(i).wait()
        wu_cp(i).wait()
        xs = xb[pl.ds(blk, 16), :]
        gt = _dot(xs, wg[i], NN).astype(bf16).astype(f32)
        up = _dot(xs, wu[i], NN).astype(bf16).astype(f32)
        hs[i] = ((gt * jax.nn.sigmoid(gt)).astype(bf16).astype(f32) * up).astype(bf16)
        out_tile(i)
        return c

    lax.fori_loop(0, 4, p3a, 0)

    def p3b(i, y):
        wd_cp(i).wait()
        y = y + _dot(hs[i], wd[i], NN)
        out_tile(4 + i)
        return y

    y = lax.fori_loop(0, 3, p3b, jnp.zeros((16, D), f32))
    wd_cp(3).wait()
    y = y + _dot(hs[3], wd[3], NN)
    sg = jax.nn.sigmoid(jnp.full((16, D), r_sel, f32)).astype(bf16).astype(f32)
    y = (y.astype(bf16).astype(f32) * sg).astype(bf16).astype(f32)
    xs = xb[pl.ds(blk, 16), :].astype(f32)
    sel = lax.broadcasted_iota(jnp.int32, (16, D), 0) == (idx - blk)
    xb[pl.ds(blk, 16), :] = jnp.where(sel, xs + y, xs).astype(bf16)
    out_tile(NT_ - 1)
    for i in range(NT_):
        out_cp(0, i).wait()


@jax.jit
def pallas_gated_mix__linear_kernel_hedgehog__moe_arch_mod__prompt_kernel(A_x, A_wqkv, A_w_phi, A_wo, B_x, B_w_r, B_w_gate, B_w_up, B_w_down, gate_w):
    hbm = pl.BlockSpec(memory_space=pl.ANY)
    vm = pl.BlockSpec(memory_space=pltpu.VMEM)
    out = pl.pallas_call(
        kernel,
        out_shape=jax.ShapeDtypeStruct((S, D), bf16),
        in_specs=[hbm, hbm, vm, hbm, vm, hbm, hbm, hbm, vm],
        out_specs=hbm,
        scratch_shapes=[
            pltpu.VMEM((S, D), bf16),
            pltpu.VMEM((24, D, 128), bf16),
            pltpu.VMEM((D, D), bf16),
            pltpu.VMEM((NFC, D, FC), bf16),
            pltpu.VMEM((NFC, D, FC), bf16),
            pltpu.VMEM((NFC, FC, D), bf16),
            pltpu.VMEM((2, 256, D), bf16),
            pltpu.VMEM((16, 80, 128), bf16),
            pltpu.VMEM((NT_, D, T), bf16),
            pltpu.VMEM((NT_, 8, T), f32),
            pltpu.VMEM((NFC, 16, FC), bf16),
            pltpu.SemaphoreType.DMA((46,)),
            pltpu.SemaphoreType.DMA((NT_,)),
        ],
        compiler_params=pltpu.CompilerParams(vmem_limit_bytes=100 * 1024 * 1024),
    )(A_x.reshape(S, D), A_wqkv, A_w_phi.reshape(H * DH, DH), A_wo,
      B_w_r.reshape(8, 128), B_w_gate, B_w_up, B_w_down, gate_w.reshape(8, 128))
    return out.reshape(1, S, D)
```

```python
import functools
import jax
import jax.numpy as jnp
import numpy as np
from jax import lax
import jax.experimental.pallas as pl
import jax.experimental.pallas.tpu as pltpu

S, D, H, DH, F = 2048, 1024, 32, 32, 3584
NG = 8
T = 256
NT_ = S // T
NFC = 4
FC = F // NFC
LOG2E = 1.4426950408889634

NT = (((1,), (1,)), ((), ()))
NN = (((1,), (0,)), ((), ()))
f32 = jnp.float32
bf16 = jnp.bfloat16


def _dot(a, b, dims):
    return lax.dot_general(a, b, dims, preferred_element_type=f32)


def _dual_softmax(p):
    outs = []
    for h in range(2):
        ph = p[h * DH:(h + 1) * DH]
        mx = jnp.max(ph, axis=0, keepdims=True)
        mn = jnp.min(ph, axis=0, keepdims=True)
        ep = jnp.exp2(ph - mx)
        en = jnp.exp2(mn - ph)
        sp = jnp.sum(ep, axis=0, keepdims=True)
        sn = jnp.sum(en, axis=0, keepdims=True)
        outs.append(ep * (1.0 / sp))
        outs.append(en * (1.0 / sn))
    return jnp.concatenate(outs, axis=0).astype(bf16)


def kernel(x_hbm, wqkv_hbm, wphi_ref, wo_hbm, wr_ref, wg_hbm, wu_hbm, wd_hbm, gw_ref,
           out_hbm,
           xs, w3, wo, wg, wu, wd, wt, kvs, os_, rs, hs, ob, sems, osems):
    XH = S // 2
    def x_cp(j, h):
        return pltpu.make_async_copy(x_hbm.at[pl.ds(h * XH, XH), pl.ds(j * 128, 128)],
                                     xs.at[j, pl.ds(h * XH, XH)], sems.at[h * 8 + j])

    def w3_cp(j):
        return pltpu.make_async_copy(wqkv_hbm.at[:, pl.ds(j * 128, 128)], w3.at[j], sems.at[16 + j])

    def wo_cp(j):
        return pltpu.make_async_copy(wo_hbm.at[:, pl.ds(j * 128, 128)], wo.at[j], sems.at[40 + j])

    def wg_cp(c):
        return pltpu.make_async_copy(wg_hbm.at[:, pl.ds(c * FC, FC)], wg.at[c], sems.at[48 + c])

    def wu_cp(c):
        return pltpu.make_async_copy(wu_hbm.at[:, pl.ds(c * FC, FC)], wu.at[c], sems.at[52 + c])

    def wd_cp(c):
        return pltpu.make_async_copy(wd_hbm.at[pl.ds(c * FC, FC)], wd.at[c], sems.at[56 + c])

    def out_cp(t, slot):
        r0 = pl.multiple_of(t * T, T)
        return pltpu.make_async_copy(ob.at[pl.ds(r0, T)], out_hbm.at[pl.ds(r0, T)], osems.at[slot])

    w3_cp(8).start()
    w3_cp(16).start()
    for h in range(2):
        for j in range(8):
            x_cp(j, h).start()
    for g in range(1, NG):
        w3_cp(8 + g).start()
        w3_cp(16 + g).start()

    row = lax.broadcasted_iota(jnp.int32, (128, 128), 0)
    col = lax.broadcasted_iota(jnp.int32, (128, 128), 1)
    e_row = lax.broadcasted_iota(jnp.int32, (128, DH), 0)
    e_col = lax.broadcasted_iota(jnp.int32, (128, DH), 1)

    def x_tile(r0, n):
        return jnp.concatenate([xs[j, pl.ds(r0, n), :] for j in range(8)], axis=1)

    def w_rows(slot, r0):
        return jnp.concatenate([wt[slot, j, pl.ds(r0, 128), :] for j in range(8)], axis=1)

    def fold(g, j):
        p = wphi_ref[pl.ds(pl.multiple_of(g * 128, 128), 128), :]
        e = jnp.where((e_row % DH) == e_col, 1.0, 0.0).astype(bf16)
        bdt = _dot(e, p, NT)
        bdt = jnp.where((row // DH) == (col // DH), bdt, 0.0).astype(bf16)
        return (_dot(bdt, w3[j], NT) * LOG2E).astype(bf16)

    def prep_kv(g, slot):
        w3_cp(8 + g).wait()
        w3_cp(16 + g).wait()
        kt = fold(g, 8 + g)
        vt = w3[16 + g].T
        for p in range(2):
            for j in range(8):
                wt[slot, j, pl.ds(p * 128, 64), :] = kt[p * 64:(p + 1) * 64, j * 128:(j + 1) * 128]
                wt[slot, j, pl.ds(p * 128 + 64, 64), :] = vt[p * 64:(p + 1) * 64, j * 128:(j + 1) * 128]

    def prep_q(g, slot):
        w3_cp(g).wait()
        qt = fold(g, g)
        for j in range(8):
            wt[slot, j, pl.ds(0, 128), :] = qt[:, j * 128:(j + 1) * 128]

    ones_rows = jnp.ones((16, T), f32)
    r80 = lax.broadcasted_iota(jnp.int32, (80, 128), 0)
    c80 = lax.broadcasted_iota(jnp.int32, (80, 128), 1)
    kv_mask = jnp.where(r80 < 64, r80 // DH, r80 - 64) == (c80 // 64)

    def kv_group(g, slot, first, tail):
        n = 2 * NT_

        def big(c):
            p, t = divmod(c, NT_)
            if first and p == 0 and (t * T) % XH == 0:
                for j in range(8):
                    x_cp(j, (t * T) // XH).wait()
            return _dot(w_rows(slot, p * 128), x_tile(t * T, T), NT)

        r = big(0)
        acc = None
        for c in range(n):
            r_next = big(c + 1) if c + 1 < n else None
            if c == n - 1:
                tail()
            phi = _dual_softmax(r[:64])
            vt = jnp.concatenate([r[64:], ones_rows], axis=0).astype(bf16)
            d = _dot(vt, phi, NT)
            acc = d if acc is None else acc + d
            if c % NT_ == NT_ - 1:
                kvs[2 * g + c // NT_] = jnp.where(kv_mask, acc, 0.0).astype(bf16)
                acc = None
            r = r_next

    prep_kv(0, 0)
    kv_group(0, 0, True, lambda: prep_kv(1, 1))
    for g in range(NG):
        w3_cp(g).start()

    def p1(g, c):
        slot = g % 2

        @pl.when(g == 2)
        def _():
            for j in range(8):
                wo_cp(j).start()

        @pl.when(jnp.logical_and(g >= 3, g < 7))
        def _():
            wg_cp(g - 3).start()
            wu_cp(g - 3).start()

        kv_group(g, slot, False, lambda: prep_kv(g + 1, 1 - slot))
        return c

    lax.fori_loop(1, NG - 1, p1, 0)
    for c in range(NFC):
        wd_cp(c).start()
    kv_group(NG - 1, 1, False, lambda: prep_q(0, 0))

    wr = wr_ref[...].astype(f32)
    wr_rows = jnp.concatenate(
        [jnp.broadcast_to(wr[j:j + 1, :], (16, 128)) for j in range(8)], axis=1).astype(bf16)

    def q_group(g, slot, tail):
        def big(t):
            return _dot(w_rows(slot, 0), x_tile(t * T, T), NT)

        r = big(0)
        for t in range(NT_):
            r_next = big(t + 1) if t + 1 < NT_ else None
            if t == NT_ - 1:
                tail()
                rs[g] = _dot(wr_rows, x_tile(pl.multiple_of(g * T, T), T), NT)[:8]
            os = []
            for p in range(2):
                phi = _dual_softmax(r[p * 64:(p + 1) * 64])
                nd = _dot(kvs[2 * g + p], phi, NN)
                inv = 1.0 / (nd[64:72] + 1e-6)
                os.append(nd[0:32] * inv[0:1])
                os.append(nd[32:64] * inv[1:2])
            o = jnp.concatenate(os, axis=0).astype(bf16)
            os_[g, pl.ds(t * T, T), :] = o.T
            r = r_next

    def p2(g, c):
        slot = g % 2
        q_group(g, slot, lambda: prep_q(g + 1, 1 - slot))
        return c

    lax.fori_loop(0, NG - 1, p2, 0)
    q_group(NG - 1, 1, lambda: None)

    r = rs[...].astype(bf16).astype(f32)
    pos = (lax.broadcasted_iota(jnp.int32, r.shape, 0) * T
           + lax.broadcasted_iota(jnp.int32, r.shape, 2))
    m = jnp.max(jnp.where(r == r, r, -jnp.inf))
    idx = jnp.min(jnp.where(r == m, pos, S))
    idx = jnp.where(idx >= S, 0, idx)
    r_sel = jnp.max(jnp.where(pos == idx, r, -jnp.inf))
    blk = pl.multiple_of((idx // 16) * 16, 16)
    t_last = idx // T

    for j in range(8):
        wo_cp(j).wait()
    gw = gw_ref[...].astype(f32)

    def out_tile(i, upd=None):
        t = (t_last + 1 + i) % NT_
        r0 = pl.multiple_of(t * T, T)
        o = jnp.concatenate([os_[j, pl.ds(r0, T), :] for j in range(8)], axis=1)
        xg = None
        for j in range(8):
            pj = xs[j, pl.ds(r0, T), :].astype(f32) * gw[j:j + 1, :]
            xg = pj if xg is None else xg + pj
        gate = jax.nn.sigmoid(jnp.sum(xg, axis=1, keepdims=True))
        NC = 256
        a = _dot(o, jnp.concatenate([wo[0], wo[1]], axis=1), NN)
        for c in range(D // NC):
            a_next = (_dot(o, jnp.concatenate([wo[2 * c + 2], wo[2 * c + 3]], axis=1), NN)
                      if c + 1 < D // NC else None)
            b = jnp.concatenate([xs[2 * c, pl.ds(r0, T), :], xs[2 * c + 1, pl.ds(r0, T), :]], axis=1).astype(f32)
            if upd is not None:
                sel = (lax.broadcasted_iota(jnp.int32, (T, NC), 0) == idx - r0)
                b = jnp.where(sel, (b + upd[0:1, c * NC:(c + 1) * NC]).astype(bf16).astype(f32), b)
            ob[pl.ds(r0, T), pl.ds(c * NC, NC)] = (gate * a + (1.0 - gate) * b).astype(bf16)
            a = a_next
        out_cp(t, i).start()

    def p3a(i, c):
        wg_cp(i).wait()
        wu_cp(i).wait()
        xsel = x_tile(blk, 16)
        gt = _dot(xsel, wg[i], NN).astype(bf16).astype(f32)
        up = _dot(xsel, wu[i], NN).astype(bf16).astype(f32)
        hs[i] = ((gt * jax.nn.sigmoid(gt)).astype(bf16).astype(f32) * up).astype(bf16)
        out_tile(i)
        return c

    lax.fori_loop(0, 4, p3a, 0)

    def p3b(i, y):
        wd_cp(i).wait()
        y = y + _dot(hs[i], wd[i], NN)
        out_tile(4 + i)
        return y

    y = lax.fori_loop(0, 3, p3b, jnp.zeros((16, D), f32))
    wd_cp(3).wait()
    y = y + _dot(hs[3], wd[3], NN)
    sg = jax.nn.sigmoid(jnp.full((16, D), r_sel, f32)).astype(bf16).astype(f32)
    y = (y.astype(bf16).astype(f32) * sg).astype(bf16).astype(f32)
    sel = lax.broadcasted_iota(jnp.int32, (16, D), 0) == (idx - blk)
    upd = jnp.sum(jnp.where(sel, y, 0.0), axis=0, keepdims=True)
    out_tile(NT_ - 1, upd)
    for i in range(NT_):
        out_cp(0, i).wait()


@jax.jit
def pallas_gated_mix__linear_kernel_hedgehog__moe_arch_mod__prompt_kernel(A_x, A_wqkv, A_w_phi, A_wo, B_x, B_w_r, B_w_gate, B_w_up, B_w_down, gate_w):
    hbm = pl.BlockSpec(memory_space=pl.ANY)
    vm = pl.BlockSpec(memory_space=pltpu.VMEM)
    out = pl.pallas_call(
        kernel,
        out_shape=jax.ShapeDtypeStruct((S, D), bf16),
        in_specs=[hbm, hbm, vm, hbm, vm, hbm, hbm, hbm, vm],
        out_specs=hbm,
        scratch_shapes=[
            pltpu.VMEM((8, S, 128), bf16),
            pltpu.VMEM((24, D, 128), bf16),
            pltpu.VMEM((8, D, 128), bf16),
            pltpu.VMEM((NFC, D, FC), bf16),
            pltpu.VMEM((NFC, D, FC), bf16),
            pltpu.VMEM((NFC, FC, D), bf16),
            pltpu.VMEM((2, 8, 256, 128), bf16),
            pltpu.VMEM((16, 80, 128), bf16),
            pltpu.VMEM((8, S, 128), bf16),
            pltpu.VMEM((NT_, 8, T), f32),
            pltpu.VMEM((NFC, 16, FC), bf16),
            pltpu.VMEM((S, D), bf16),
            pltpu.SemaphoreType.DMA((60,)),
            pltpu.SemaphoreType.DMA((NT_,)),
        ],
        compiler_params=pltpu.CompilerParams(vmem_limit_bytes=100 * 1024 * 1024),
    )(A_x.reshape(S, D), A_wqkv, A_w_phi.reshape(H * DH, DH), A_wo,
      B_w_r.reshape(8, 128), B_w_gate, B_w_up, B_w_down, gate_w.reshape(8, 128))
    return out.reshape(1, S, D)
```

```python
import functools
import os
import jax
import jax.numpy as jnp
import numpy as np
from jax import lax
import jax.experimental.pallas as pl
import jax.experimental.pallas.tpu as pltpu

S, D, H, DH, F = 2048, 1024, 32, 32, 3584
NG = 8
T = 256
NT_ = S // T
NF = F // 128
LOG2E = 1.4426950408889634
LAG = 2
TM = 128
NC = 128
LAG3 = 1

NT = (((1,), (1,)), ((), ()))
NN = (((1,), (0,)), ((), ()))
f32 = jnp.float32
bf16 = jnp.bfloat16
i32 = jnp.int32

XBLK = [(0, 1), (1, 1), (2, 1), (3, 1), (4, 1), (5, 1), (6, 2)]


def _dot(a, b, dims):
    return lax.dot_general(a, b, dims, preferred_element_type=f32)


def _recip(x):
    r = pl.reciprocal(x, approx=True)
    return r * (2.0 - x * r)


def _sigmoid(x):
    return jax.nn.sigmoid(x)


def _r16(x):
    return x.astype(bf16).astype(f32)


def _ld(ref, r0, n, c0=None, nc=None):
    h0 = r0 // 2 if isinstance(r0, int) else pl.multiple_of(r0 // 2, 8)
    cols = slice(None) if c0 is None else pl.ds(c0, nc)
    return pltpu.bitcast(ref[pl.ds(h0, n // 2), cols], bf16)


def _st(ref, r0, val, c0=None):
    h0 = r0 // 2 if isinstance(r0, int) else pl.multiple_of(r0 // 2, 8)
    cols = slice(None) if c0 is None else pl.ds(c0, val.shape[1])
    ref[pl.ds(h0, val.shape[0] // 2), cols] = pltpu.bitcast(val, i32)


def _dual_softmax(p):
    outs = []
    for h in range(2):
        ph = p[h * DH:(h + 1) * DH]
        mx = jnp.max(ph, axis=0, keepdims=True)
        mn = jnp.min(ph, axis=0, keepdims=True)
        ep = jnp.exp2(ph - mx)
        en = jnp.exp2(mn - ph)
        sp = jnp.sum(ep, axis=0, keepdims=True)
        sn = jnp.sum(en, axis=0, keepdims=True)
        outs.append(ep * _recip(sp))
        outs.append(en * _recip(sn))
    return jnp.concatenate(outs, axis=0)


def _col(row):
    return jnp.broadcast_to(row, (128, 128)).T


def _pipeline(jobs, lag):
    rs = []
    for c, (big, post) in enumerate(jobs):
        rs.append(big())
        if c >= lag:
            jobs[c - lag][1](rs[c - lag])
            rs[c - lag] = None
    for c in range(max(len(jobs) - lag, 0), len(jobs)):
        jobs[c][1](rs[c])


def kernel(x_hbm, wqkv_hbm, wphi_hbm, wo_hbm, wr_hbm, wg_hbm, wu_hbm, wd_hbm, gw_hbm,
           out_hbm,
           xs, w3, wphi, wv2, wo, wg, wu, wd, wt, bd, kvs, os_, gs, rs, xsel, ob, sems, osems):
    def x_cp(b):
        t0, n = XBLK[b]
        return pltpu.make_async_copy(x_hbm.at[pl.ds(t0 * T, n * T)],
                                     xs.bitcast(bf16).at[pl.ds(t0 * T, n * T)], sems.at[b])

    def w3_cp(c0, nc, s):
        return pltpu.make_async_copy(wqkv_hbm.at[:, pl.ds(c0, nc)],
                                     w3.bitcast(bf16).at[:, pl.ds(c0, nc)], sems.at[s])

    def whole(src, dst, s):
        return pltpu.make_async_copy(src, dst.bitcast(bf16), sems.at[s])

    grp0 = [pltpu.make_async_copy(wphi_hbm, wphi, sems.at[8]), w3_cp(D, 128, 8), w3_cp(2 * D, 128, 8),
            pltpu.make_async_copy(wr_hbm, wv2.at[0], sems.at[8]),
            pltpu.make_async_copy(gw_hbm, wv2.at[1], sems.at[8])]
    grp1a = [w3_cp(D + 128, 128, 9), w3_cp(2 * D + 128, 128, 9)]
    grp1b = [w3_cp(D + 256, 256, 10), w3_cp(2 * D + 256, 256, 10)]
    grp1c = [w3_cp(D + 512, 512, 11), w3_cp(2 * D + 512, 512, 11)]
    grp2 = [w3_cp(0, D, 12), whole(wg_hbm, wg, 12), whole(wu_hbm, wu, 12),
            whole(wo_hbm, wo, 12), whole(wd_hbm, wd, 12)]

    def out_cp(t, c):
        r0 = pl.multiple_of(t * T, T)
        return pltpu.make_async_copy(ob.bitcast(bf16).at[pl.ds(r0, T), pl.ds(c * 256, 256)],
                                     out_hbm.at[pl.ds(r0, T), pl.ds(c * 256, 256)], osems.at[0])

    for cp in grp0:
        cp.start()
    x_cp(0).start()
    x_cp(1).start()

    row = lax.broadcasted_iota(i32, (128, 128), 0)
    col = lax.broadcasted_iota(i32, (128, 128), 1)
    e_row = lax.broadcasted_iota(i32, (128, DH), 0)
    e_col = lax.broadcasted_iota(i32, (128, DH), 1)
    e = jnp.where((e_row % DH) == e_col, 1.0, 0.0).astype(bf16)
    for cp in grp0:
        cp.wait()
    x_cp(2).start()

    def make_bd(g):
        m = _dot(e, wphi[pl.ds(g * 128, 128), :], NT)
        _st(bd, g * 128, jnp.where((row // DH) == (col // DH), m, 0.0).astype(bf16))

    def fold(g, c0):
        return (_dot(_ld(bd, g * 128, 128), _ld(w3, 0, D, c0, 128), NT) * LOG2E).astype(bf16)

    def prep_kv(g):
        r0 = (g % 2) * 256
        make_bd(g)
        kt = fold(g, D + g * 128)
        vt = _ld(w3, 0, D, 2 * D + g * 128, 128).T
        for p in range(2):
            _st(wt, r0 + p * 128, kt[p * 64:(p + 1) * 64])
            _st(wt, r0 + p * 128 + 64, vt[p * 64:(p + 1) * 64])

    def prep_q(g):
        _st(wt, (g % 2) * 256, fold(g, g * 128))

    r80 = lax.broadcasted_iota(i32, (80, 128), 0)
    c80 = lax.broadcasted_iota(i32, (80, 128), 1)
    kv_mask = jnp.where(r80 < 64, r80 // DH, r80 - 64) == (c80 // 64)

    wr = wv2[0].astype(f32)
    gw = wv2[1].astype(f32)
    score_rows = jnp.concatenate(
        [jnp.concatenate([jnp.broadcast_to(wr[j:j + 1, :], (8, 128)),
                          jnp.broadcast_to(gw[j:j + 1, :], (8, 128))], axis=0) for j in range(8)],
        axis=1).astype(bf16)

    st = {}

    def route():
        r = rs[...]
        pos = lax.broadcasted_iota(i32, r.shape, 0) * T + lax.broadcasted_iota(i32, r.shape, 2)
        m = jnp.max(jnp.where(r == r, r, -jnp.inf))
        idx = jnp.min(jnp.where(r == m, pos, S))
        idx = jnp.where(idx >= S, 0, idx)
        r_sel = jnp.max(jnp.where(pos == idx, r, -jnp.inf))
        st['idx'] = idx
        st['blk'] = blk = pl.multiple_of((idx // 16) * 16, 16)
        st['sg'] = _r16(_sigmoid(jnp.full((16, 128), r_sel, f32)))
        _st(xsel, 0, _ld(xs, blk, 16))

    def ffn_step(k):
        if k < 2 * NF:
            n = k // 2
            if k % 2 == 0:
                st['gt'] = _r16(_dot(_ld(xsel, 0, 16), _ld(wg, 0, D, n * 128, 128), NN))
            else:
                up = _r16(_dot(_ld(xsel, 0, 16), _ld(wu, 0, D, n * 128, 128), NN))
                gt = st.pop('gt')
                st['h', n] = (_r16(gt * _sigmoid(gt)) * up).astype(bf16)
        else:
            n = k - 2 * NF
            yk = _dot(st.pop(('h', n)), _ld(wd, n * 128, 128), NN)
            st['y'] = yk if n == 0 else st['y'] + yk

    jobs = []
    accs = {}

    prep_kv(0)

    def kv_job(g, p, t, c):
        scored = g == 0 and p == 0

        def big():
            if scored:
                for b, (t0, n) in enumerate(XBLK):
                    if t0 == t:
                        x_cp(b).wait()
                        if b + 3 < len(XBLK):
                            x_cp(b + 3).start()
                        if b + 4 == len(XBLK):
                            for cp in grp1a:
                                cp.start()
                        if b + 3 == len(XBLK):
                            for cp in grp1b:
                                cp.start()
                        if b + 1 == len(XBLK):
                            for cp in grp1a:
                                cp.wait()
                            for cp in grp1c:
                                cp.start()
            if g == 1 and c == 2:
                for cp in grp1b:
                    cp.wait()
                for cp in grp2:
                    cp.start()
            if g == 3 and c == 2:
                for cp in grp1c:
                    cp.wait()
            if g == 7 and c == 14:
                for cp in grp2:
                    cp.wait()
            w = _ld(wt, (g % 2) * 256 + p * 128, 128)
            if scored:
                w = jnp.concatenate([w, score_rows], axis=0)
            r = _dot(w, _ld(xs, t * T, T), NT)
            if c == (12 if g == 0 else 14 if g == 7 else 2):
                if g + 1 < NG:
                    prep_kv(g + 1)
                else:
                    prep_q(0)
            if g == 2 and c == 4:
                route()
            return r

        def post(r):
            if scored:
                rs[t] = _r16(r[128:136])
                gate = _sigmoid(r[136:137])
                for u in range(T // 128):
                    gs[pl.ds(t * T + u * 128, 128), :] = _col(gate[:, u * 128:(u + 1) * 128])
            phi = _dual_softmax(r[:64])
            d = _dot(r[64:128].astype(bf16), phi.astype(bf16), NT)
            z = phi[:, :128] + phi[:, 128:]
            key = 2 * g + p
            accs[key] = (d, z) if t == 0 else (accs[key][0] + d, accs[key][1] + z)
            if t == NT_ - 1:
                d, z = accs.pop(key)
                zr = jnp.sum(z.T, axis=0, keepdims=True)
                kv = jnp.concatenate([d, jnp.broadcast_to(zr, (16, 128))], axis=0)
                _st(kvs, key * 80, jnp.where(kv_mask, kv, 0.0).astype(bf16))

        return big, post

    for g in range(NG):
        if g == 0:
            order = [(p, t) for t in range(NT_) for p in range(2)]
        else:
            order = [(p, t) for p in range(2) for t in range(NT_)]
        for c, (p, t) in enumerate(order):
            jobs.append(kv_job(g, p, t, c))

    def q_job(g, t):
        k = g * NT_ + t

        def big():
            r = _dot(_ld(wt, (g % 2) * 256, 128), _ld(xs, t * T, T), NT)
            if t == 2 and g + 1 < NG:
                prep_q(g + 1)
            ffn_step(k)
            return r

        def post(r):
            os = []
            for p in range(2):
                phi = _dual_softmax(r[p * 64:(p + 1) * 64]).astype(bf16)
                nd = _dot(_ld(kvs, (2 * g + p) * 80, 80), phi, NN)
                inv = _recip(nd[64:72] + 1e-6)
                os.append(nd[0:32] * inv[0:1])
                os.append(nd[32:64] * inv[1:2])
            o = jnp.concatenate(os, axis=0).astype(bf16)
            _st(os_, t * T, o.T, g * 128)

        return big, post

    for g in range(NG):
        for t in range(NT_):
            jobs.append(q_job(g, t))
    _pipeline(jobs, LAG)

    idx, blk = st['idx'], st['blk']
    t_last = idx // T
    nsub = (T // TM) * (D // NC)

    def patch():
        y = _r16(_r16(st.pop('y')) * jnp.concatenate([st['sg']] * 8, axis=1))
        sel = lax.broadcasted_iota(i32, (16, D), 0) == (idx - blk)
        xr = _ld(xs, blk, 16).astype(f32)
        _st(xs, blk, jnp.where(sel, xr + y, xr).astype(bf16))

    def out_job(i, m, c):
        t = (t_last + 1 + i) % NT_
        r0 = pl.multiple_of(t * T + m * TM, TM)
        k = NG * NT_ + i * nsub + c * (T // TM) + m

        def big():
            a = _dot(_ld(os_, r0, TM), _ld(wo, 0, D, c * NC, NC), NN)
            if k < 3 * NF:
                ffn_step(k)
            if k == 3 * NF + 2:
                patch()
            return a

        def post(a):
            gate = jnp.concatenate([gs[pl.ds(r0, TM), :]] * (NC // 128), axis=1)
            b = _ld(xs, r0, TM, c * NC, NC).astype(f32)
            _st(ob, r0, (b + gate * (a - b)).astype(bf16), c * NC)
            if m == T // TM - 1 and ((c + 1) * NC) % 256 == 0:
                out_cp(t, ((c + 1) * NC) // 256 - 1).start()

        return big, post

    assert NG * NT_ + (NT_ - 1) * nsub > 3 * NF + 2
    _pipeline([out_job(i, m, c) for i in range(NT_) for c in range(D // NC) for m in range(T // TM)], LAG3)
    pltpu.make_async_copy(ob.bitcast(bf16), out_hbm, osems.at[0]).wait()


@jax.jit
def pallas_gated_mix__linear_kernel_hedgehog__moe_arch_mod__prompt_kernel(A_x, A_wqkv, A_w_phi, A_wo, B_x, B_w_r, B_w_gate, B_w_up, B_w_down, gate_w):
    hbm = pl.BlockSpec(memory_space=pl.ANY)
    out = pl.pallas_call(
        kernel,
        out_shape=jax.ShapeDtypeStruct((S, D), bf16),
        in_specs=[hbm] * 9,
        out_specs=hbm,
        scratch_shapes=[
            pltpu.VMEM((S // 2, D), i32),
            pltpu.VMEM((D // 2, 3 * D), i32),
            pltpu.VMEM((H * DH, DH), bf16),
            pltpu.VMEM((2, 8, 128), bf16),
            pltpu.VMEM((D // 2, D), i32),
            pltpu.VMEM((D // 2, F), i32),
            pltpu.VMEM((D // 2, F), i32),
            pltpu.VMEM((F // 2, D), i32),
            pltpu.VMEM((512 // 2, D), i32),
            pltpu.VMEM((NG * 128 // 2, 128), i32),
            pltpu.VMEM((16 * 80 // 2, 128), i32),
            pltpu.VMEM((S // 2, D), i32),
            pltpu.VMEM((S, 128), f32),
            pltpu.VMEM((NT_, 8, T), f32),
            pltpu.VMEM((8, D), i32),
            pltpu.VMEM((S // 2, D), i32),
            pltpu.SemaphoreType.DMA((13,)),
            pltpu.SemaphoreType.DMA((1,)),
        ],
        compiler_params=pltpu.CompilerParams(vmem_limit_bytes=100 * 1024 * 1024, disable_bounds_checks=True),
    )(A_x.reshape(S, D), A_wqkv, A_w_phi.reshape(H * DH, DH), A_wo,
      B_w_r.reshape(8, 128), B_w_gate, B_w_up, B_w_down, gate_w.reshape(8, 128))
    return out.reshape(1, S, D)
```

```python
import functools
import os
import jax
import jax.numpy as jnp
import numpy as np
from jax import lax
import jax.experimental.pallas as pl
import jax.experimental.pallas.tpu as pltpu

S, D, H, DH, F = 2048, 1024, 32, 32, 3584
NG = 8
T = 256
HT = T // 2
HD = D // 2
NT_ = S // T
NF = F // 128
LOG2E = 1.4426950408889634
ODELAY = int(os.environ.get('ODELAY', 3))
QPOS = tuple(int(v) for v in os.environ.get('QPOS', '0,2,4,6').split(','))
FFN0 = 12
LAGS = tuple(int(v) for v in os.environ.get('LAGS', '2,2,2,2').split(','))

NT = (((1,), (1,)), ((), ()))
NN = (((1,), (0,)), ((), ()))
f32 = jnp.float32
bf16 = jnp.bfloat16
i32 = jnp.int32


def _dot(a, b, dims):
    return lax.dot_general(a, b, dims, preferred_element_type=f32)


def _recip(x):
    r = pl.reciprocal(x, approx=True)
    return r * (2.0 - x * r)


def _sigmoid(x):
    return jax.nn.sigmoid(x)


def _r16(x):
    return x.astype(bf16).astype(f32)


def _ld(ref, r0, n, c0=None, nc=None, dz=None):
    h0 = r0 // 2 if isinstance(r0, int) else pl.multiple_of(r0 // 2, 8)
    if dz is not None:
        h0 = pl.multiple_of(h0 + dz, 8)
    cols = slice(None) if c0 is None else pl.ds(c0, nc)
    return pltpu.bitcast(ref[pl.ds(h0, n // 2), cols], bf16)


def _st(ref, r0, val, c0=None):
    h0 = r0 // 2 if isinstance(r0, int) else pl.multiple_of(r0 // 2, 8)
    cols = slice(None) if c0 is None else pl.ds(c0, val.shape[1])
    ref[pl.ds(h0, val.shape[0] // 2), cols] = pltpu.bitcast(val.astype(bf16), i32)


def _dual_softmax(p):
    outs = []
    for h in range(p.shape[0] // DH):
        ph = p[h * DH:(h + 1) * DH]
        mx = jnp.max(ph, axis=0, keepdims=True)
        mn = jnp.min(ph, axis=0, keepdims=True)
        ep = jnp.exp2(ph - mx)
        en = jnp.exp2(mn - ph)
        sp = jnp.sum(ep, axis=0, keepdims=True)
        sn = jnp.sum(en, axis=0, keepdims=True)
        outs.append(ep * _recip(sp))
        outs.append(en * _recip(sn))
    return jnp.concatenate(outs, axis=0)


def _col(row):
    return jnp.broadcast_to(row, (128, 128)).T


def _lhs_terms(a11, a12, a21, a22):
    return [a11 + a22, a21 + a22, a11, a22, a11 + a12, a21 - a11, a12 - a22]


def _lhs_sums(a11, a12, a21, a22):
    return [a11 + a22, a21 + a22, a11 + a12, a21 - a11, a12 - a22]


def _rhs_sums(b11, b12, b21, b22):
    return [b11 + b22, b12 - b22, b21 - b11, b11 + b12, b21 + b22]


LHS_SLOT = {0: 0, 1: 1, 4: 2, 5: 3, 6: 4}
RHS_SLOT = {0: 0, 2: 1, 3: 2, 5: 3, 6: 4}


def _strassen(prod, between, out):
    m4 = prod(3)
    between(0)
    m2 = prod(1)
    out(2, m2 + m4)
    between(1)
    c11 = m4 + prod(6)
    between(2)
    m1 = prod(0)
    c11 = c11 + m1
    c22 = m1 - m2
    between(3)
    m5 = prod(4)
    out(0, c11 - m5)
    between(4)
    m3 = prod(2)
    out(1, m3 + m5)
    c22 = c22 + m3
    between(5)
    out(3, c22 + prod(5))
    between(6)


def kernel(x_hbm, wqkv_hbm, wphi_hbm, wo_hbm, wr_hbm, wg_hbm, wu_hbm, wd_hbm, gw_hbm,
           out_hbm,
           xs, xq, w3, wphi, wv2, wg, wu, wd, bd, kvs, gs, rs, xsel, ob,
           sems, osems, zsem, *wt):
    OS0 = 5 * HD
    WO0 = 12 * HD
    WS0 = 14 * HD
    zero = pl.semaphore_read(zsem)
    uses = [0]

    def dz():
        uses[0] += 1
        return zero * (8 * uses[0])

    def x_cp(t):
        return pltpu.make_async_copy(x_hbm.at[pl.ds(t * T, T)],
                                     xs.bitcast(bf16).at[pl.ds(t * T, T)], sems.at[t])

    def w3_cp(c0, nc, s):
        return pltpu.make_async_copy(wqkv_hbm.at[:, pl.ds(c0, nc)],
                                     w3.bitcast(bf16).at[:, pl.ds(c0, nc)], sems.at[s])

    def whole(src, dst, s):
        return pltpu.make_async_copy(src, dst.bitcast(bf16), sems.at[s])

    grp0 = [pltpu.make_async_copy(wphi_hbm, wphi, sems.at[8]), w3_cp(D, 128, 8), w3_cp(2 * D, 128, 8),
            pltpu.make_async_copy(wr_hbm, wv2.at[0], sems.at[8]),
            pltpu.make_async_copy(gw_hbm, wv2.at[1], sems.at[8])]
    grp1a = [w3_cp(D + 128, 128, 9), w3_cp(2 * D + 128, 128, 9)]
    grp1b = [w3_cp(D + 256, 256, 10), w3_cp(2 * D + 256, 256, 10)]
    grp1c = [w3_cp(D + 512, 512, 11), w3_cp(2 * D + 512, 512, 11)]
    grp2 = [w3_cp(0, D, 12)]
    for j in range(NT_):
        for u in range(2):
            grp2.append(pltpu.make_async_copy(
                wo_hbm.at[pl.ds(u * HD + j * 64, 64)],
                xq.bitcast(bf16).at[pl.ds(j * HT + u * 64, 64), pl.ds(WO0, D)], sems.at[12]))
    grp3 = [whole(wg_hbm, wg, 13), whole(wu_hbm, wu, 13), whole(wd_hbm, wd, 13)]

    def out_cp(r0, c0, nc):
        return pltpu.make_async_copy(ob.bitcast(bf16).at[pl.ds(r0, T), pl.ds(c0, nc)],
                                     out_hbm.at[pl.ds(r0, T), pl.ds(c0, nc)], osems.at[0])

    for cp in grp0:
        cp.start()
    x_cp(0).start()
    x_cp(1).start()

    row = lax.broadcasted_iota(i32, (128, 128), 0)
    col = lax.broadcasted_iota(i32, (128, 128), 1)
    e_row = lax.broadcasted_iota(i32, (128, DH), 0)
    e_col = lax.broadcasted_iota(i32, (128, DH), 1)
    e = jnp.where((e_row % DH) == e_col, 1.0, 0.0).astype(bf16)
    for cp in grp0:
        cp.wait()
    x_cp(2).start()

    delayed = []

    def defer(gaps, fn):
        delayed.append([gaps, fn])

    def tick():
        for item in delayed:
            item[0] -= 1
        due = [item for item in delayed if item[0] <= 0]
        delayed[:] = [item for item in delayed if item[0] > 0]
        for _, fn in due:
            fn()

    def make_bd(g0, n, gaps=0):
        m = _dot(e, wphi[pl.ds(g0 * 128, n * 128), :], NT)

        def store():
            for g in range(n):
                _st(bd, (g0 + g) * 128,
                    jnp.where((row // DH) == (col // DH), m[:, g * 128:(g + 1) * 128], 0.0))

        defer(gaps, store) if gaps else store()

    def fold(g, c0):
        return _dot(_ld(bd, g * 128, 128), _ld(w3, 0, D, c0, 128), NT) * LOG2E

    def put_lhs(slot, r0, top, bot):
        terms = _lhs_terms(top[:, :HD], top[:, HD:], bot[:, :HD], bot[:, HD:])
        for i, s in enumerate(terms):
            _st(wt[slot], r0, s, i * HD)

    def prep_kv(g):
        kt = fold(g, D + g * 128)
        vt = _ld(w3, 0, D, 2 * D + g * 128, 128).T.astype(f32)
        put_lhs(g, 64, vt[:64], vt[64:])
        put_lhs(g, 0, kt[:64], kt[64:])

    def prep_q(g):
        put_lhs(NG + g, 0, fold(g, g * 128), fold(g + 4, (g + 4) * 128))

    def put_sums(sums, load, dst, rd, cd, n):
        for r in range(0, n, 16):
            for c in range(0, HD, 128):
                b = [load(q, r, c).astype(f32) for q in range(4)]
                for i, s in enumerate(sums(*b)):
                    _st(dst, rd + r, s, cd + i * HD + c)

    def prep_wo(j, r):
        off = dz()
        put_sums(_rhs_sums,
                 lambda q, _, c: _ld(xq, j * HT + (q // 2) * 64 + r, 16, WO0 + (q % 2) * HD + c, 128, off),
                 xq, j * HT + r, WS0, 16)

    def prep_x(t):
        put_sums(_rhs_sums,
                 lambda q, r, c: _ld(xs, t * T + (q % 2) * HT + r, 16, (q // 2) * HD + c, 128),
                 xq, t * HT, 0, HT)

    st = {}
    wr = wv2[0].astype(f32)
    gw = wv2[1].astype(f32)
    score_rows = jnp.concatenate(
        [jnp.concatenate([jnp.broadcast_to(wr[j:j + 1, :], (8, 128)),
                          jnp.broadcast_to(gw[j:j + 1, :], (8, 128))], axis=0) for j in range(8)],
        axis=1).astype(bf16)

    def score_step(t, j):
        u, k0 = j // 2, (j % 2) * HD
        r0 = t * T + u * HT
        d = _dot(score_rows[:, k0:k0 + HD], _ld(xs, r0, HT, k0, HD), NT)
        if j % 2 == 0:
            st['sc'] = d
        else:
            d = d + st.pop('sc')
            rs[:, pl.ds(r0, HT)] = _r16(d[:8])
            gs[pl.ds(r0, HT), :] = _col(_sigmoid(d[8:9]))

    def x_term(i, t):
        if i == 1:
            return _ld(xs, t * T, HT, 0, HD, dz())
        if i == 4:
            return _ld(xs, t * T + HT, HT, HD, HD, dz())
        return _ld(xq, t * HT, HT, RHS_SLOT[i] * HD, HD, dz())

    def proj(slot, t, between, out):
        _strassen(lambda i: _dot(_ld(wt[slot], 0, 128, i * HD, HD, dz()), x_term(i, t), NT), between, out)

    r80 = lax.broadcasted_iota(i32, (80, 128), 0)
    c80 = lax.broadcasted_iota(i32, (80, 128), 1)
    kv_mask = jnp.where(r80 < 64, r80 // DH, r80 - 64) == (c80 // 64)

    def route():
        r = rs[...]
        pos = lax.broadcasted_iota(i32, r.shape, 1)
        m = jnp.max(jnp.where(r == r, r, -jnp.inf))
        idx = jnp.min(jnp.where(r == m, pos, S))
        idx = jnp.where(idx >= S, 0, idx)
        r_sel = jnp.max(jnp.where(pos == idx, r, -jnp.inf))
        st['idx'] = idx
        st['blk'] = blk = pl.multiple_of((idx // 16) * 16, 16)
        st['r_sel'] = r_sel
        _st(xsel, 0, _ld(xs, blk, 16))

    def ffn_step(k):
        n, j = divmod(k, 6)
        if j < 4 and n < NF:
            w = wg if j < 2 else wu
            k0 = (j % 2) * HD
            st['f', j] = _dot(_ld(xsel, 0, 16, k0, HD, dz()), _ld(w, k0, HD, n * 128, 128), NN)
            if j == 3:
                gt = _r16(st.pop(('f', 0)) + st.pop(('f', 1)))
                up = _r16(st.pop(('f', 2)) + st.pop(('f', 3)))
                st['h', n] = (_r16(gt * _sigmoid(gt)) * up).astype(bf16)
        if j >= 4 and 1 <= n <= NF:
            u = j - 4
            yk = _dot(st['h', n - 1], _ld(wd, (n - 1) * 128, 128, u * HD, HD), NN)
            st['y', u] = yk if n == 1 else st['y', u] + yk

    accs = {}

    def kv_post(key, first, last, r):
        phi = _dual_softmax(r[:64])
        d = _dot(r[64:].astype(bf16), phi.astype(bf16), NT)
        accs[key] = (d, phi) if first else (accs[key][0] + d, accs[key][1] + phi)
        if last:
            d, z = accs.pop(key)
            zr = jnp.sum(z.T, axis=0, keepdims=True)
            kv = jnp.concatenate([d, jnp.broadcast_to(zr, (16, 128))], axis=0)
            defer(2, lambda: _st(kvs, key * 80, jnp.where(kv_mask, kv, 0.0)))

    make_bd(0, 4)
    prep_kv(0)
    x_cp(0).wait()
    x_cp(3).start()
    prep_x(0)
    for g in range(NG):
        for t in range(NT_):
            if g == 0 and t + 1 < NT_:
                x_cp(t + 1).wait()
                if t + 4 < NT_:
                    x_cp(t + 4).start()
                if t == 3:
                    for cp in grp1a:
                        cp.start()
                if t == 4:
                    for cp in grp1b:
                        cp.start()
                if t == 6:
                    for cp in grp1a:
                        cp.wait()
                    for cp in grp1c + grp2 + grp3:
                        cp.start()
            if g == 1 and t == 1:
                for cp in grp1b:
                    cp.wait()
            if g == 3 and t == 1:
                for cp in grp1c:
                    cp.wait()
            if g == 7 and t == 1:
                for cp in grp2:
                    cp.wait()

            def between(j):
                tick()
                if g == 0 and j in (0, 1, 3, 4):
                    score_step(t, (0, 1, 3, 4).index(j))
                if j == 0 and t == 4 and g == 1:
                    make_bd(4, 4, 2)
                if j == 6:
                    if g == 0 and t + 1 < NT_:
                        prep_x(t + 1)
                    if t == (6 if g == 0 else 1):
                        if g + 1 < NG:
                            prep_kv(g + 1)
                        else:
                            prep_q(0)
                    if g == 2 and t == 3:
                        route()

            def out(q, c):
                defer(1 + LAGS[q], functools.partial(
                    kv_post, 2 * g + q // 2, t == 0 and q % 2 == 0, t == NT_ - 1 and q % 2 == 1, c))

            proj(g, t, between, out)

    pend = []

    def q_post(g, t, u, r):
        key = 2 * (g + 4 * (u % 2)) + u // 2
        phi = _dual_softmax(r).astype(bf16)
        nd = _dot(_ld(kvs, key * 80, 80, dz=dz()), phi, NN)
        inv = _recip(nd[64:72] + 1e-6)
        o = jnp.concatenate([nd[0:32] * inv[0:1], nd[32:64] * inv[1:2]], axis=0)
        if u % 2 == 0:
            st['o'] = o
            return
        lo = st.pop('o')
        terms = [pltpu.bitcast(v.astype(bf16), i32)
                 for v in _lhs_terms(lo[:, :HT], o[:, :HT], lo[:, HT:], o[:, HT:])]
        if u == 1:
            st['terms'] = terms
            return
        terms = [jnp.concatenate([a, b], axis=0) for a, b in zip(st.pop('terms'), terms)]

        def store(i, n):
            v = pltpu.bitcast(jnp.concatenate(terms[i:i + n], axis=1), bf16).T
            for k in range(n):
                _st(xq, t * HT, v[k * HT:(k + 1) * HT], OS0 + (i + k) * HD + g * 128)

        for i in range(0, 7, 2):
            defer(ODELAY + i // 2, functools.partial(store, i, min(2, 7 - i)))

    for g in range(NG // 2):
        for t in range(NT_):
            if g == 2 and t == 4:
                for cp in grp3:
                    cp.wait()

            def between(j):
                tick()
                if j in QPOS and pend:
                    pend.pop(0)()
                if j in (1, 5) and g in (1, 2):
                    prep_wo((g - 1) * 4 + t // 2, ((t % 2) * 2 + j // 4) * 16)
                if j == 6 and t == 1 and g + 1 < NG // 2:
                    prep_q(g + 1)

            cs = {}
            proj(NG + g, t, between, cs.__setitem__)
            lo = jnp.concatenate([cs[0], cs[1]], axis=1)
            hi = jnp.concatenate([cs[2], cs[3]], axis=1)
            for u, r in enumerate((lo[:64], hi[:64], lo[64:], hi[64:])):
                pend.append(functools.partial(q_post, g, t, u, r))

    while pend:
        pend.pop(0)()
    for k in range(FFN0):
        ffn_step(k)
    while delayed:
        tick()
    idx, blk = st['idx'], st['blk']
    t_last = idx // T

    tiles = [(t_last + 1 + i) & (NT_ - 1) for i in range(NT_)]

    def tile_of(i):
        return tiles[i]

    def o_term(i, k):
        return _ld(xq, 0, HT, OS0 + k * HD, HD, tile_of(i) * (HT // 2) + dz())

    def wo_term(k, c):
        r0, c0 = (0, WO0) if k == 1 else (64, WO0 + HD) if k == 4 else (0, WS0 + RHS_SLOT[k] * HD)
        off = dz()
        return jnp.concatenate(
            [_ld(xq, j * HT + r0, 64, c0 + c * 128, 128, off) for j in range(NT_)], axis=0)

    def patch():
        sg = _r16(_sigmoid(jnp.full((16, D), st['r_sel'], f32)))
        y = jnp.concatenate([st.pop(('y', 0)), st.pop(('y', 1))], axis=1)
        y = _r16(_r16(y) * sg)
        sel = lax.broadcasted_iota(i32, (16, D), 0) == (idx - blk)
        xr = _ld(xs, blk, 16).astype(f32)
        _st(xs, blk, jnp.where(sel, xr + y, xr))

    step = [FFN0]
    for i in range(NT_):
        r0 = pl.multiple_of(tile_of(i) * T, T)
        for c in range(4):
            def between(j):
                tick()
                k = step[0]
                step[0] += 1
                if k < 6 * (NF + 1):
                    ffn_step(k)
                if k == 6 * (NF + 1) + 2:
                    patch()

            def out(q, a):
                rq, cq = r0 + (q // 2) * HT, (q % 2) * HD + c * 128
                gate = gs[pl.ds(pl.multiple_of(rq, HT), HT), :]
                b = _ld(xs, rq, HT, cq, 128).astype(f32)
                _st(ob, rq, b + gate * (a - b), cq)

            _strassen(lambda k: _dot(o_term(i, k), wo_term(k, c), NN), between, out)
            if i == NT_ - 1:
                defer(2, out_cp(r0, c * 128, 128).start)
                defer(2, out_cp(r0, HD + c * 128, 128).start)
        if i < NT_ - 1:
            defer(2, out_cp(r0, 0, D).start)
    assert (NT_ - 1) * 28 > 6 * (NF + 1) + 2
    while delayed:
        tick()
    pltpu.make_async_copy(ob.bitcast(bf16), out_hbm, osems.at[0]).wait()


@jax.jit
def pallas_gated_mix__linear_kernel_hedgehog__moe_arch_mod__prompt_kernel(A_x, A_wqkv, A_w_phi, A_wo, B_x, B_w_r, B_w_gate, B_w_up, B_w_down, gate_w):
    hbm = pl.BlockSpec(memory_space=pl.ANY)
    out = pl.pallas_call(
        kernel,
        out_shape=jax.ShapeDtypeStruct((S, D), bf16),
        in_specs=[hbm] * 9,
        out_specs=hbm,
        scratch_shapes=[
            pltpu.VMEM((S // 2, D), i32),
            pltpu.VMEM((S // 4, 19 * HD), i32),
            pltpu.VMEM((D // 2, 3 * D), i32),
            pltpu.VMEM((H * DH, DH), bf16),
            pltpu.VMEM((2, 8, 128), bf16),
            pltpu.VMEM((D // 2, F), i32),
            pltpu.VMEM((D // 2, F), i32),
            pltpu.VMEM((F // 2, D), i32),
            pltpu.VMEM((NG * 128 // 2, 128), i32),
            pltpu.VMEM((16 * 80 // 2, 128), i32),
            pltpu.VMEM((S, 128), f32),
            pltpu.VMEM((8, S), f32),
            pltpu.VMEM((8, D), i32),
            pltpu.VMEM((S // 2, D), i32),
            pltpu.SemaphoreType.DMA((14,)),
            pltpu.SemaphoreType.DMA((1,)),
            pltpu.SemaphoreType.REGULAR,
        ] + [pltpu.VMEM((64, 7 * HD), i32)] * 12,
        compiler_params=pltpu.CompilerParams(vmem_limit_bytes=110 * 1024 * 1024, disable_bounds_checks=True),
    )(A_x.reshape(S, D), A_wqkv, A_w_phi.reshape(H * DH, DH), A_wo,
      B_w_r.reshape(8, 128), B_w_gate, B_w_up, B_w_down, gate_w.reshape(8, 128))
    return out.reshape(1, S, D)
```

```python
import functools
import os
import jax
import jax.numpy as jnp
import numpy as np
from jax import lax
import jax.experimental.pallas as pl
import jax.experimental.pallas.tpu as pltpu

S, D, H, DH, F = 2048, 1024, 32, 32, 3584
NG = 8
T = 256
HT = T // 2
HD = D // 2
NT_ = S // T
NF = F // 128
LOG2E = 1.4426950408889634
ODELAY = int(os.environ.get('ODELAY', 3))
QPOS = tuple(int(v) for v in os.environ.get('QPOS', '0,2,4,6').split(','))
FFN0 = 12
LAGS = tuple(int(v) for v in os.environ.get('LAGS', '2,2,2,2').split(','))

NT = (((1,), (1,)), ((), ()))
NN = (((1,), (0,)), ((), ()))
f32 = jnp.float32
bf16 = jnp.bfloat16
i32 = jnp.int32


def _dot(a, b, dims):
    return lax.dot_general(a, b, dims, preferred_element_type=f32)


def _recip(x):
    r = pl.reciprocal(x, approx=True)
    return r * (2.0 - x * r)


def _sigmoid(x):
    return jax.nn.sigmoid(x)


def _r16(x):
    return x.astype(bf16).astype(f32)


def _ld(ref, r0, n, c0=None, nc=None, dz=None):
    h0 = r0 // 2 if isinstance(r0, int) else pl.multiple_of(r0 // 2, 8)
    if dz is not None:
        h0 = pl.multiple_of(h0 + dz, 8)
    cols = slice(None) if c0 is None else pl.ds(c0, nc)
    return pltpu.bitcast(ref[pl.ds(h0, n // 2), cols], bf16)


def _st(ref, r0, val, c0=None):
    h0 = r0 // 2 if isinstance(r0, int) else pl.multiple_of(r0 // 2, 8)
    cols = slice(None) if c0 is None else pl.ds(c0, val.shape[1])
    ref[pl.ds(h0, val.shape[0] // 2), cols] = pltpu.bitcast(val.astype(bf16), i32)


def _dual_softmax(p):
    outs = []
    for h in range(p.shape[0] // DH):
        ph = p[h * DH:(h + 1) * DH]
        mx = jnp.max(ph, axis=0, keepdims=True)
        mn = jnp.min(ph, axis=0, keepdims=True)
        ep = jnp.exp2(ph - mx)
        en = jnp.exp2(mn - ph)
        sp = jnp.sum(ep, axis=0, keepdims=True)
        sn = jnp.sum(en, axis=0, keepdims=True)
        outs.append(ep * _recip(sp))
        outs.append(en * _recip(sn))
    return jnp.concatenate(outs, axis=0)


def _col(row):
    return jnp.broadcast_to(row, (128, 128)).T


def _lhs_terms(a11, a12, a21, a22):
    return [a11 + a22, a21 + a22, a11, a22, a11 + a12, a21 - a11, a12 - a22]


def _lhs_sums(a11, a12, a21, a22):
    return [a11 + a22, a21 + a22, a11 + a12, a21 - a11, a12 - a22]


def _rhs_sums(b11, b12, b21, b22):
    return [b11 + b22, b12 - b22, b21 - b11, b11 + b12, b21 + b22]


LHS_SLOT = {0: 0, 1: 1, 4: 2, 5: 3, 6: 4}
RHS_SLOT = {0: 0, 2: 1, 3: 2, 5: 3, 6: 4}


def _strassen(prod, between, out):
    m4 = prod(3)
    between(0)
    m2 = prod(1)
    out(2, m2 + m4)
    between(1)
    c11 = m4 + prod(6)
    between(2)
    m1 = prod(0)
    c11 = c11 + m1
    c22 = m1 - m2
    between(3)
    m5 = prod(4)
    out(0, c11 - m5)
    between(4)
    m3 = prod(2)
    out(1, m3 + m5)
    c22 = c22 + m3
    between(5)
    out(3, c22 + prod(5))
    between(6)


def kernel(x_hbm, wqkv_hbm, wphi_hbm, wo_hbm, wr_hbm, wg_hbm, wu_hbm, wd_hbm, gw_hbm,
           out_hbm,
           xs, xq, w3, wphi, wv2, wg, wu, wd, bd, kvs, gs, rs, xsel, ob,
           sems, osems, zsem, *wt):
    OS0 = 5 * HD
    WO0 = 12 * HD
    WS0 = 14 * HD
    zero = pl.semaphore_read(zsem)
    uses = [0]

    def dz():
        uses[0] += 1
        return zero * (8 * uses[0])

    def x_cp(t):
        return pltpu.make_async_copy(x_hbm.at[pl.ds(t * T, T)],
                                     xs.bitcast(bf16).at[pl.ds(t * T, T)], sems.at[t])

    def w3_cp(c0, nc, s):
        return pltpu.make_async_copy(wqkv_hbm.at[:, pl.ds(c0, nc)],
                                     w3.bitcast(bf16).at[:, pl.ds(c0, nc)], sems.at[s])

    def whole(src, dst, s):
        return pltpu.make_async_copy(src, dst.bitcast(bf16), sems.at[s])

    grp0 = [pltpu.make_async_copy(wphi_hbm, wphi, sems.at[8]), w3_cp(D, 128, 8), w3_cp(2 * D, 128, 8),
            pltpu.make_async_copy(wr_hbm, wv2.at[0], sems.at[8]),
            pltpu.make_async_copy(gw_hbm, wv2.at[1], sems.at[8])]
    grp1a = [w3_cp(D + 128, 128, 9), w3_cp(2 * D + 128, 128, 9)]
    grp1b = [w3_cp(D + 256, 256, 10), w3_cp(2 * D + 256, 256, 10)]
    grp1c = [w3_cp(D + 512, 512, 11), w3_cp(2 * D + 512, 512, 11)]
    grp2 = [w3_cp(0, D, 12)]
    for j in range(NT_):
        for u in range(2):
            grp2.append(pltpu.make_async_copy(
                wo_hbm.at[pl.ds(u * HD + j * 64, 64)],
                xq.bitcast(bf16).at[pl.ds(j * HT + u * 64, 64), pl.ds(WO0, D)], sems.at[12]))
    grp3 = [whole(wg_hbm, wg, 13), whole(wu_hbm, wu, 13), whole(wd_hbm, wd, 13)]

    def out_cp(r0, c0, nc):
        return pltpu.make_async_copy(ob.bitcast(bf16).at[pl.ds(r0, T), pl.ds(c0, nc)],
                                     out_hbm.at[pl.ds(r0, T), pl.ds(c0, nc)], osems.at[0])

    for cp in grp0:
        cp.start()
    x_cp(0).start()
    x_cp(1).start()

    row = lax.broadcasted_iota(i32, (128, 128), 0)
    col = lax.broadcasted_iota(i32, (128, 128), 1)
    e_row = lax.broadcasted_iota(i32, (128, DH), 0)
    e_col = lax.broadcasted_iota(i32, (128, DH), 1)
    e = jnp.where((e_row % DH) == e_col, 1.0, 0.0).astype(bf16)
    for cp in grp0:
        cp.wait()
    x_cp(2).start()

    delayed = []

    def defer(gaps, fn):
        delayed.append([gaps, fn])

    def tick():
        for item in delayed:
            item[0] -= 1
        due = [item for item in delayed if item[0] <= 0]
        delayed[:] = [item for item in delayed if item[0] > 0]
        for _, fn in due:
            fn()

    def make_bd(g0, n, gaps=0):
        m = _dot(e, wphi[pl.ds(g0 * 128, n * 128), :], NT)

        def store():
            for g in range(n):
                _st(bd, (g0 + g) * 128,
                    jnp.where((row // DH) == (col // DH), m[:, g * 128:(g + 1) * 128], 0.0))

        defer(gaps, store) if gaps else store()

    def fold(g, c0):
        return _dot(_ld(bd, g * 128, 128), _ld(w3, 0, D, c0, 128), NT) * LOG2E

    def put_lhs(slot, r0, top, bot):
        terms = _lhs_terms(top[:, :HD], top[:, HD:], bot[:, :HD], bot[:, HD:])
        for i, s in enumerate(terms):
            _st(wt[slot], r0, s, i * HD)

    def prep_kv(g):
        kt = fold(g, D + g * 128)
        vt = _ld(w3, 0, D, 2 * D + g * 128, 128).T.astype(f32)
        put_lhs(g, 64, vt[:64], vt[64:])
        put_lhs(g, 0, kt[:64], kt[64:])

    def prep_q(g):
        put_lhs(NG + g, 0, fold(g, g * 128), fold(g + 4, (g + 4) * 128))

    def put_sums(sums, load, dst, rd, cd, n):
        for r in range(0, n, 16):
            for c in range(0, HD, 128):
                b = [load(q, r, c).astype(f32) for q in range(4)]
                for i, s in enumerate(sums(*b)):
                    _st(dst, rd + r, s, cd + i * HD + c)

    def prep_wo(j, r):
        off = dz()
        put_sums(_rhs_sums,
                 lambda q, _, c: _ld(xq, j * HT + (q // 2) * 64 + r, 16, WO0 + (q % 2) * HD + c, 128, off),
                 xq, j * HT + r, WS0, 16)

    def prep_x(t):
        put_sums(_rhs_sums,
                 lambda q, r, c: _ld(xs, t * T + (q % 2) * HT + r, 16, (q // 2) * HD + c, 128),
                 xq, t * HT, 0, HT)

    st = {}
    wr = wv2[0].astype(f32)
    gw = wv2[1].astype(f32)
    score_rows = jnp.concatenate(
        [jnp.concatenate([jnp.broadcast_to(wr[j:j + 1, :], (8, 128)),
                          jnp.broadcast_to(gw[j:j + 1, :], (8, 128))], axis=0) for j in range(8)],
        axis=1).astype(bf16)

    def score_step(t, j):
        u, k0 = j // 2, (j % 2) * HD
        r0 = t * T + u * HT
        d = _dot(score_rows[:, k0:k0 + HD], _ld(xs, r0, HT, k0, HD), NT)
        if j % 2 == 0:
            st['sc'] = d
        else:
            d = d + st.pop('sc')
            rs[:, pl.ds(r0, HT)] = _r16(d[:8])
            gs[pl.ds(r0, HT), :] = _col(_sigmoid(d[8:9]))

    def x_term(i, t):
        if i == 1:
            return _ld(xs, t * T, HT, 0, HD, dz())
        if i == 4:
            return _ld(xs, t * T + HT, HT, HD, HD, dz())
        return _ld(xq, t * HT, HT, RHS_SLOT[i] * HD, HD, dz())

    def proj(slot, t, between, out):
        _strassen(lambda i: _dot(_ld(wt[slot], 0, 128, i * HD, HD, dz()), x_term(i, t), NT), between, out)

    r80 = lax.broadcasted_iota(i32, (80, 128), 0)
    c80 = lax.broadcasted_iota(i32, (80, 128), 1)
    kv_mask = jnp.where(r80 < 64, r80 // DH, r80 - 64) == (c80 // 64)

    def route():
        r = rs[...]
        pos = lax.broadcasted_iota(i32, r.shape, 1)
        m = jnp.max(jnp.where(r == r, r, -jnp.inf))
        idx = jnp.min(jnp.where(r == m, pos, S))
        idx = jnp.where(idx >= S, 0, idx)
        r_sel = jnp.max(jnp.where(pos == idx, r, -jnp.inf))
        st['idx'] = idx
        st['blk'] = blk = pl.multiple_of((idx // 16) * 16, 16)
        st['r_sel'] = r_sel
        _st(xsel, 0, _ld(xs, blk, 16))

    def ffn_step(k):
        n, j = divmod(k, 3)
        if j < 2 and n < NF:
            st['f', j] = _dot(_ld(xsel, 0, 16, dz=dz()), _ld((wg, wu)[j], 0, D, n * 128, 128), NN)
            if j == 1:
                gt = _r16(st.pop(('f', 0)))
                up = _r16(st.pop(('f', 1)))
                st['h', n] = (_r16(gt * _sigmoid(gt)) * up).astype(bf16)
        if j == 2 and 1 <= n <= NF:
            yk = _dot(st.pop(('h', n - 1)), _ld(wd, (n - 1) * 128, 128), NN)
            st['y'] = yk if n == 1 else st['y'] + yk

    accs = {}

    def kv_post(key, first, last, r):
        phi = _dual_softmax(r[:64])
        d = _dot(r[64:].astype(bf16), phi.astype(bf16), NT)
        accs[key] = (d, phi) if first else (accs[key][0] + d, accs[key][1] + phi)
        if last:
            d, z = accs.pop(key)
            zr = jnp.sum(z.T, axis=0, keepdims=True)
            kv = jnp.concatenate([d, jnp.broadcast_to(zr, (16, 128))], axis=0)
            defer(2, lambda: _st(kvs, key * 80, jnp.where(kv_mask, kv, 0.0)))

    make_bd(0, 4)
    prep_kv(0)
    x_cp(0).wait()
    x_cp(3).start()
    prep_x(0)
    for g in range(NG):
        for t in range(NT_):
            if g == 0 and t + 1 < NT_:
                x_cp(t + 1).wait()
                if t + 4 < NT_:
                    x_cp(t + 4).start()
                if t == 3:
                    for cp in grp1a:
                        cp.start()
                if t == 4:
                    for cp in grp1b:
                        cp.start()
                if t == 6:
                    for cp in grp1a:
                        cp.wait()
                    for cp in grp1c + grp2 + grp3:
                        cp.start()
            if g == 1 and t == 1:
                for cp in grp1b:
                    cp.wait()
            if g == 3 and t == 1:
                for cp in grp1c:
                    cp.wait()
            if g == 7 and t == 1:
                for cp in grp2:
                    cp.wait()

            def between(j):
                tick()
                if g == 0 and j in (0, 1, 3, 4):
                    score_step(t, (0, 1, 3, 4).index(j))
                if j == 0 and t == 4 and g == 1:
                    make_bd(4, 4, 2)
                if j == 6:
                    if g == 0 and t + 1 < NT_:
                        prep_x(t + 1)
                    if t == (6 if g == 0 else 1):
                        if g + 1 < NG:
                            prep_kv(g + 1)
                        else:
                            prep_q(0)
                    if g == 2 and t == 3:
                        route()

            def out(q, c):
                defer(1 + LAGS[q], functools.partial(
                    kv_post, 2 * g + q // 2, t == 0 and q % 2 == 0, t == NT_ - 1 and q % 2 == 1, c))

            proj(g, t, between, out)

    pend = []

    def q_post(g, t, u, r):
        key = 2 * (g + 4 * (u % 2)) + u // 2
        phi = _dual_softmax(r).astype(bf16)
        nd = _dot(_ld(kvs, key * 80, 80, dz=dz()), phi, NN)
        inv = _recip(nd[64:72] + 1e-6)
        o = jnp.concatenate([nd[0:32] * inv[0:1], nd[32:64] * inv[1:2]], axis=0)
        if u % 2 == 0:
            st['o'] = o
            return
        lo = st.pop('o')
        terms = [pltpu.bitcast(v.astype(bf16), i32)
                 for v in _lhs_terms(lo[:, :HT], o[:, :HT], lo[:, HT:], o[:, HT:])]
        if u == 1:
            st['terms'] = terms
            return
        terms = [jnp.concatenate([a, b], axis=0) for a, b in zip(st.pop('terms'), terms)]

        def store(i, n):
            v = pltpu.bitcast(jnp.concatenate(terms[i:i + n], axis=1), bf16).T
            for k in range(n):
                _st(xq, t * HT, v[k * HT:(k + 1) * HT], OS0 + (i + k) * HD + g * 128)

        for i in range(0, 7, 2):
            defer(ODELAY + i // 2, functools.partial(store, i, min(2, 7 - i)))

    for g in range(NG // 2):
        for t in range(NT_):
            if g == 2 and t == 4:
                for cp in grp3:
                    cp.wait()

            def between(j):
                tick()
                if j in QPOS and pend:
                    pend.pop(0)()
                if j in (1, 5) and g in (1, 2):
                    prep_wo((g - 1) * 4 + t // 2, ((t % 2) * 2 + j // 4) * 16)
                if j == 6 and t == 1 and g + 1 < NG // 2:
                    prep_q(g + 1)

            cs = {}
            proj(NG + g, t, between, cs.__setitem__)
            lo = jnp.concatenate([cs[0], cs[1]], axis=1)
            hi = jnp.concatenate([cs[2], cs[3]], axis=1)
            for u, r in enumerate((lo[:64], hi[:64], lo[64:], hi[64:])):
                pend.append(functools.partial(q_post, g, t, u, r))

    while pend:
        pend.pop(0)()
    for k in range(FFN0 // 2):
        ffn_step(k)
    while delayed:
        tick()
    idx, blk = st['idx'], st['blk']
    t_last = idx // T

    tiles = [(t_last + 1 + i) & (NT_ - 1) for i in range(NT_)]

    def tile_of(i):
        return tiles[i]

    def o_term(i, k):
        return _ld(xq, 0, HT, OS0 + k * HD, HD, tile_of(i) * (HT // 2) + dz())

    def wo_term(k, c):
        r0, c0 = (0, WO0) if k == 1 else (64, WO0 + HD) if k == 4 else (0, WS0 + RHS_SLOT[k] * HD)
        off = dz()
        return jnp.concatenate(
            [_ld(xq, j * HT + r0, 64, c0 + c * 128, 128, off) for j in range(NT_)], axis=0)

    def patch():
        sg = _r16(_sigmoid(jnp.full((16, D), st['r_sel'], f32)))
        y = _r16(_r16(st.pop('y')) * sg)
        sel = lax.broadcasted_iota(i32, (16, D), 0) == (idx - blk)
        xr = _ld(xs, blk, 16).astype(f32)
        _st(xs, blk, jnp.where(sel, xr + y, xr))

    step = [FFN0]
    for i in range(NT_):
        r0 = pl.multiple_of(tile_of(i) * T, T)
        for c in range(4):
            def between(j):
                tick()
                k = step[0]
                step[0] += 1
                if k % 2 == 0 and k < 6 * (NF + 1):
                    ffn_step(k // 2)
                if k == 6 * (NF + 1) + 2:
                    patch()

            def out(q, a):
                rq, cq = r0 + (q // 2) * HT, (q % 2) * HD + c * 128
                gate = gs[pl.ds(pl.multiple_of(rq, HT), HT), :]
                b = _ld(xs, rq, HT, cq, 128).astype(f32)
                _st(ob, rq, b + gate * (a - b), cq)

            _strassen(lambda k: _dot(o_term(i, k), wo_term(k, c), NN), between, out)
            defer(4, out_cp(r0, c * 128, 128).start)
            defer(4, out_cp(r0, HD + c * 128, 128).start)
    assert (NT_ - 1) * 28 > 6 * (NF + 1) + 2
    while delayed:
        tick()
    pltpu.make_async_copy(ob.bitcast(bf16), out_hbm, osems.at[0]).wait()


@jax.jit
def pallas_gated_mix__linear_kernel_hedgehog__moe_arch_mod__prompt_kernel(A_x, A_wqkv, A_w_phi, A_wo, B_x, B_w_r, B_w_gate, B_w_up, B_w_down, gate_w):
    hbm = pl.BlockSpec(memory_space=pl.ANY)
    out = pl.pallas_call(
        kernel,
        out_shape=jax.ShapeDtypeStruct((S, D), bf16),
        in_specs=[hbm] * 9,
        out_specs=hbm,
        scratch_shapes=[
            pltpu.VMEM((S // 2, D), i32),
            pltpu.VMEM((S // 4, 19 * HD), i32),
            pltpu.VMEM((D // 2, 3 * D), i32),
            pltpu.VMEM((H * DH, DH), bf16),
            pltpu.VMEM((2, 8, 128), bf16),
            pltpu.VMEM((D // 2, F), i32),
            pltpu.VMEM((D // 2, F), i32),
            pltpu.VMEM((F // 2, D), i32),
            pltpu.VMEM((NG * 128 // 2, 128), i32),
            pltpu.VMEM((16 * 80 // 2, 128), i32),
            pltpu.VMEM((S, 128), f32),
            pltpu.VMEM((8, S), f32),
            pltpu.VMEM((8, D), i32),
            pltpu.VMEM((S // 2, D), i32),
            pltpu.SemaphoreType.DMA((14,)),
            pltpu.SemaphoreType.DMA((1,)),
            pltpu.SemaphoreType.REGULAR,
        ] + [pltpu.VMEM((64, 7 * HD), i32)] * 12,
        compiler_params=pltpu.CompilerParams(vmem_limit_bytes=110 * 1024 * 1024, disable_bounds_checks=True),
    )(A_x.reshape(S, D), A_wqkv, A_w_phi.reshape(H * DH, DH), A_wo,
      B_w_r.reshape(8, 128), B_w_gate, B_w_up, B_w_down, gate_w.reshape(8, 128))
    return out.reshape(1, S, D)
```

```python
import functools
import os
import jax
import jax.numpy as jnp
import numpy as np
from jax import lax
import jax.experimental.pallas as pl
import jax.experimental.pallas.tpu as pltpu

S, D, H, DH, F = 2048, 1024, 32, 32, 3584
NG = 8
T = 256
HT = T // 2
HD = D // 2
NT_ = S // T
NF = F // 128
LOG2E = 1.4426950408889634
ODELAY = int(os.environ.get('ODELAY', 3))
QPOS = tuple(int(v) for v in os.environ.get('QPOS', '0,2,4,6').split(','))
FFN0 = 12
LAGS = tuple(int(v) for v in os.environ.get('LAGS', '2,2,2,2').split(','))

NT = (((1,), (1,)), ((), ()))
NN = (((1,), (0,)), ((), ()))
f32 = jnp.float32
bf16 = jnp.bfloat16
i32 = jnp.int32


def _dot(a, b, dims):
    return lax.dot_general(a, b, dims, preferred_element_type=f32)


def _recip(x):
    r = pl.reciprocal(x, approx=True)
    return r * (2.0 - x * r)


def _sigmoid(x):
    return jax.nn.sigmoid(x)


def _r16(x):
    return x.astype(bf16).astype(f32)


def _ld(ref, r0, n, c0=None, nc=None, dz=None):
    h0 = r0 // 2 if isinstance(r0, int) else pl.multiple_of(r0 // 2, 8)
    if dz is not None:
        h0 = pl.multiple_of(h0 + dz, 8)
    cols = slice(None) if c0 is None else pl.ds(c0, nc)
    return pltpu.bitcast(ref[pl.ds(h0, n // 2), cols], bf16)


def _st(ref, r0, val, c0=None):
    h0 = r0 // 2 if isinstance(r0, int) else pl.multiple_of(r0 // 2, 8)
    cols = slice(None) if c0 is None else pl.ds(c0, val.shape[1])
    ref[pl.ds(h0, val.shape[0] // 2), cols] = pltpu.bitcast(val.astype(bf16), i32)


def _dual_softmax(p):
    outs = []
    for h in range(p.shape[0] // DH):
        ph = p[h * DH:(h + 1) * DH]
        mx = jnp.max(ph, axis=0, keepdims=True)
        mn = jnp.min(ph, axis=0, keepdims=True)
        ep = jnp.exp2(ph - mx)
        en = jnp.exp2(mn - ph)
        sp = jnp.sum(ep, axis=0, keepdims=True)
        sn = jnp.sum(en, axis=0, keepdims=True)
        outs.append(ep * _recip(sp))
        outs.append(en * _recip(sn))
    return jnp.concatenate(outs, axis=0)


def _col(row):
    return jnp.broadcast_to(row, (128, 128)).T


def _lhs_terms(a11, a12, a21, a22):
    return [a11 + a22, a21 + a22, a11, a22, a11 + a12, a21 - a11, a12 - a22]


def _lhs_sums(a11, a12, a21, a22):
    return [a11 + a22, a21 + a22, a11 + a12, a21 - a11, a12 - a22]


def _rhs_sums(b11, b12, b21, b22):
    return [b11 + b22, b12 - b22, b21 - b11, b11 + b12, b21 + b22]


LHS_SLOT = {0: 0, 1: 1, 4: 2, 5: 3, 6: 4}
RHS_SLOT = {0: 0, 2: 1, 3: 2, 5: 3, 6: 4}


def _strassen(prod, between, out):
    m4 = prod(3)
    between(0)
    m2 = prod(1)
    out(2, m2 + m4)
    between(1)
    c11 = m4 + prod(6)
    between(2)
    m1 = prod(0)
    c11 = c11 + m1
    c22 = m1 - m2
    between(3)
    m5 = prod(4)
    out(0, c11 - m5)
    between(4)
    m3 = prod(2)
    out(1, m3 + m5)
    c22 = c22 + m3
    between(5)
    out(3, c22 + prod(5))
    between(6)


def kernel(x_hbm, wqkv_hbm, wphi_hbm, wo_hbm, wr_hbm, wg_hbm, wu_hbm, wd_hbm, gw_hbm,
           out_hbm,
           xs, xq, w3, wphi, wv2, wg, wu, wd, bd, kvs, gs, rs, xsel, ob,
           sems, osems, zsem, *wt):
    OS0 = 5 * HD
    WO0 = 12 * HD
    WS0 = 14 * HD
    zero = pl.semaphore_read(zsem)
    uses = [0]

    def dz():
        uses[0] += 1
        return zero * (8 * uses[0])

    def x_cp(t):
        return pltpu.make_async_copy(x_hbm.at[pl.ds(t * T, T)],
                                     xs.bitcast(bf16).at[pl.ds(t * T, T)], sems.at[t])

    def w3_cp(c0, nc, s):
        return pltpu.make_async_copy(wqkv_hbm.at[:, pl.ds(c0, nc)],
                                     w3.bitcast(bf16).at[:, pl.ds(c0, nc)], sems.at[s])

    def whole(src, dst, s):
        return pltpu.make_async_copy(src, dst.bitcast(bf16), sems.at[s])

    grp0 = [pltpu.make_async_copy(wphi_hbm.at[pl.ds(0, 128)], wphi.at[pl.ds(0, 128)], sems.at[8]),
            w3_cp(D, 128, 8), w3_cp(2 * D, 128, 8),
            pltpu.make_async_copy(wr_hbm, wv2.at[0], sems.at[8]),
            pltpu.make_async_copy(gw_hbm, wv2.at[1], sems.at[8])]
    grp1 = [pltpu.make_async_copy(wphi_hbm.at[pl.ds(128, 896)], wphi.at[pl.ds(128, 896)], sems.at[9]),
            w3_cp(D + 128, 128, 9), w3_cp(2 * D + 128, 128, 9)]
    grp2 = [w3_cp(c0 + g * 128, 128, 10) for g in (2, 3) for c0 in (D, 2 * D)]

    def rows(src, dst, r0, n, s):
        return pltpu.make_async_copy(src.at[pl.ds(r0, n)], dst.bitcast(bf16).at[pl.ds(r0, n)], sems.at[s])

    grp3 = [w3_cp(D + 512, 512, 11), w3_cp(2 * D + 512, 512, 11), w3_cp(0, D, 11)]
    for j in range(NT_):
        for u in range(2):
            grp3.append(pltpu.make_async_copy(
                wo_hbm.at[pl.ds(u * HD + j * 64, 64)],
                xq.bitcast(bf16).at[pl.ds(j * HT + u * 64, 64), pl.ds(WO0, D)], sems.at[11]))
    grp4 = [rows(src, dst, r, 64, 12) for src, dst in ((wg_hbm, wg), (wu_hbm, wu)) for r in range(0, D, 64)]
    grp4 += [rows(wd_hbm, wd, r, 128, 12) for r in range(0, F, 128)]
    stream = list(grp4)

    def feed(n):
        for _ in range(n):
            if stream:
                stream.pop(0).start()

    def out_cp(r0, c0, nc):
        return pltpu.make_async_copy(ob.bitcast(bf16).at[pl.ds(r0, T), pl.ds(c0, nc)],
                                     out_hbm.at[pl.ds(r0, T), pl.ds(c0, nc)], osems.at[0])

    for cp in grp0:
        cp.start()
    x_cp(0).start()
    for cp in grp1:
        cp.start()
    x_cp(1).start()

    row = lax.broadcasted_iota(i32, (128, 128), 0)
    col = lax.broadcasted_iota(i32, (128, 128), 1)
    e_row = lax.broadcasted_iota(i32, (128, DH), 0)
    e_col = lax.broadcasted_iota(i32, (128, DH), 1)
    e = jnp.where((e_row % DH) == e_col, 1.0, 0.0).astype(bf16)
    for cp in grp0:
        cp.wait()
    x_cp(2).start()

    delayed = []

    def defer(gaps, fn):
        delayed.append([gaps, fn])

    def tick():
        for item in delayed:
            item[0] -= 1
        due = [item for item in delayed if item[0] <= 0]
        delayed[:] = [item for item in delayed if item[0] > 0]
        for _, fn in due:
            fn()

    def make_bd(g0, n, gaps=0):
        m = _dot(e, wphi[pl.ds(g0 * 128, n * 128), :], NT)

        def store():
            for g in range(n):
                _st(bd, (g0 + g) * 128,
                    jnp.where((row // DH) == (col // DH), m[:, g * 128:(g + 1) * 128], 0.0))

        defer(gaps, store) if gaps else store()

    def fold(g, c0):
        return _dot(_ld(bd, g * 128, 128), _ld(w3, 0, D, c0, 128), NT) * LOG2E

    def put_lhs(slot, r0, top, bot):
        terms = _lhs_terms(top[:, :HD], top[:, HD:], bot[:, :HD], bot[:, HD:])
        for i, s in enumerate(terms):
            _st(wt[slot], r0, s, i * HD)

    def prep_kv(g):
        kt = fold(g, D + g * 128)
        vt = _ld(w3, 0, D, 2 * D + g * 128, 128).T.astype(f32)
        put_lhs(g, 64, vt[:64], vt[64:])
        put_lhs(g, 0, kt[:64], kt[64:])

    def prep_q(g):
        put_lhs(NG + g, 0, fold(g, g * 128), fold(g + 4, (g + 4) * 128))

    def put_sums(sums, load, dst, rd, cd, n):
        for r in range(0, n, 16):
            for c in range(0, HD, 128):
                b = [load(q, r, c).astype(f32) for q in range(4)]
                for i, s in enumerate(sums(*b)):
                    _st(dst, rd + r, s, cd + i * HD + c)

    def prep_wo(j, r):
        off = dz()
        put_sums(_rhs_sums,
                 lambda q, _, c: _ld(xq, j * HT + (q // 2) * 64 + r, 16, WO0 + (q % 2) * HD + c, 128, off),
                 xq, j * HT + r, WS0, 16)

    def prep_x(t):
        put_sums(_rhs_sums,
                 lambda q, r, c: _ld(xs, t * T + (q % 2) * HT + r, 16, (q // 2) * HD + c, 128),
                 xq, t * HT, 0, HT)

    st = {}
    wr = wv2[0].astype(f32)
    gw = wv2[1].astype(f32)
    score_rows = jnp.concatenate(
        [jnp.concatenate([jnp.broadcast_to(wr[j:j + 1, :], (8, 128)),
                          jnp.broadcast_to(gw[j:j + 1, :], (8, 128))], axis=0) for j in range(8)],
        axis=1).astype(bf16)

    def score_step(t, j):
        u, k0 = j // 2, (j % 2) * HD
        r0 = t * T + u * HT
        d = _dot(score_rows[:, k0:k0 + HD], _ld(xs, r0, HT, k0, HD), NT)
        if j % 2 == 0:
            st['sc'] = d
        else:
            d = d + st.pop('sc')
            rs[:, pl.ds(r0, HT)] = _r16(d[:8])
            gs[pl.ds(r0, HT), :] = _col(_sigmoid(d[8:9]))

    def x_term(i, t):
        if i == 1:
            return _ld(xs, t * T, HT, 0, HD, dz())
        if i == 4:
            return _ld(xs, t * T + HT, HT, HD, HD, dz())
        return _ld(xq, t * HT, HT, RHS_SLOT[i] * HD, HD, dz())

    def proj(slot, t, between, out):
        _strassen(lambda i: _dot(_ld(wt[slot], 0, 128, i * HD, HD, dz()), x_term(i, t), NT), between, out)

    r80 = lax.broadcasted_iota(i32, (80, 128), 0)
    c80 = lax.broadcasted_iota(i32, (80, 128), 1)
    kv_mask = jnp.where(r80 < 64, r80 // DH, r80 - 64) == (c80 // 64)

    def route():
        r = rs[...]
        pos = lax.broadcasted_iota(i32, r.shape, 1)
        m = jnp.max(jnp.where(r == r, r, -jnp.inf))
        idx = jnp.min(jnp.where(r == m, pos, S))
        idx = jnp.where(idx >= S, 0, idx)
        r_sel = jnp.max(jnp.where(pos == idx, r, -jnp.inf))
        st['idx'] = idx
        st['blk'] = blk = pl.multiple_of((idx // 16) * 16, 16)
        st['r_sel'] = r_sel
        _st(xsel, 0, _ld(xs, blk, 16))

    def ffn_step(k):
        n, j = divmod(k, 3)
        if j < 2 and n < NF:
            st['f', j] = _dot(_ld(xsel, 0, 16, dz=dz()), _ld((wg, wu)[j], 0, D, n * 128, 128), NN)
            if j == 1:
                gt = _r16(st.pop(('f', 0)))
                up = _r16(st.pop(('f', 1)))
                st['h', n] = (_r16(gt * _sigmoid(gt)) * up).astype(bf16)
        if j == 2 and 1 <= n <= NF:
            yk = _dot(st.pop(('h', n - 1)), _ld(wd, (n - 1) * 128, 128), NN)
            st['y'] = yk if n == 1 else st['y'] + yk

    accs = {}

    def kv_post(key, first, last, r):
        phi = _dual_softmax(r[:64])
        d = _dot(r[64:].astype(bf16), phi.astype(bf16), NT)
        accs[key] = (d, phi) if first else (accs[key][0] + d, accs[key][1] + phi)
        if last:
            d, z = accs.pop(key)
            zr = jnp.sum(z.T, axis=0, keepdims=True)
            kv = jnp.concatenate([d, jnp.broadcast_to(zr, (16, 128))], axis=0)
            defer(2, lambda: _st(kvs, key * 80, jnp.where(kv_mask, kv, 0.0)))

    make_bd(0, 1)
    prep_kv(0)
    xblocks = {0: (0,), 1: (1,), 2: (2, 3), 4: (4, 5), 6: (6, 7)}
    order = [(g, t) for t in range(NT_) for g in range(2)] + [(g, t) for g in range(2, NG) for t in range(NT_)]
    for g, t in order:
        if True:
            if g == 0 and t in xblocks:
                for u in xblocks[t]:
                    x_cp(u).wait()
                if t == 0:
                    x_cp(3).start()
                if t == 1:
                    x_cp(4).start()
                    x_cp(5).start()
                if t == 2:
                    x_cp(6).start()
                    x_cp(7).start()
                    for cp in grp2:
                        cp.start()
                if t == 4:
                    for cp in grp3:
                        cp.start()
                if t == 6:
                    for cp in grp2:
                        cp.wait()
                prep_x(t)
            if g == 1 and t == 0:
                for cp in grp1:
                    cp.wait()
                make_bd(1, 7)
                prep_kv(1)
            if g == 3 and t == 1:
                for cp in grp3:
                    cp.wait()

            def between(j):
                tick()
                if g == 1 and j in (0, 1, 3, 4):
                    score_step(t, (0, 1, 3, 4).index(j))
                if j == 3 and g >= 3:
                    feed(1)
                if j == 2 and g == 1 and t + 1 < NT_ and t + 1 not in xblocks:
                    prep_x(t + 1)
                if j == 6:
                    if g >= 1 and t == (6 if g == 1 else 1):
                        if g + 1 < NG:
                            prep_kv(g + 1)
                        else:
                            prep_q(0)
                    if g == 2 and t == 3:
                        route()

            def out(q, c):
                defer(1 + LAGS[q], functools.partial(
                    kv_post, 2 * g + q // 2, t == 0 and q % 2 == 0, t == NT_ - 1 and q % 2 == 1, c))

            proj(g, t, between, out)

    pend = []

    def q_post(g, t, u, r):
        key = 2 * (g + 4 * (u % 2)) + u // 2
        phi = _dual_softmax(r).astype(bf16)
        nd = _dot(_ld(kvs, key * 80, 80, dz=dz()), phi, NN)
        inv = _recip(nd[64:72] + 1e-6)
        o = jnp.concatenate([nd[0:32] * inv[0:1], nd[32:64] * inv[1:2]], axis=0)
        if u % 2 == 0:
            st['o'] = o
            return
        lo = st.pop('o')
        terms = [pltpu.bitcast(v.astype(bf16), i32)
                 for v in _lhs_terms(lo[:, :HT], o[:, :HT], lo[:, HT:], o[:, HT:])]
        if u == 1:
            st['terms'] = terms
            return
        terms = [jnp.concatenate([a, b], axis=0) for a, b in zip(st.pop('terms'), terms)]

        def store(i, n):
            v = pltpu.bitcast(jnp.concatenate(terms[i:i + n], axis=1), bf16).T
            for k in range(n):
                _st(xq, t * HT, v[k * HT:(k + 1) * HT], OS0 + (i + k) * HD + g * 128)

        for i in range(0, 7, 2):
            defer(ODELAY + i // 2, functools.partial(store, i, min(2, 7 - i)))

    for g in range(NG // 2):
        for t in range(NT_):
            def between(j):
                tick()
                if j == 3:
                    feed(1)
                if j in QPOS and pend:
                    pend.pop(0)()
                if j in (1, 5) and g in (1, 2):
                    prep_wo((g - 1) * 4 + t // 2, ((t % 2) * 2 + j // 4) * 16)
                if j == 6 and t == 1 and g + 1 < NG // 2:
                    prep_q(g + 1)

            cs = {}
            proj(NG + g, t, between, cs.__setitem__)
            lo = jnp.concatenate([cs[0], cs[1]], axis=1)
            hi = jnp.concatenate([cs[2], cs[3]], axis=1)
            for u, r in enumerate((lo[:64], hi[:64], lo[64:], hi[64:])):
                pend.append(functools.partial(q_post, g, t, u, r))

    assert not stream
    for cp in grp4:
        cp.wait()
    while pend:
        pend.pop(0)()
    for k in range(FFN0 // 2):
        ffn_step(k)
    while delayed:
        tick()
    idx, blk = st['idx'], st['blk']
    t_last = idx // T

    tiles = [(t_last + 1 + i) & (NT_ - 1) for i in range(NT_)]

    def tile_of(i):
        return tiles[i]

    def o_term(i, k):
        return _ld(xq, 0, HT, OS0 + k * HD, HD, tile_of(i) * (HT // 2) + dz())

    def wo_term(k, c):
        r0, c0 = (0, WO0) if k == 1 else (64, WO0 + HD) if k == 4 else (0, WS0 + RHS_SLOT[k] * HD)
        off = dz()
        return jnp.concatenate(
            [_ld(xq, j * HT + r0, 64, c0 + c * 128, 128, off) for j in range(NT_)], axis=0)

    def patch():
        sg = _r16(_sigmoid(jnp.full((16, D), st['r_sel'], f32)))
        y = _r16(_r16(st.pop('y')) * sg)
        sel = lax.broadcasted_iota(i32, (16, D), 0) == (idx - blk)
        xr = _ld(xs, blk, 16).astype(f32)
        _st(xs, blk, jnp.where(sel, xr + y, xr))

    step = [FFN0]
    for i in range(NT_):
        r0 = pl.multiple_of(tile_of(i) * T, T)
        for c in range(4):
            def between(j):
                tick()
                k = step[0]
                step[0] += 1
                if k % 2 == 0 and k < 6 * (NF + 1):
                    ffn_step(k // 2)
                if k == 6 * (NF + 1) + 2:
                    patch()

            def out(q, a):
                rq, cq = r0 + (q // 2) * HT, (q % 2) * HD + c * 128
                gate = gs[pl.ds(pl.multiple_of(rq, HT), HT), :]
                b = _ld(xs, rq, HT, cq, 128).astype(f32)
                _st(ob, rq, b + gate * (a - b), cq)

            _strassen(lambda k: _dot(o_term(i, k), wo_term(k, c), NN), between, out)
            defer(4, out_cp(r0, c * 128, 128).start)
            defer(4, out_cp(r0, HD + c * 128, 128).start)
    assert (NT_ - 1) * 28 > 6 * (NF + 1) + 2
    while delayed:
        tick()
    pltpu.make_async_copy(ob.bitcast(bf16), out_hbm, osems.at[0]).wait()


@jax.jit
def pallas_gated_mix__linear_kernel_hedgehog__moe_arch_mod__prompt_kernel(A_x, A_wqkv, A_w_phi, A_wo, B_x, B_w_r, B_w_gate, B_w_up, B_w_down, gate_w):
    hbm = pl.BlockSpec(memory_space=pl.ANY)
    out = pl.pallas_call(
        kernel,
        out_shape=jax.ShapeDtypeStruct((S, D), bf16),
        in_specs=[hbm] * 9,
        out_specs=hbm,
        scratch_shapes=[
            pltpu.VMEM((S // 2, D), i32),
            pltpu.VMEM((S // 4, 19 * HD), i32),
            pltpu.VMEM((D // 2, 3 * D), i32),
            pltpu.VMEM((H * DH, DH), bf16),
            pltpu.VMEM((2, 8, 128), bf16),
            pltpu.VMEM((D // 2, F), i32),
            pltpu.VMEM((D // 2, F), i32),
            pltpu.VMEM((F // 2, D), i32),
            pltpu.VMEM((NG * 128 // 2, 128), i32),
            pltpu.VMEM((16 * 80 // 2, 128), i32),
            pltpu.VMEM((S, 128), f32),
            pltpu.VMEM((8, S), f32),
            pltpu.VMEM((8, D), i32),
            pltpu.VMEM((S // 2, D), i32),
            pltpu.SemaphoreType.DMA((13,)),
            pltpu.SemaphoreType.DMA((1,)),
            pltpu.SemaphoreType.REGULAR,
        ] + [pltpu.VMEM((64, 7 * HD), i32)] * 12,
        compiler_params=pltpu.CompilerParams(vmem_limit_bytes=110 * 1024 * 1024, disable_bounds_checks=True),
    )(A_x.reshape(S, D), A_wqkv, A_w_phi.reshape(H * DH, DH), A_wo,
      B_w_r.reshape(8, 128), B_w_gate, B_w_up, B_w_down, gate_w.reshape(8, 128))
    return out.reshape(1, S, D)
```

```python
import functools
import os
import jax
import jax.numpy as jnp
import numpy as np
from jax import lax
import jax.experimental.pallas as pl
import jax.experimental.pallas.tpu as pltpu

S, D, H, DH, F = 2048, 1024, 32, 32, 3584
NG = 8
T = 256
HT = T // 2
HD = D // 2
NT_ = S // T
NF = F // 128
LOG2E = 1.4426950408889634
ODELAY = int(os.environ.get('ODELAY', 3))
QPOS = tuple(int(v) for v in os.environ.get('QPOS', '0,1,3,5').split(','))
FFN0 = 0
NW = int(os.environ.get('NW', 2))
NO = int(os.environ.get('NO', 2))
WJ = int(os.environ.get('WJ', 2))
LAGS = tuple(int(v) for v in os.environ.get('LAGS', '2,2,2,2').split(','))

NT = (((1,), (1,)), ((), ()))
NN = (((1,), (0,)), ((), ()))
f32 = jnp.float32
bf16 = jnp.bfloat16
i32 = jnp.int32


def _dot(a, b, dims):
    return lax.dot_general(a, b, dims, preferred_element_type=f32)


def _recip(x):
    r = pl.reciprocal(x, approx=True)
    return r * (2.0 - x * r)


def _sigmoid(x):
    return jax.nn.sigmoid(x)


def _r16(x):
    return x.astype(bf16).astype(f32)


def _ld(ref, r0, n, c0=None, nc=None, dz=None):
    h0 = r0 // 2 if isinstance(r0, int) else pl.multiple_of(r0 // 2, 8)
    if dz is not None:
        h0 = pl.multiple_of(h0 + dz, 8)
    cols = slice(None) if c0 is None else pl.ds(c0, nc)
    return pltpu.bitcast(ref[pl.ds(h0, n // 2), cols], bf16)


def _st(ref, r0, val, c0=None):
    h0 = r0 // 2 if isinstance(r0, int) else pl.multiple_of(r0 // 2, 8)
    cols = slice(None) if c0 is None else pl.ds(c0, val.shape[1])
    ref[pl.ds(h0, val.shape[0] // 2), cols] = pltpu.bitcast(val.astype(bf16), i32)


def _dual_softmax(p):
    outs = []
    for h in range(p.shape[0] // DH):
        ph = p[h * DH:(h + 1) * DH]
        mx = jnp.max(ph, axis=0, keepdims=True)
        mn = jnp.min(ph, axis=0, keepdims=True)
        ep = jnp.exp2(ph - mx)
        en = jnp.exp2(mn - ph)
        sp = jnp.sum(ep, axis=0, keepdims=True)
        sn = jnp.sum(en, axis=0, keepdims=True)
        outs.append(ep * _recip(sp))
        outs.append(en * _recip(sn))
    return jnp.concatenate(outs, axis=0)


def _col(row):
    return jnp.broadcast_to(row, (128, 128)).T


def _lhs_terms(a11, a12, a21, a22):
    return [a11 + a22, a21 + a22, a11, a22, a11 + a12, a21 - a11, a12 - a22]


def _lhs_sums(a11, a12, a21, a22):
    return [a11 + a22, a21 + a22, a11 + a12, a21 - a11, a12 - a22]


def _rhs_sums(b11, b12, b21, b22):
    return [b11 + b22, b12 - b22, b21 - b11, b11 + b12, b21 + b22]


LHS_SLOT = {0: 0, 1: 1, 4: 2, 5: 3, 6: 4}
RHS_SLOT = {0: 0, 2: 1, 3: 2, 5: 3, 6: 4}


def _strassen(prod, between, out):
    m4 = prod(3)
    between(0)
    m2 = prod(1)
    out(2, m2 + m4)
    between(1)
    c11 = m4 + prod(6)
    between(2)
    m1 = prod(0)
    c11 = c11 + m1
    c22 = m1 - m2
    between(3)
    m5 = prod(4)
    out(0, c11 - m5)
    between(4)
    m3 = prod(2)
    out(1, m3 + m5)
    c22 = c22 + m3
    between(5)
    out(3, c22 + prod(5))
    between(6)


def kernel(x_hbm, wqkv_hbm, wphi_hbm, wo_hbm, wr_hbm, wg_hbm, wu_hbm, wd_hbm, gw_hbm,
           out_hbm,
           xs, xq, w3, wphi, wv2, wg, wu, wd, bd, kvs, gs, rs, xsel, ob,
           sems, osems, zsem, *wt):
    OS0 = 5 * HD
    WO0 = 12 * HD
    WS0 = 14 * HD
    zero = pl.semaphore_read(zsem)
    uses = [0]

    def dz():
        uses[0] += 1
        return zero * (8 * uses[0])

    def x_cp(t):
        return pltpu.make_async_copy(x_hbm.at[pl.ds(t * T, T)],
                                     xs.bitcast(bf16).at[pl.ds(t * T, T)], sems.at[t])

    def w3_cp(c0, nc, s):
        return pltpu.make_async_copy(wqkv_hbm.at[:, pl.ds(c0, nc)],
                                     w3.bitcast(bf16).at[:, pl.ds(c0, nc)], sems.at[s])

    def whole(src, dst, s):
        return pltpu.make_async_copy(src, dst.bitcast(bf16), sems.at[s])

    grp0 = [pltpu.make_async_copy(wphi_hbm.at[pl.ds(0, 128)], wphi.at[pl.ds(0, 128)], sems.at[8]),
            w3_cp(D, 128, 8), w3_cp(2 * D, 128, 8),
            pltpu.make_async_copy(wr_hbm, wv2.at[0], sems.at[8]),
            pltpu.make_async_copy(gw_hbm, wv2.at[1], sems.at[8])]
    grp1 = [pltpu.make_async_copy(wphi_hbm.at[pl.ds(128, 128)], wphi.at[pl.ds(128, 128)], sems.at[9]),
            w3_cp(D + 128, 128, 9), w3_cp(2 * D + 128, 128, 9)]
    grp2 = [w3_cp(c0 + g * 128, 128, 10) for g in (2, 3) for c0 in (D, 2 * D)]
    grp2.append(pltpu.make_async_copy(wphi_hbm.at[pl.ds(256, 768)], wphi.at[pl.ds(256, 768)], sems.at[10]))

    def rows(src, dst, r0, n, s):
        return pltpu.make_async_copy(src.at[pl.ds(r0, n)], dst.bitcast(bf16).at[pl.ds(r0, n)], sems.at[s])

    grp3 = [w3_cp(D + 512, 512, 11), w3_cp(2 * D + 512, 512, 11), w3_cp(0, D, 11)]
    for j in range(NT_):
        for u in range(2):
            grp3.append(pltpu.make_async_copy(
                wo_hbm.at[pl.ds(u * HD + j * 64, 64)],
                xq.bitcast(bf16).at[pl.ds(j * HT + u * 64, 64), pl.ds(WO0, D)], sems.at[11]))
    grp4 = [rows(src, dst, r, 64, 12) for src, dst in ((wg_hbm, wg), (wu_hbm, wu)) for r in range(0, D, 64)]
    grp4 += [rows(wd_hbm, wd, r, 128, 12) for r in range(0, F, 128)]
    stream = list(grp4)

    def feed(n):
        for _ in range(n):
            if stream:
                stream.pop(0).start()

    def out_cp(r0, c0, nc):
        return pltpu.make_async_copy(ob.bitcast(bf16).at[pl.ds(r0, T), pl.ds(c0, nc)],
                                     out_hbm.at[pl.ds(r0, T), pl.ds(c0, nc)], osems.at[0])

    for cp in grp0:
        cp.start()
    x_cp(0).start()

    row = lax.broadcasted_iota(i32, (128, 128), 0)
    col = lax.broadcasted_iota(i32, (128, 128), 1)
    e_row = lax.broadcasted_iota(i32, (128, DH), 0)
    e_col = lax.broadcasted_iota(i32, (128, DH), 1)
    e = jnp.where((e_row % DH) == e_col, 1.0, 0.0).astype(bf16)
    for cp in grp0:
        cp.wait()
    for cp in grp1:
        cp.start()
    x_cp(1).start()

    delayed = []

    def defer(gaps, fn):
        delayed.append([gaps, fn])

    def tick():
        for item in delayed:
            item[0] -= 1
        due = [item for item in delayed if item[0] <= 0]
        delayed[:] = [item for item in delayed if item[0] > 0]
        for _, fn in due:
            fn()

    def make_bd(g0, n, gaps=0):
        m = _dot(e, wphi[pl.ds(g0 * 128, n * 128), :], NT)

        def store():
            for g in range(n):
                _st(bd, (g0 + g) * 128,
                    jnp.where((row // DH) == (col // DH), m[:, g * 128:(g + 1) * 128], 0.0))

        defer(gaps, store) if gaps else store()

    def fold(g, c0):
        return _dot(_ld(bd, g * 128, 128), _ld(w3, 0, D, c0, 128), NT) * LOG2E

    def put_lhs(slot, r0, top, bot):
        terms = _lhs_terms(top[:, :HD], top[:, HD:], bot[:, :HD], bot[:, HD:])
        for i, s in enumerate(terms):
            _st(wt[slot], r0, s, i * HD)

    def prep_kv(g):
        kt = fold(g, D + g * 128)
        vt = _ld(w3, 0, D, 2 * D + g * 128, 128).T.astype(f32)
        put_lhs(g, 64, vt[:64], vt[64:])
        put_lhs(g, 0, kt[:64], kt[64:])

    def prep_q(g):
        put_lhs(NG + g, 0, fold(g, g * 128), fold(g + 4, (g + 4) * 128))

    def put_sums(sums, load, dst, rd, cd, n):
        for r in range(0, n, 16):
            for c in range(0, HD, 128):
                b = [load(q, r, c).astype(f32) for q in range(4)]
                for i, s in enumerate(sums(*b)):
                    _st(dst, rd + r, s, cd + i * HD + c)

    def prep_wo(j, r):
        off = dz()
        put_sums(_rhs_sums,
                 lambda q, _, c: _ld(xq, j * HT + (q // 2) * 64 + r, 16, WO0 + (q % 2) * HD + c, 128, off),
                 xq, j * HT + r, WS0, 16)

    def prep_x(t):
        put_sums(_rhs_sums,
                 lambda q, r, c: _ld(xs, t * T + (q % 2) * HT + r, 16, (q // 2) * HD + c, 128),
                 xq, t * HT, 0, HT)

    st = {}
    wr = wv2[0].astype(f32)
    gw = wv2[1].astype(f32)
    score_rows = jnp.concatenate(
        [jnp.concatenate([jnp.broadcast_to(wr[j:j + 1, :], (8, 128)),
                          jnp.broadcast_to(gw[j:j + 1, :], (8, 128))], axis=0) for j in range(8)],
        axis=1).astype(bf16)

    def score_step(t, j):
        u, k0 = j // 2, (j % 2) * HD
        r0 = t * T + u * HT
        d = _dot(score_rows[:, k0:k0 + HD], _ld(xs, r0, HT, k0, HD), NT)
        if j % 2 == 0:
            st['sc'] = d
        else:
            d = d + st.pop('sc')
            rs[:, pl.ds(r0, HT)] = _r16(d[:8])
            gs[pl.ds(r0, HT), :] = _col(_sigmoid(d[8:9]))

    def x_term(i, t):
        if i == 1:
            return _ld(xs, t * T, HT, 0, HD, dz())
        if i == 4:
            return _ld(xs, t * T + HT, HT, HD, HD, dz())
        return _ld(xq, t * HT, HT, RHS_SLOT[i] * HD, HD, dz())

    def proj(slot, t, between, out):
        _strassen(lambda i: _dot(_ld(wt[slot], 0, 128, i * HD, HD, dz()), x_term(i, t), NT), between, out)

    r80 = lax.broadcasted_iota(i32, (80, 128), 0)
    c80 = lax.broadcasted_iota(i32, (80, 128), 1)
    kv_mask = jnp.where(r80 < 64, r80 // DH, r80 - 64) == (c80 // 64)

    def route():
        r = rs[...]
        pos = lax.broadcasted_iota(i32, r.shape, 1)
        m = jnp.max(jnp.where(r == r, r, -jnp.inf))
        idx = jnp.min(jnp.where(r == m, pos, S))
        idx = jnp.where(idx >= S, 0, idx)
        r_sel = jnp.max(jnp.where(pos == idx, r, -jnp.inf))
        st['idx'] = idx
        st['blk'] = blk = pl.multiple_of((idx // 16) * 16, 16)
        st['r_sel'] = r_sel
        _st(xsel, 0, _ld(xs, blk, 16))

    def ffn_step(k):
        n, j = divmod(k, 3)
        if j < 2 and n < NF:
            st['f', j] = _dot(_ld(xsel, 0, 16, dz=dz()), _ld((wg, wu)[j], 0, D, n * 128, 128), NN)
            if j == 1:
                gt = _r16(st.pop(('f', 0)))
                up = _r16(st.pop(('f', 1)))
                st['h', n] = (_r16(gt * _sigmoid(gt)) * up).astype(bf16)
        if j == 2 and 1 <= n <= NF:
            yk = _dot(st.pop(('h', n - 1)), _ld(wd, (n - 1) * 128, 128), NN)
            st['y'] = yk if n == 1 else st['y'] + yk

    accs = {}

    def kv_post(key, first, last, r):
        phi = _dual_softmax(r[:64])
        d = _dot(r[64:].astype(bf16), phi.astype(bf16), NT)
        accs[key] = (d, phi) if first else (accs[key][0] + d, accs[key][1] + phi)
        if last:
            d, z = accs.pop(key)
            zr = jnp.sum(z.T, axis=0, keepdims=True)
            kv = jnp.concatenate([d, jnp.broadcast_to(zr, (16, 128))], axis=0)
            defer(2, lambda: _st(kvs, key * 80, jnp.where(kv_mask, kv, 0.0)))

    make_bd(0, 1)
    prep_kv(0)
    xblocks = {0: (0,), 1: (1, 2), 2: (3, 4), 4: (5, 6), 6: (7,)}
    order = [(g, t) for t in range(NT_) for g in range(2)] + [(g, t) for g in range(2, NG) for t in range(NT_)]
    for g, t in order:
        if True:
            if g == 0 and t in xblocks:
                for u in xblocks[t]:
                    x_cp(u).wait()
                if t == 0:
                    x_cp(2).start()
                    prep_x(0)
                if t == 1:
                    x_cp(5).start()
                    prep_x(1)
                if t == 2:
                    x_cp(6).start()
                    x_cp(7).start()
                if t == 4:
                    for cp in grp2:
                        cp.start()
                if t == 6:
                    for cp in grp2:
                        cp.wait()
                    for cp in grp3:
                        cp.start()
            if g == 1 and t == 0:
                for cp in grp1:
                    cp.wait()
                x_cp(3).start()
                x_cp(4).start()
                make_bd(1, 1)
                prep_kv(1)
            if g == 3 and t == 1:
                for cp in grp3:
                    cp.wait()

            def between(j):
                tick()
                if g == 1 and j in (0, 1, 3, 4):
                    score_step(t, (0, 1, 3, 4).index(j))
                if j == 3 and g >= 3:
                    feed(1)
                if j == WJ and g >= 4:
                    k = (g - 4) * NT_ + t
                    prep_wo(k // 4, (k % 4) * 16)
                if j == 2 and g == 1 and 1 < t + 1 < NT_:
                    prep_x(t + 1)
                if j == 0 and g == 0 and t == 6:
                    make_bd(2, 6, 2)
                if j == 6:
                    if g >= 1 and t == (6 if g == 1 else 1):
                        if g + 1 < NG:
                            prep_kv(g + 1)
                        else:
                            prep_q(0)
                    if g == 2 and t == 3:
                        route()

            def out(q, c):
                defer(1 + LAGS[q], functools.partial(
                    kv_post, 2 * g + q // 2, t == 0 and q % 2 == 0, t == NT_ - 1 and q % 2 == 1, c))

            proj(g, t, between, out)

    pend = []

    def q_post(g, t, u, r):
        key = 2 * (g + 4 * (u % 2)) + u // 2
        phi = _dual_softmax(r).astype(bf16)
        nd = _dot(_ld(kvs, key * 80, 80, dz=dz()), phi, NN)
        inv = _recip(nd[64:72] + 1e-6)
        o = jnp.concatenate([nd[0:32] * inv[0:1], nd[32:64] * inv[1:2]], axis=0)
        st['o', u] = o
        if u < 3:
            return
        lo = jnp.concatenate([st.pop(('o', 0)), st.pop(('o', 2))], axis=0)
        hi = jnp.concatenate([st.pop(('o', 1)), st.pop(('o', 3))], axis=0)
        terms = _lhs_terms(lo[:, :HT], hi[:, :HT], lo[:, HT:], hi[:, HT:])

        def store(i, n):
            v = jnp.concatenate(terms[i:i + n], axis=1).astype(bf16).T
            for k in range(n):
                _st(xq, t * HT, v[k * HT:(k + 1) * HT], OS0 + (i + k) * HD + g * 128)

        for i in range(0, 7, 2):
            defer(ODELAY + i // 2, functools.partial(store, i, min(2, 7 - i)))

    for g in range(NG // 2):
        for t in range(NT_):
            if g == 3 and t == 4:
                assert not stream
                for cp in grp4:
                    cp.wait()

            def between(j):
                tick()
                if j == 3:
                    feed(1)
                if j in QPOS and pend:
                    pend.pop(0)()
                if j == 6 and t == 1 and g + 1 < NG // 2:
                    prep_q(g + 1)

            cs = {}
            proj(NG + g, t, between, cs.__setitem__)
            lo = jnp.concatenate([cs[0], cs[1]], axis=1)
            hi = jnp.concatenate([cs[2], cs[3]], axis=1)
            for u, r in enumerate((lo[:64], hi[:64], lo[64:], hi[64:])):
                pend.append(functools.partial(q_post, g, t, u, r))

    idx, blk = st['idx'], st['blk']
    t_last = idx // T

    tiles = [i + (t_last <= i).astype(i32) for i in range(NT_ - 1)] + [t_last]

    def tile_of(i):
        return tiles[i]

    def o_term(i, k):
        return _ld(xq, 0, HT, OS0 + k * HD, HD, tile_of(i) * (HT // 2) + dz())

    def wo_term(k, c):
        r0, c0 = (0, WO0) if k == 1 else (64, WO0 + HD) if k == 4 else (0, WS0 + RHS_SLOT[k] * HD)
        off = dz()
        return jnp.concatenate(
            [_ld(xq, j * HT + r0, 64, c0 + c * 128, 128, off) for j in range(NT_)], axis=0)

    def patch():
        sg = _r16(_sigmoid(jnp.full((16, D), st['r_sel'], f32)))
        y = _r16(_r16(st.pop('y')) * sg)
        sel = lax.broadcasted_iota(i32, (16, D), 0) == (idx - blk)
        xr = _ld(xs, blk, 16).astype(f32)
        _st(xs, blk, jnp.where(sel, xr + y, xr))

    step = [FFN0]
    for i in range(NT_):
        r0 = pl.multiple_of(tile_of(i) * T, T)
        for c in range(4):
            def between(j):
                tick()
                if j in QPOS and pend:
                    pend.pop(0)()
                k = step[0]
                step[0] += 1
                if k % 2 == 0 and k < 6 * (NF + 1):
                    ffn_step(k // 2)
                if k == 6 * (NF + 1) + 2:
                    patch()

            def out(q, a):
                rq, cq = r0 + (q // 2) * HT, (q % 2) * HD + c * 128
                gate = gs[pl.ds(pl.multiple_of(rq, HT), HT), :]
                b = _ld(xs, rq, HT, cq, 128).astype(f32)
                _st(ob, rq, b + gate * (a - b), cq)

            _strassen(lambda k: _dot(o_term(i, k), wo_term(k, c), NN), between, out)
            n = 1 if i == NT_ - 1 else 8 // NO
            if (c + 1) % n == 0:
                for u in range(2):
                    defer(4, out_cp(r0, u * HD + (c + 1 - n) * 128, n * 128).start)
    assert (NT_ - 1) * 28 > 6 * (NF + 1) + 2
    while delayed:
        tick()
    pltpu.make_async_copy(ob.bitcast(bf16), out_hbm, osems.at[0]).wait()


@jax.jit
def pallas_gated_mix__linear_kernel_hedgehog__moe_arch_mod__prompt_kernel(A_x, A_wqkv, A_w_phi, A_wo, B_x, B_w_r, B_w_gate, B_w_up, B_w_down, gate_w):
    hbm = pl.BlockSpec(memory_space=pl.ANY)
    out = pl.pallas_call(
        kernel,
        out_shape=jax.ShapeDtypeStruct((S, D), bf16),
        in_specs=[hbm] * 9,
        out_specs=hbm,
        scratch_shapes=[
            pltpu.VMEM((S // 2, D), i32),
            pltpu.VMEM((S // 4, 19 * HD), i32),
            pltpu.VMEM((D // 2, 3 * D), i32),
            pltpu.VMEM((H * DH, DH), bf16),
            pltpu.VMEM((2, 8, 128), bf16),
            pltpu.VMEM((D // 2, F), i32),
            pltpu.VMEM((D // 2, F), i32),
            pltpu.VMEM((F // 2, D), i32),
            pltpu.VMEM((NG * 128 // 2, 128), i32),
            pltpu.VMEM((16 * 80 // 2, 128), i32),
            pltpu.VMEM((S, 128), f32),
            pltpu.VMEM((8, S), f32),
            pltpu.VMEM((8, D), i32),
            pltpu.VMEM((S // 2, D), i32),
            pltpu.SemaphoreType.DMA((13,)),
            pltpu.SemaphoreType.DMA((1,)),
            pltpu.SemaphoreType.REGULAR,
        ] + [pltpu.VMEM((64, 7 * HD), i32)] * 12,
        compiler_params=pltpu.CompilerParams(vmem_limit_bytes=110 * 1024 * 1024, disable_bounds_checks=True),
    )(A_x.reshape(S, D), A_wqkv, A_w_phi.reshape(H * DH, DH), A_wo,
      B_w_r.reshape(8, 128), B_w_gate, B_w_up, B_w_down, gate_w.reshape(8, 128))
    return out.reshape(1, S, D)
```

```python
import functools
import os
import jax
import jax.numpy as jnp
import numpy as np
from jax import lax
import jax.experimental.pallas as pl
import jax.experimental.pallas.tpu as pltpu

S, D, H, DH, F = 2048, 1024, 32, 32, 3584
NG = 8
T = 256
HT = T // 2
HD = D // 2
NT_ = S // T
NF = F // 128
LOG2E = 1.4426950408889634
ODELAY = int(os.environ.get('ODELAY', 3))
QPOS = tuple(int(v) for v in os.environ.get('QPOS', '0,1,3,5').split(','))
FFN0 = 0
XGAPS = tuple(int(v) for v in os.environ.get('XGAPS', '1,2,4,5,7,9,10,12').split(','))
NW = int(os.environ.get('NW', 2))
NO = int(os.environ.get('NO', 2))
WJ = int(os.environ.get('WJ', 3))
LAGS = tuple(int(v) for v in os.environ.get('LAGS', '2,4,2,5').split(','))

NT = (((1,), (1,)), ((), ()))
NN = (((1,), (0,)), ((), ()))
f32 = jnp.float32
bf16 = jnp.bfloat16
i32 = jnp.int32


def _dot(a, b, dims):
    return lax.dot_general(a, b, dims, preferred_element_type=f32)


def _recip(x):
    r = pl.reciprocal(x, approx=True)
    return r * (2.0 - x * r)


def _sigmoid(x):
    return jax.nn.sigmoid(x)


def _r16(x):
    return x.astype(bf16).astype(f32)


def _ld(ref, r0, n, c0=None, nc=None, dz=None):
    h0 = r0 // 2 if isinstance(r0, int) else pl.multiple_of(r0 // 2, 8)
    if dz is not None:
        h0 = pl.multiple_of(h0 + dz, 8)
    cols = slice(None) if c0 is None else pl.ds(c0, nc)
    return pltpu.bitcast(ref[pl.ds(h0, n // 2), cols], bf16)


def _st(ref, r0, val, c0=None):
    h0 = r0 // 2 if isinstance(r0, int) else pl.multiple_of(r0 // 2, 8)
    cols = slice(None) if c0 is None else pl.ds(c0, val.shape[1])
    ref[pl.ds(h0, val.shape[0] // 2), cols] = pltpu.bitcast(val.astype(bf16), i32)


def _dual_softmax(p):
    outs = []
    for h in range(p.shape[0] // DH):
        ph = p[h * DH:(h + 1) * DH]
        mx = jnp.max(ph, axis=0, keepdims=True)
        mn = jnp.min(ph, axis=0, keepdims=True)
        ep = jnp.exp2(ph - mx)
        en = jnp.exp2(mn - ph)
        sp = jnp.sum(ep, axis=0, keepdims=True)
        sn = jnp.sum(en, axis=0, keepdims=True)
        outs.append(ep * _recip(sp))
        outs.append(en * _recip(sn))
    return jnp.concatenate(outs, axis=0)


def _col(row):
    return jnp.broadcast_to(row, (128, 128)).T


def _lhs_terms(a11, a12, a21, a22):
    return [a11 + a22, a21 + a22, a11, a22, a11 + a12, a21 - a11, a12 - a22]


def _lhs_sums(a11, a12, a21, a22):
    return [a11 + a22, a21 + a22, a11 + a12, a21 - a11, a12 - a22]


def _rhs_sums(b11, b12, b21, b22):
    return [b11 + b22, b12 - b22, b21 - b11, b11 + b12, b21 + b22]


LHS_SLOT = {0: 0, 1: 1, 4: 2, 5: 3, 6: 4}
RHS_SLOT = {0: 0, 2: 1, 3: 2, 5: 3, 6: 4}


def _strassen(prod, between, out):
    m4 = prod(3)
    between(0)
    m2 = prod(1)
    out(2, m2 + m4)
    between(1)
    c11 = m4 + prod(6)
    between(2)
    m1 = prod(0)
    c11 = c11 + m1
    c22 = m1 - m2
    between(3)
    m5 = prod(4)
    out(0, c11 - m5)
    between(4)
    m3 = prod(2)
    out(1, m3 + m5)
    c22 = c22 + m3
    between(5)
    out(3, c22 + prod(5))
    between(6)


def kernel(x_hbm, wqkv_hbm, wphi_hbm, wo_hbm, wr_hbm, wg_hbm, wu_hbm, wd_hbm, gw_hbm,
           out_hbm,
           xs, xq, w3, wphi, wv2, wg, wu, wd, bd, kvs, gs, rs, xsel, ob,
           sems, osems, zsem, *wt):
    OS0 = 5 * HD
    WO0 = 12 * HD
    WS0 = 14 * HD
    zero = pl.semaphore_read(zsem)
    uses = [0]

    def dz():
        uses[0] += 1
        return zero * (8 * uses[0])

    def x_cp(t):
        return pltpu.make_async_copy(x_hbm.at[pl.ds(t * T, T)],
                                     xs.bitcast(bf16).at[pl.ds(t * T, T)], sems.at[t])

    def w3_cp(c0, nc, s):
        return pltpu.make_async_copy(wqkv_hbm.at[:, pl.ds(c0, nc)],
                                     w3.bitcast(bf16).at[:, pl.ds(c0, nc)], sems.at[s])

    def whole(src, dst, s):
        return pltpu.make_async_copy(src, dst.bitcast(bf16), sems.at[s])

    grp0 = [pltpu.make_async_copy(wphi_hbm.at[pl.ds(0, 128)], wphi.at[pl.ds(0, 128)], sems.at[8]),
            w3_cp(D, 128, 8), w3_cp(2 * D, 128, 8),
            pltpu.make_async_copy(wr_hbm, wv2.at[0], sems.at[8]),
            pltpu.make_async_copy(gw_hbm, wv2.at[1], sems.at[8])]
    grp1 = [pltpu.make_async_copy(wphi_hbm.at[pl.ds(128, 128)], wphi.at[pl.ds(128, 128)], sems.at[9]),
            w3_cp(D + 128, 128, 9), w3_cp(2 * D + 128, 128, 9)]
    grp2 = [w3_cp(c0 + g * 128, 128, 10) for g in (2, 3) for c0 in (D, 2 * D)]
    grp2.append(pltpu.make_async_copy(wphi_hbm.at[pl.ds(256, 768)], wphi.at[pl.ds(256, 768)], sems.at[10]))

    def rows(src, dst, r0, n, s):
        return pltpu.make_async_copy(src.at[pl.ds(r0, n)], dst.bitcast(bf16).at[pl.ds(r0, n)], sems.at[s])

    grp3 = [w3_cp(D + 512, 512, 11), w3_cp(2 * D + 512, 512, 11), w3_cp(0, D, 11)]
    for j in range(NT_):
        for u in range(2):
            grp3.append(pltpu.make_async_copy(
                wo_hbm.at[pl.ds(u * HD + j * 64, 64)],
                xq.bitcast(bf16).at[pl.ds(j * HT + u * 64, 64), pl.ds(WO0, D)], sems.at[11]))
    grp4 = [rows(src, dst, r, 64, 12) for src, dst in ((wg_hbm, wg), (wu_hbm, wu)) for r in range(0, D, 64)]
    grp4 += [rows(wd_hbm, wd, r, 128, 12) for r in range(0, F, 128)]
    stream = list(grp4)

    def feed(n):
        for _ in range(n):
            if stream:
                stream.pop(0).start()

    def out_cp(r0, c0, nc):
        return pltpu.make_async_copy(ob.bitcast(bf16).at[pl.ds(r0, T), pl.ds(c0, nc)],
                                     out_hbm.at[pl.ds(r0, T), pl.ds(c0, nc)], osems.at[0])

    for cp in grp0:
        cp.start()
    x_cp(0).start()

    row = lax.broadcasted_iota(i32, (128, 128), 0)
    col = lax.broadcasted_iota(i32, (128, 128), 1)
    e_row = lax.broadcasted_iota(i32, (128, DH), 0)
    e_col = lax.broadcasted_iota(i32, (128, DH), 1)
    e = jnp.where((e_row % DH) == e_col, 1.0, 0.0).astype(bf16)
    for cp in grp0:
        cp.wait()
    for cp in grp1:
        cp.start()
    x_cp(1).start()

    delayed = []

    def defer(gaps, fn):
        delayed.append([gaps, fn])

    def tick():
        for item in delayed:
            item[0] -= 1
        due = [item for item in delayed if item[0] <= 0]
        delayed[:] = [item for item in delayed if item[0] > 0]
        for _, fn in due:
            fn()

    def make_bd(g0, n, gaps=0):
        m = _dot(e, wphi[pl.ds(g0 * 128, n * 128), :], NT)

        def store():
            for g in range(n):
                _st(bd, (g0 + g) * 128,
                    jnp.where((row // DH) == (col // DH), m[:, g * 128:(g + 1) * 128], 0.0))

        defer(gaps, store) if gaps else store()

    def fold(g, c0):
        return _dot(_ld(bd, g * 128, 128), _ld(w3, 0, D, c0, 128), NT) * LOG2E

    def put_lhs(slot, r0, top, bot):
        terms = _lhs_terms(top[:, :HD], top[:, HD:], bot[:, :HD], bot[:, HD:])
        for i, s in enumerate(terms):
            _st(wt[slot], r0, s, i * HD)

    def prep_kv(g):
        kt = fold(g, D + g * 128)
        vt = _ld(w3, 0, D, 2 * D + g * 128, 128).T.astype(f32)
        put_lhs(g, 64, vt[:64], vt[64:])
        put_lhs(g, 0, kt[:64], kt[64:])

    def prep_q(g):
        put_lhs(NG + g, 0, fold(g, g * 128), fold(g + 4, (g + 4) * 128))

    def put_sums(sums, load, dst, rd, cd, n):
        for r in range(0, n, 16):
            for c in range(0, HD, 128):
                b = [load(q, r, c).astype(f32) for q in range(4)]
                for i, s in enumerate(sums(*b)):
                    _st(dst, rd + r, s, cd + i * HD + c)

    def prep_wo(j, r):
        off = dz()
        put_sums(_rhs_sums,
                 lambda q, _, c: _ld(xq, j * HT + (q // 2) * 64 + r, 16, WO0 + (q % 2) * HD + c, 128, off),
                 xq, j * HT + r, WS0, 16)

    def prep_x(t, r0=0, n=HT):
        put_sums(_rhs_sums,
                 lambda q, r, c: _ld(xs, t * T + (q % 2) * HT + r0 + r, 16, (q // 2) * HD + c, 128),
                 xq, t * HT + r0, 0, n)

    st = {}
    wr = wv2[0].astype(f32)
    gw = wv2[1].astype(f32)
    score_rows = jnp.concatenate(
        [jnp.concatenate([jnp.broadcast_to(wr[j:j + 1, :], (8, 128)),
                          jnp.broadcast_to(gw[j:j + 1, :], (8, 128))], axis=0) for j in range(8)],
        axis=1).astype(bf16)

    def score_step(t, j):
        u, k0 = j // 2, (j % 2) * HD
        r0 = t * T + u * HT
        d = _dot(score_rows[:, k0:k0 + HD], _ld(xs, r0, HT, k0, HD), NT)
        if j % 2 == 0:
            st['sc'] = d
        else:
            d = d + st.pop('sc')
            rs[:, pl.ds(r0, HT)] = _r16(d[:8])
            gs[pl.ds(r0, HT), :] = _col(_sigmoid(d[8:9]))

    def x_term(i, t):
        if i == 1:
            return _ld(xs, t * T, HT, 0, HD, dz())
        if i == 4:
            return _ld(xs, t * T + HT, HT, HD, HD, dz())
        return _ld(xq, t * HT, HT, RHS_SLOT[i] * HD, HD, dz())

    def proj(slot, t, between, out):
        _strassen(lambda i: _dot(_ld(wt[slot], 0, 128, i * HD, HD, dz()), x_term(i, t), NT), between, out)

    r80 = lax.broadcasted_iota(i32, (80, 128), 0)
    c80 = lax.broadcasted_iota(i32, (80, 128), 1)
    kv_mask = jnp.where(r80 < 64, r80 // DH, r80 - 64) == (c80 // 64)

    def route():
        r = rs[...]
        pos = lax.broadcasted_iota(i32, r.shape, 1)
        m = jnp.max(jnp.where(r == r, r, -jnp.inf))
        idx = jnp.min(jnp.where(r == m, pos, S))
        idx = jnp.where(idx >= S, 0, idx)
        r_sel = jnp.max(jnp.where(pos == idx, r, -jnp.inf))
        st['idx'] = idx
        st['blk'] = blk = pl.multiple_of((idx // 16) * 16, 16)
        st['r_sel'] = r_sel
        _st(xsel, 0, _ld(xs, blk, 16))

    def ffn_step(k):
        n, j = divmod(k, 3)
        if j < 2 and n < NF:
            st['f', j] = _dot(_ld(xsel, 0, 16, dz=dz()), _ld((wg, wu)[j], 0, D, n * 128, 128), NN)
            if j == 1:
                gt = _r16(st.pop(('f', 0)))
                up = _r16(st.pop(('f', 1)))
                st['h', n] = (_r16(gt * _sigmoid(gt)) * up).astype(bf16)
        if j == 2 and 1 <= n <= NF:
            yk = _dot(st.pop(('h', n - 1)), _ld(wd, (n - 1) * 128, 128), NN)
            st['y'] = yk if n == 1 else st['y'] + yk

    accs = {}

    def kv_post(key, first, last, r):
        phi = _dual_softmax(r[:64])
        d = _dot(r[64:].astype(bf16), phi.astype(bf16), NT)
        accs[key] = (d, phi) if first else (accs[key][0] + d, accs[key][1] + phi)
        if last:
            d, z = accs.pop(key)
            zr = jnp.sum(z.T, axis=0, keepdims=True)
            kv = jnp.concatenate([d, jnp.broadcast_to(zr, (16, 128))], axis=0)
            defer(2, lambda: _st(kvs, key * 80, jnp.where(kv_mask, kv, 0.0)))

    make_bd(0, 1)
    prep_kv(0)
    xblocks = {0: (0,), 1: (1, 2), 2: (3, 4), 4: (5, 6), 6: (7,)}
    order = [(g, t) for t in range(NT_) for g in range(2)] + [(g, t) for g in range(2, NG) for t in range(NT_)]
    for g, t in order:
        if True:
            if g == 0 and t in xblocks:
                for u in xblocks[t]:
                    x_cp(u).wait()
                if t == 0:
                    x_cp(2).start()
                    prep_x(0)
                if t == 1:
                    x_cp(5).start()
                    prep_x(1)
                if t == 2:
                    x_cp(6).start()
                    x_cp(7).start()
                if t == 4:
                    for cp in grp2:
                        cp.start()
                if t == 6:
                    for cp in grp2:
                        cp.wait()
                    for cp in grp3:
                        cp.start()
            if g == 1 and t == 0:
                for cp in grp1:
                    cp.wait()
                x_cp(3).start()
                x_cp(4).start()
                make_bd(1, 1)
                prep_kv(1)
            if g == 3 and t == 1:
                for cp in grp3:
                    cp.wait()

            def between(j):
                tick()
                if g == 1 and j in (0, 1, 3, 4):
                    score_step(t, (0, 1, 3, 4).index(j))
                if j == 3 and g >= 3:
                    feed(1)
                if j == WJ and g >= 4:
                    k = (g - 4) * NT_ + t
                    prep_wo(k // 4, (k % 4) * 16)
                if g < 2 and 1 < t + 1 < NT_ and g * 7 + j in XGAPS:
                    prep_x(t + 1, XGAPS.index(g * 7 + j) * 16, 16)
                if j == 0 and g == 0 and t == 6:
                    make_bd(2, 6, 2)
                if j == 6:
                    if g >= 1 and t == (6 if g == 1 else 1):
                        if g + 1 < NG:
                            prep_kv(g + 1)
                        else:
                            prep_q(0)
                    if g == 2 and t == 3:
                        route()

            def out(q, c):
                defer(1 + LAGS[q], functools.partial(
                    kv_post, 2 * g + q // 2, t == 0 and q % 2 == 0, t == NT_ - 1 and q % 2 == 1, c))

            proj(g, t, between, out)

    pend = []

    def q_post(g, t, u, r):
        key = 2 * (g + 4 * (u % 2)) + u // 2
        phi = _dual_softmax(r).astype(bf16)
        nd = _dot(_ld(kvs, key * 80, 80, dz=dz()), phi, NN)
        inv = _recip(nd[64:72] + 1e-6)
        o = jnp.concatenate([nd[0:32] * inv[0:1], nd[32:64] * inv[1:2]], axis=0)
        st['o', u] = o
        if u < 3:
            return
        lo = jnp.concatenate([st.pop(('o', 0)), st.pop(('o', 2))], axis=0)
        hi = jnp.concatenate([st.pop(('o', 1)), st.pop(('o', 3))], axis=0)
        terms = _lhs_terms(lo[:, :HT], hi[:, :HT], lo[:, HT:], hi[:, HT:])

        def store(i, n):
            v = jnp.concatenate(terms[i:i + n], axis=1).astype(bf16).T
            for k in range(n):
                _st(xq, t * HT, v[k * HT:(k + 1) * HT], OS0 + (i + k) * HD + g * 128)

        for i in range(0, 7, 2):
            defer(ODELAY + i // 2, functools.partial(store, i, min(2, 7 - i)))

    for g in range(NG // 2):
        for t in range(NT_):
            if g == 3 and t == 4:
                assert not stream
                for cp in grp4:
                    cp.wait()

            def between(j):
                tick()
                if j == 3:
                    feed(1)
                if j in QPOS and pend:
                    pend.pop(0)()
                if j == 6 and t == 1 and g + 1 < NG // 2:
                    prep_q(g + 1)

            cs = {}
            proj(NG + g, t, between, cs.__setitem__)
            lo = jnp.concatenate([cs[0], cs[1]], axis=1)
            hi = jnp.concatenate([cs[2], cs[3]], axis=1)
            for u, r in enumerate((lo[:64], hi[:64], lo[64:], hi[64:])):
                pend.append(functools.partial(q_post, g, t, u, r))

    idx, blk = st['idx'], st['blk']
    t_last = idx // T

    tiles = [i + (t_last <= i).astype(i32) for i in range(NT_ - 1)] + [t_last]

    def tile_of(i):
        return tiles[i]

    def o_term(i, k):
        return _ld(xq, 0, HT, OS0 + k * HD, HD, tile_of(i) * (HT // 2) + dz())

    def wo_term(k, c):
        r0, c0 = (0, WO0) if k == 1 else (64, WO0 + HD) if k == 4 else (0, WS0 + RHS_SLOT[k] * HD)
        off = dz()
        return jnp.concatenate(
            [_ld(xq, j * HT + r0, 64, c0 + c * 128, 128, off) for j in range(NT_)], axis=0)

    def patch():
        sg = _r16(_sigmoid(jnp.full((16, D), st['r_sel'], f32)))
        y = _r16(_r16(st.pop('y')) * sg)
        sel = lax.broadcasted_iota(i32, (16, D), 0) == (idx - blk)
        xr = _ld(xs, blk, 16).astype(f32)
        _st(xs, blk, jnp.where(sel, xr + y, xr))

    step = [FFN0]
    for i in range(NT_):
        r0 = pl.multiple_of(tile_of(i) * T, T)
        for c in range(4):
            def between(j):
                tick()
                if j in QPOS and pend:
                    pend.pop(0)()
                k = step[0]
                step[0] += 1
                if k % 2 == 0 and k < 6 * (NF + 1):
                    ffn_step(k // 2)
                if k == 6 * (NF + 1) + 2:
                    patch()

            def out(q, a):
                rq, cq = r0 + (q // 2) * HT, (q % 2) * HD + c * 128
                gate = gs[pl.ds(pl.multiple_of(rq, HT), HT), :]
                b = _ld(xs, rq, HT, cq, 128).astype(f32)
                _st(ob, rq, b + gate * (a - b), cq)

            _strassen(lambda k: _dot(o_term(i, k), wo_term(k, c), NN), between, out)
            n = 1 if i == NT_ - 1 else 8 // NO
            if (c + 1) % n == 0:
                for u in range(2):
                    defer(4, out_cp(r0, u * HD + (c + 1 - n) * 128, n * 128).start)
    assert (NT_ - 1) * 28 > 6 * (NF + 1) + 2
    while delayed:
        tick()
    pltpu.make_async_copy(ob.bitcast(bf16), out_hbm, osems.at[0]).wait()


@jax.jit
def pallas_gated_mix__linear_kernel_hedgehog__moe_arch_mod__prompt_kernel(A_x, A_wqkv, A_w_phi, A_wo, B_x, B_w_r, B_w_gate, B_w_up, B_w_down, gate_w):
    hbm = pl.BlockSpec(memory_space=pl.ANY)
    out = pl.pallas_call(
        kernel,
        out_shape=jax.ShapeDtypeStruct((S, D), bf16),
        in_specs=[hbm] * 9,
        out_specs=hbm,
        scratch_shapes=[
            pltpu.VMEM((S // 2, D), i32),
            pltpu.VMEM((S // 4, 19 * HD), i32),
            pltpu.VMEM((D // 2, 3 * D), i32),
            pltpu.VMEM((H * DH, DH), bf16),
            pltpu.VMEM((2, 8, 128), bf16),
            pltpu.VMEM((D // 2, F), i32),
            pltpu.VMEM((D // 2, F), i32),
            pltpu.VMEM((F // 2, D), i32),
            pltpu.VMEM((NG * 128 // 2, 128), i32),
            pltpu.VMEM((16 * 80 // 2, 128), i32),
            pltpu.VMEM((S, 128), f32),
            pltpu.VMEM((8, S), f32),
            pltpu.VMEM((8, D), i32),
            pltpu.VMEM((S // 2, D), i32),
            pltpu.SemaphoreType.DMA((13,)),
            pltpu.SemaphoreType.DMA((1,)),
            pltpu.SemaphoreType.REGULAR,
        ] + [pltpu.VMEM((64, 7 * HD), i32)] * 12,
        compiler_params=pltpu.CompilerParams(vmem_limit_bytes=110 * 1024 * 1024, disable_bounds_checks=True),
    )(A_x.reshape(S, D), A_wqkv, A_w_phi.reshape(H * DH, DH), A_wo,
      B_w_r.reshape(8, 128), B_w_gate, B_w_up, B_w_down, gate_w.reshape(8, 128))
    return out.reshape(1, S, D)
```

```python
import functools
import os
import jax
import jax.numpy as jnp
import numpy as np
from jax import lax
import jax.experimental.pallas as pl
import jax.experimental.pallas.tpu as pltpu

S, D, H, DH, F = 2048, 1024, 32, 32, 3584
NG = 8
T = 256
HT = T // 2
HD = D // 2
NT_ = S // T
NF = F // 128
LOG2E = 1.4426950408889634
ODELAY = int(os.environ.get('ODELAY', 3))
QPOS = tuple(int(v) for v in os.environ.get('QPOS', '0,1,3,5').split(','))
FFN0 = 0
XGAPS = tuple(int(v) for v in os.environ.get('XGAPS', '1,2,4,5,7,9,10,12').split(','))
NW = int(os.environ.get('NW', 2))
NO = int(os.environ.get('NO', 2))
WJ = int(os.environ.get('WJ', 3))
LAGS = tuple(int(v) for v in os.environ.get('LAGS', '2,4,2,5').split(','))

NT = (((1,), (1,)), ((), ()))
NN = (((1,), (0,)), ((), ()))
f32 = jnp.float32
bf16 = jnp.bfloat16
i32 = jnp.int32


def _dot(a, b, dims):
    return lax.dot_general(a, b, dims, preferred_element_type=f32)


def _recip(x):
    r = pl.reciprocal(x, approx=True)
    return r * (2.0 - x * r)


def _sigmoid(x):
    return jax.nn.sigmoid(x)


def _r16(x):
    return x.astype(bf16).astype(f32)


def _ld(ref, r0, n, c0=None, nc=None, dz=None):
    h0 = r0 // 2 if isinstance(r0, int) else pl.multiple_of(r0 // 2, 8)
    if dz is not None:
        h0 = pl.multiple_of(h0 + dz, 8)
    cols = slice(None) if c0 is None else pl.ds(c0, nc)
    return pltpu.bitcast(ref[pl.ds(h0, n // 2), cols], bf16)


def _st(ref, r0, val, c0=None):
    h0 = r0 // 2 if isinstance(r0, int) else pl.multiple_of(r0 // 2, 8)
    cols = slice(None) if c0 is None else pl.ds(c0, val.shape[1])
    ref[pl.ds(h0, val.shape[0] // 2), cols] = pltpu.bitcast(val.astype(bf16), i32)


def _dual_softmax(p):
    outs = []
    for h in range(p.shape[0] // DH):
        ph = p[h * DH:(h + 1) * DH]
        mx = jnp.max(ph, axis=0, keepdims=True)
        mn = jnp.min(ph, axis=0, keepdims=True)
        ep = jnp.exp2(ph - mx)
        en = jnp.exp2(mn - ph)
        sp = jnp.sum(ep, axis=0, keepdims=True)
        sn = jnp.sum(en, axis=0, keepdims=True)
        outs.append(ep * _recip(sp))
        outs.append(en * _recip(sn))
    return jnp.concatenate(outs, axis=0)


def _col(row):
    return jnp.broadcast_to(row, (128, 128)).T


def _lhs_terms(a11, a12, a21, a22):
    return [a11 + a22, a21 + a22, a11, a22, a11 + a12, a21 - a11, a12 - a22]


def _lhs_sums(a11, a12, a21, a22):
    return [a11 + a22, a21 + a22, a11 + a12, a21 - a11, a12 - a22]


def _rhs_sums(b11, b12, b21, b22):
    return [b11 + b22, b12 - b22, b21 - b11, b11 + b12, b21 + b22]


LHS_SLOT = {0: 0, 1: 1, 4: 2, 5: 3, 6: 4}
RHS_SLOT = {0: 0, 2: 1, 3: 2, 5: 3, 6: 4}


def _strassen(prod, between, out):
    m4 = prod(3)
    between(0)
    m2 = prod(1)
    out(2, m2 + m4)
    between(1)
    c11 = m4 + prod(6)
    between(2)
    m1 = prod(0)
    c11 = c11 + m1
    c22 = m1 - m2
    between(3)
    m5 = prod(4)
    out(0, c11 - m5)
    between(4)
    m3 = prod(2)
    out(1, m3 + m5)
    c22 = c22 + m3
    between(5)
    out(3, c22 + prod(5))
    between(6)


def kernel(x_hbm, wqkv_hbm, wphi_hbm, wo_hbm, wr_hbm, wg_hbm, wu_hbm, wd_hbm, gw_hbm,
           out_hbm,
           xs, xq, w3, wphi, wv2, wg, wu, wd, bd, kvs, gs, rs, xsel, ob,
           sems, osems, zsem, *wt):
    OS0 = 5 * HD
    WO0 = 12 * HD
    WS0 = 14 * HD
    zero = pl.semaphore_read(zsem)
    uses = [0]

    def dz():
        uses[0] += 1
        return zero * (8 * uses[0])

    def x_cp(t):
        return pltpu.make_async_copy(x_hbm.at[pl.ds(t * T, T)],
                                     xs.bitcast(bf16).at[pl.ds(t * T, T)], sems.at[t])

    def w3_cp(c0, nc, s):
        return pltpu.make_async_copy(wqkv_hbm.at[:, pl.ds(c0, nc)],
                                     w3.bitcast(bf16).at[:, pl.ds(c0, nc)], sems.at[s])

    def whole(src, dst, s):
        return pltpu.make_async_copy(src, dst.bitcast(bf16), sems.at[s])

    grp0 = [pltpu.make_async_copy(wphi_hbm.at[pl.ds(0, 256)], wphi.at[pl.ds(0, 256)], sems.at[8]),
            w3_cp(D, 256, 8), w3_cp(2 * D, 256, 8),
            pltpu.make_async_copy(wr_hbm, wv2.at[0], sems.at[8]),
            pltpu.make_async_copy(gw_hbm, wv2.at[1], sems.at[8])]
    grp2 = [w3_cp(D + 256, 128, 9), w3_cp(2 * D + 256, 128, 9),
            pltpu.make_async_copy(wphi_hbm.at[pl.ds(256, 768)], wphi.at[pl.ds(256, 768)], sems.at[9])]
    grp2b = [w3_cp(D + 384, 640, 10), w3_cp(2 * D + 384, 640, 10)]

    def rows(src, dst, r0, n, s):
        return pltpu.make_async_copy(src.at[pl.ds(r0, n)], dst.bitcast(bf16).at[pl.ds(r0, n)], sems.at[s])

    grp3 = [w3_cp(0, D, 11)]
    for j in range(NT_):
        for u in range(2):
            grp3.append(pltpu.make_async_copy(
                wo_hbm.at[pl.ds(u * HD + j * 64, 64)],
                xq.bitcast(bf16).at[pl.ds(j * HT + u * 64, 64), pl.ds(WO0, D)], sems.at[11]))
    grp4 = [rows(src, dst, r, 64, 12) for src, dst in ((wg_hbm, wg), (wu_hbm, wu)) for r in range(0, D, 64)]
    grp4 += [rows(wd_hbm, wd, r, 128, 12) for r in range(0, F, 128)]
    stream = list(grp4)

    def feed(n):
        for _ in range(n):
            if stream:
                stream.pop(0).start()

    def out_cp(r0, c0, nc):
        return pltpu.make_async_copy(ob.bitcast(bf16).at[pl.ds(r0, T), pl.ds(c0, nc)],
                                     out_hbm.at[pl.ds(r0, T), pl.ds(c0, nc)], osems.at[0])

    for cp in grp0:
        cp.start()
    x_cp(0).start()

    row = lax.broadcasted_iota(i32, (128, 128), 0)
    col = lax.broadcasted_iota(i32, (128, 128), 1)
    e_row = lax.broadcasted_iota(i32, (128, DH), 0)
    e_col = lax.broadcasted_iota(i32, (128, DH), 1)
    e = jnp.where((e_row % DH) == e_col, 1.0, 0.0).astype(bf16)
    for cp in grp0:
        cp.wait()
    x_cp(1).start()
    x_cp(2).start()

    delayed = []

    def defer(gaps, fn):
        delayed.append([gaps, fn])

    def tick():
        for item in delayed:
            item[0] -= 1
        due = [item for item in delayed if item[0] <= 0]
        delayed[:] = [item for item in delayed if item[0] > 0]
        for _, fn in due:
            fn()

    def make_bd(g0, n, gaps=0):
        m = _dot(e, wphi[pl.ds(g0 * 128, n * 128), :], NT)

        def store():
            for g in range(n):
                _st(bd, (g0 + g) * 128,
                    jnp.where((row // DH) == (col // DH), m[:, g * 128:(g + 1) * 128], 0.0))

        defer(gaps, store) if gaps else store()

    def fold(g, c0):
        return _dot(_ld(bd, g * 128, 128), _ld(w3, 0, D, c0, 128), NT) * LOG2E

    def put_lhs(slot, r0, top, bot):
        terms = _lhs_terms(top[:, :HD], top[:, HD:], bot[:, :HD], bot[:, HD:])
        for i, s in enumerate(terms):
            _st(wt[slot], r0, s, i * HD)

    def prep_kv(g):
        kt = fold(g, D + g * 128)
        vt = _ld(w3, 0, D, 2 * D + g * 128, 128).T.astype(f32)
        put_lhs(g, 64, vt[:64], vt[64:])
        put_lhs(g, 0, kt[:64], kt[64:])

    def prep_q(g):
        put_lhs(NG + g, 0, fold(g, g * 128), fold(g + 4, (g + 4) * 128))

    def put_sums(sums, load, dst, rd, cd, n):
        for r in range(0, n, 16):
            for c in range(0, HD, 128):
                b = [load(q, r, c).astype(f32) for q in range(4)]
                for i, s in enumerate(sums(*b)):
                    _st(dst, rd + r, s, cd + i * HD + c)

    def prep_wo(j, r):
        off = dz()
        put_sums(_rhs_sums,
                 lambda q, _, c: _ld(xq, j * HT + (q // 2) * 64 + r, 16, WO0 + (q % 2) * HD + c, 128, off),
                 xq, j * HT + r, WS0, 16)

    def prep_x(t, r0=0, n=HT):
        put_sums(_rhs_sums,
                 lambda q, r, c: _ld(xs, t * T + (q % 2) * HT + r0 + r, 16, (q // 2) * HD + c, 128),
                 xq, t * HT + r0, 0, n)

    st = {}
    wr = wv2[0].astype(f32)
    gw = wv2[1].astype(f32)
    score_rows = jnp.concatenate(
        [jnp.concatenate([jnp.broadcast_to(wr[j:j + 1, :], (8, 128)),
                          jnp.broadcast_to(gw[j:j + 1, :], (8, 128))], axis=0) for j in range(8)],
        axis=1).astype(bf16)

    def score_step(t, j):
        u, k0 = j // 2, (j % 2) * HD
        r0 = t * T + u * HT
        d = _dot(score_rows[:, k0:k0 + HD], _ld(xs, r0, HT, k0, HD), NT)
        if j % 2 == 0:
            st['sc'] = d
        else:
            d = d + st.pop('sc')
            rs[:, pl.ds(r0, HT)] = _r16(d[:8])
            gs[pl.ds(r0, HT), :] = _col(_sigmoid(d[8:9]))

    def x_term(i, t):
        if i == 1:
            return _ld(xs, t * T, HT, 0, HD, dz())
        if i == 4:
            return _ld(xs, t * T + HT, HT, HD, HD, dz())
        return _ld(xq, t * HT, HT, RHS_SLOT[i] * HD, HD, dz())

    def proj(slot, t, between, out):
        _strassen(lambda i: _dot(_ld(wt[slot], 0, 128, i * HD, HD, dz()), x_term(i, t), NT), between, out)

    r80 = lax.broadcasted_iota(i32, (80, 128), 0)
    c80 = lax.broadcasted_iota(i32, (80, 128), 1)
    kv_mask = jnp.where(r80 < 64, r80 // DH, r80 - 64) == (c80 // 64)

    def route():
        r = rs[...]
        pos = lax.broadcasted_iota(i32, r.shape, 1)
        m = jnp.max(jnp.where(r == r, r, -jnp.inf))
        idx = jnp.min(jnp.where(r == m, pos, S))
        idx = jnp.where(idx >= S, 0, idx)
        r_sel = jnp.max(jnp.where(pos == idx, r, -jnp.inf))
        st['idx'] = idx
        st['blk'] = blk = pl.multiple_of((idx // 16) * 16, 16)
        st['r_sel'] = r_sel
        _st(xsel, 0, _ld(xs, blk, 16))

    def ffn_step(k):
        n, j = divmod(k, 3)
        if j < 2 and n < NF:
            st['f', j] = _dot(_ld(xsel, 0, 16, dz=dz()), _ld((wg, wu)[j], 0, D, n * 128, 128), NN)
            if j == 1:
                gt = _r16(st.pop(('f', 0)))
                up = _r16(st.pop(('f', 1)))
                st['h', n] = (_r16(gt * _sigmoid(gt)) * up).astype(bf16)
        if j == 2 and 1 <= n <= NF:
            yk = _dot(st.pop(('h', n - 1)), _ld(wd, (n - 1) * 128, 128), NN)
            st['y'] = yk if n == 1 else st['y'] + yk

    accs = {}

    def kv_post(key, first, last, r):
        phi = _dual_softmax(r[:64])
        d = _dot(r[64:].astype(bf16), phi.astype(bf16), NT)
        accs[key] = (d, phi) if first else (accs[key][0] + d, accs[key][1] + phi)
        if last:
            d, z = accs.pop(key)
            zr = jnp.sum(z.T, axis=0, keepdims=True)
            kv = jnp.concatenate([d, jnp.broadcast_to(zr, (16, 128))], axis=0)
            defer(2, lambda: _st(kvs, key * 80, jnp.where(kv_mask, kv, 0.0)))

    make_bd(0, 2)
    prep_kv(0)
    prep_kv(1)
    xblocks = {0: (0,), 1: (1, 2), 2: (3,), 3: (4, 5), 5: (6, 7)}
    order = [(g, t) for t in range(NT_) for g in range(2)] + [(g, t) for g in range(2, NG) for t in range(NT_)]
    for g, t in order:
        if True:
            if g == 0 and t in xblocks:
                for u in xblocks[t]:
                    x_cp(u).wait()
                if t == 0:
                    x_cp(3).start()
                    x_cp(4).start()
                    prep_x(0)
                if t == 1:
                    x_cp(5).start()
                    x_cp(6).start()
                    prep_x(1)
                if t == 2:
                    x_cp(7).start()
                    for cp in grp2:
                        cp.start()
                if t == 3:
                    for cp in grp2b:
                        cp.start()
                if t == 5:
                    for cp in grp2:
                        cp.wait()
                    for cp in grp3:
                        cp.start()
            if g == 2 and t == 1:
                for cp in grp2b:
                    cp.wait()
            if g == 4 and t == 0:
                for cp in grp3:
                    cp.wait()

            def between(j):
                tick()
                if g == 1 and j in (0, 1, 3, 4):
                    score_step(t, (0, 1, 3, 4).index(j))
                if j == 3 and g >= 3:
                    feed(1)
                if j == WJ and g >= 4:
                    k = (g - 4) * NT_ + t
                    prep_wo(k // 4, (k % 4) * 16)
                if g < 2 and 1 < t + 1 < NT_ and g * 7 + j in XGAPS:
                    prep_x(t + 1, XGAPS.index(g * 7 + j) * 16, 16)
                if j == 0 and g == 0 and t == 5:
                    make_bd(2, 6, 2)
                if j == 6:
                    if g >= 1 and t == (6 if g == 1 else 1):
                        if g + 1 < NG:
                            prep_kv(g + 1)
                        else:
                            prep_q(0)
                    if g == 2 and t == 3:
                        route()

            def out(q, c):
                defer(1 + LAGS[q], functools.partial(
                    kv_post, 2 * g + q // 2, t == 0 and q % 2 == 0, t == NT_ - 1 and q % 2 == 1, c))

            proj(g, t, between, out)

    pend = []

    def q_post(g, t, u, r):
        key = 2 * (g + 4 * (u % 2)) + u // 2
        phi = _dual_softmax(r).astype(bf16)
        nd = _dot(_ld(kvs, key * 80, 80, dz=dz()), phi, NN)
        inv = _recip(nd[64:72] + 1e-6)
        o = jnp.concatenate([nd[0:32] * inv[0:1], nd[32:64] * inv[1:2]], axis=0)
        st['o', u] = o
        if u < 3:
            return
        lo = jnp.concatenate([st.pop(('o', 0)), st.pop(('o', 2))], axis=0)
        hi = jnp.concatenate([st.pop(('o', 1)), st.pop(('o', 3))], axis=0)
        terms = _lhs_terms(lo[:, :HT], hi[:, :HT], lo[:, HT:], hi[:, HT:])

        def store(i, n):
            v = jnp.concatenate(terms[i:i + n], axis=1).astype(bf16).T
            for k in range(n):
                _st(xq, t * HT, v[k * HT:(k + 1) * HT], OS0 + (i + k) * HD + g * 128)

        for i in range(0, 7, 2):
            defer(ODELAY + i // 2, functools.partial(store, i, min(2, 7 - i)))

    for g in range(NG // 2):
        for t in range(NT_):
            if g == 3 and t == 4:
                assert not stream
                for cp in grp4:
                    cp.wait()

            def between(j):
                tick()
                if j == 3:
                    feed(1)
                if j in QPOS and pend:
                    pend.pop(0)()
                if j == 6 and t == 1 and g + 1 < NG // 2:
                    prep_q(g + 1)

            cs = {}
            proj(NG + g, t, between, cs.__setitem__)
            lo = jnp.concatenate([cs[0], cs[1]], axis=1)
            hi = jnp.concatenate([cs[2], cs[3]], axis=1)
            for u, r in enumerate((lo[:64], hi[:64], lo[64:], hi[64:])):
                pend.append(functools.partial(q_post, g, t, u, r))

    idx, blk = st['idx'], st['blk']
    t_last = idx // T

    tiles = [i + (t_last <= i).astype(i32) for i in range(NT_ - 1)] + [t_last]

    def tile_of(i):
        return tiles[i]

    def o_term(i, k):
        return _ld(xq, 0, HT, OS0 + k * HD, HD, tile_of(i) * (HT // 2) + dz())

    def wo_term(k, c):
        r0, c0 = (0, WO0) if k == 1 else (64, WO0 + HD) if k == 4 else (0, WS0 + RHS_SLOT[k] * HD)
        off = dz()
        return jnp.concatenate(
            [_ld(xq, j * HT + r0, 64, c0 + c * 128, 128, off) for j in range(NT_)], axis=0)

    def patch():
        sg = _r16(_sigmoid(jnp.full((16, D), st['r_sel'], f32)))
        y = _r16(_r16(st.pop('y')) * sg)
        sel = lax.broadcasted_iota(i32, (16, D), 0) == (idx - blk)
        xr = _ld(xs, blk, 16).astype(f32)
        _st(xs, blk, jnp.where(sel, xr + y, xr))

    step = [FFN0]
    for i in range(NT_):
        r0 = pl.multiple_of(tile_of(i) * T, T)
        for c in range(4):
            def between(j):
                tick()
                if j in QPOS and pend:
                    pend.pop(0)()
                k = step[0]
                step[0] += 1
                if k % 2 == 0 and k < 6 * (NF + 1):
                    ffn_step(k // 2)
                if k == 6 * (NF + 1) + 2:
                    patch()

            def out(q, a):
                rq, cq = r0 + (q // 2) * HT, (q % 2) * HD + c * 128
                gate = gs[pl.ds(pl.multiple_of(rq, HT), HT), :]
                b = _ld(xs, rq, HT, cq, 128).astype(f32)
                _st(ob, rq, b + gate * (a - b), cq)

            _strassen(lambda k: _dot(o_term(i, k), wo_term(k, c), NN), between, out)
            n = 1 if i == NT_ - 1 else 8 // NO
            if (c + 1) % n == 0:
                for u in range(2):
                    defer(4, out_cp(r0, u * HD + (c + 1 - n) * 128, n * 128).start)
    assert (NT_ - 1) * 28 > 6 * (NF + 1) + 2
    while delayed:
        tick()
    pltpu.make_async_copy(ob.bitcast(bf16), out_hbm, osems.at[0]).wait()


@jax.jit
def pallas_gated_mix__linear_kernel_hedgehog__moe_arch_mod__prompt_kernel(A_x, A_wqkv, A_w_phi, A_wo, B_x, B_w_r, B_w_gate, B_w_up, B_w_down, gate_w):
    hbm = pl.BlockSpec(memory_space=pl.ANY)
    out = pl.pallas_call(
        kernel,
        out_shape=jax.ShapeDtypeStruct((S, D), bf16),
        in_specs=[hbm] * 9,
        out_specs=hbm,
        scratch_shapes=[
            pltpu.VMEM((S // 2, D), i32),
            pltpu.VMEM((S // 4, 19 * HD), i32),
            pltpu.VMEM((D // 2, 3 * D), i32),
            pltpu.VMEM((H * DH, DH), bf16),
            pltpu.VMEM((2, 8, 128), bf16),
            pltpu.VMEM((D // 2, F), i32),
            pltpu.VMEM((D // 2, F), i32),
            pltpu.VMEM((F // 2, D), i32),
            pltpu.VMEM((NG * 128 // 2, 128), i32),
            pltpu.VMEM((16 * 80 // 2, 128), i32),
            pltpu.VMEM((S, 128), f32),
            pltpu.VMEM((8, S), f32),
            pltpu.VMEM((8, D), i32),
            pltpu.VMEM((S // 2, D), i32),
            pltpu.SemaphoreType.DMA((13,)),
            pltpu.SemaphoreType.DMA((1,)),
            pltpu.SemaphoreType.REGULAR,
        ] + [pltpu.VMEM((64, 7 * HD), i32)] * 12,
        compiler_params=pltpu.CompilerParams(vmem_limit_bytes=110 * 1024 * 1024, disable_bounds_checks=True),
    )(A_x.reshape(S, D), A_wqkv, A_w_phi.reshape(H * DH, DH), A_wo,
      B_w_r.reshape(8, 128), B_w_gate, B_w_up, B_w_down, gate_w.reshape(8, 128))
    return out.reshape(1, S, D)
```

```python
import functools

import jax
import jax.numpy as jnp
from jax import lax
import jax.experimental.pallas as pl
import jax.experimental.pallas.tpu as pltpu

S, D, H, DH, F = 2048, 1024, 32, 32, 3584
NG = 8
T = 256
HT = T // 2
HD = D // 2
NTILE = S // T
NF = F // 128
LOG2E = 1.4426950408889634

OS0, WO0, WS0, XQ_COLS = 5 * HD, 12 * HD, 14 * HD, 19 * HD

KV_LAG = (3, 5, 3, 6)
X_GAPS = (1, 2, 4, 5, 7, 9, 10, 12)
Q_GAPS = (0, 1, 3, 5)
O_LAG = 3
DMA_LAG = 4

NT = (((1,), (1,)), ((), ()))
NN = (((1,), (0,)), ((), ()))
f32 = jnp.float32
bf16 = jnp.bfloat16
i32 = jnp.int32


def _dot(a, b, dims):
    return lax.dot_general(a, b, dims, preferred_element_type=f32)


def _recip(x):
    r = pl.reciprocal(x, approx=True)
    return r * (2.0 - x * r)


def _r16(x):
    return x.astype(bf16).astype(f32)


def _ld(ref, r0, n, c0=None, nc=None, off=None):
    h0 = r0 // 2 if isinstance(r0, int) else pl.multiple_of(r0 // 2, 8)
    if off is not None:
        h0 = pl.multiple_of(h0 + off, 8)
    cols = slice(None) if c0 is None else pl.ds(c0, nc)
    return pltpu.bitcast(ref[pl.ds(h0, n // 2), cols], bf16)


def _st(ref, r0, val, c0=None):
    h0 = r0 // 2 if isinstance(r0, int) else pl.multiple_of(r0 // 2, 8)
    cols = slice(None) if c0 is None else pl.ds(c0, val.shape[1])
    ref[pl.ds(h0, val.shape[0] // 2), cols] = pltpu.bitcast(val.astype(bf16), i32)


def _dual_softmax(p):
    outs = []
    for h in range(p.shape[0] // DH):
        ph = p[h * DH:(h + 1) * DH]
        mx = jnp.max(ph, axis=0, keepdims=True)
        mn = jnp.min(ph, axis=0, keepdims=True)
        ep = jnp.exp2(ph - mx)
        en = jnp.exp2(mn - ph)
        outs.append(ep * _recip(jnp.sum(ep, axis=0, keepdims=True)))
        outs.append(en * _recip(jnp.sum(en, axis=0, keepdims=True)))
    return jnp.concatenate(outs, axis=0)


def _col(row):
    return jnp.broadcast_to(row, (128, 128)).T


def _lhs_terms(a11, a12, a21, a22):
    return [a11 + a22, a21 + a22, a11, a22, a11 + a12, a21 - a11, a12 - a22]


def _rhs_sums(b11, b12, b21, b22):
    return [b11 + b22, b12 - b22, b21 - b11, b11 + b12, b21 + b22]


RHS_SLOT = {0: 0, 2: 1, 3: 2, 5: 3, 6: 4}


def _strassen(prod, between, out):
    m4 = prod(3)
    between(0)
    m2 = prod(1)
    out(2, m2 + m4)
    between(1)
    c11 = m4 + prod(6)
    between(2)
    m1 = prod(0)
    c11 = c11 + m1
    c22 = m1 - m2
    between(3)
    m5 = prod(4)
    out(0, c11 - m5)
    between(4)
    m3 = prod(2)
    out(1, m3 + m5)
    c22 = c22 + m3
    between(5)
    out(3, c22 + prod(5))
    between(6)


def _kernel(x_hbm, wqkv_hbm, wphi_hbm, wo_hbm, wr_hbm, wg_hbm, wu_hbm, wd_hbm, gw_hbm,
            out_hbm,
            xs, xq, w3, wphi, wv2, wg, wu, wd, bd, kvs, gs, rs, xsel, ob,
            sems, osem, zsem, *wt):
    zero = pl.semaphore_read(zsem)
    uses = [0]

    def dz():
        uses[0] += 1
        return zero * (8 * uses[0])

    delayed = []

    def defer(gaps, fn):
        delayed.append([gaps, fn])

    def tick():
        for item in delayed:
            item[0] -= 1
        due = [item for item in delayed if item[0] <= 0]
        delayed[:] = [item for item in delayed if item[0] > 0]
        for _, fn in due:
            fn()

    def rows_cp(src, dst, r0, n, s):
        return pltpu.make_async_copy(src.at[pl.ds(r0, n)], dst.bitcast(bf16).at[pl.ds(r0, n)], sems.at[s])

    def w3_cp(c0, nc, s):
        return pltpu.make_async_copy(wqkv_hbm.at[:, pl.ds(c0, nc)],
                                     w3.bitcast(bf16).at[:, pl.ds(c0, nc)], sems.at[s])

    def wphi_cp(r0, n, s):
        return pltpu.make_async_copy(wphi_hbm.at[pl.ds(r0, n)], wphi.at[pl.ds(r0, n)], sems.at[s])

    def out_cp(r0, c0, nc):
        return pltpu.make_async_copy(ob.bitcast(bf16).at[pl.ds(r0, T), pl.ds(c0, nc)],
                                     out_hbm.at[pl.ds(r0, T), pl.ds(c0, nc)], osem)

    def start(cps):
        for cp in cps:
            cp.start()

    def wait(cps):
        for cp in cps:
            cp.wait()

    x_cps = [rows_cp(x_hbm, xs, t * T, T, t) for t in range(NTILE)]
    first = [wphi_cp(0, 256, 8), w3_cp(D, 256, 8), w3_cp(2 * D, 256, 8),
             pltpu.make_async_copy(wr_hbm, wv2.at[0], sems.at[8]),
             pltpu.make_async_copy(gw_hbm, wv2.at[1], sems.at[8])]
    second = [w3_cp(D + 256, 128, 9), w3_cp(2 * D + 256, 128, 9), wphi_cp(256, 768, 9)]
    third = [w3_cp(D + 384, 640, 10), w3_cp(2 * D + 384, 640, 10)]
    fourth = [w3_cp(0, D, 11)]
    for j in range(NTILE):
        for u in range(2):
            fourth.append(pltpu.make_async_copy(
                wo_hbm.at[pl.ds(u * HD + j * 64, 64)],
                xq.bitcast(bf16).at[pl.ds(j * HT + u * 64, 64), pl.ds(WO0, D)], sems.at[11]))
    ffn_cps = [rows_cp(src, dst, r, 64, 12)
               for src, dst in ((wg_hbm, wg), (wu_hbm, wu)) for r in range(0, D, 64)]
    ffn_cps += [rows_cp(wd_hbm, wd, r, 128, 12) for r in range(0, F, 128)]
    stream = list(ffn_cps)

    def feed():
        if stream:
            stream.pop(0).start()

    start(first + x_cps[:1])
    row = lax.broadcasted_iota(i32, (128, 128), 0)
    col = lax.broadcasted_iota(i32, (128, 128), 1)
    eye = jnp.where(lax.broadcasted_iota(i32, (128, DH), 0) % DH
                    == lax.broadcasted_iota(i32, (128, DH), 1), 1.0, 0.0).astype(bf16)
    wait(first)
    start(x_cps[1:3])

    def make_bd(g0, n, gaps=0):
        m = _dot(eye, wphi[pl.ds(g0 * 128, n * 128), :], NT)

        def store():
            for g in range(n):
                _st(bd, (g0 + g) * 128, jnp.where(row // DH == col // DH, m[:, g * 128:(g + 1) * 128], 0.0))

        if gaps:
            defer(gaps, store)
        else:
            store()

    def fold(g, c0):
        return _dot(_ld(bd, g * 128, 128), _ld(w3, 0, D, c0, 128), NT) * LOG2E

    def put_lhs(slot, r0, top, bot):
        for i, s in enumerate(_lhs_terms(top[:, :HD], top[:, HD:], bot[:, :HD], bot[:, HD:])):
            _st(wt[slot], r0, s, i * HD)

    def prep_kv(g):
        kt = fold(g, D + g * 128)
        vt = _ld(w3, 0, D, 2 * D + g * 128, 128).T.astype(f32)
        put_lhs(g, 64, vt[:64], vt[64:])
        put_lhs(g, 0, kt[:64], kt[64:])

    def prep_q(g):
        put_lhs(NG + g, 0, fold(g, g * 128), fold(g + 4, (g + 4) * 128))

    def put_rhs(load, rd, cd, n):
        for r in range(0, n, 16):
            for c in range(0, HD, 128):
                for i, s in enumerate(_rhs_sums(*[load(q, r, c).astype(f32) for q in range(4)])):
                    _st(xq, rd + r, s, cd + i * HD + c)

    def prep_x(t, r0, n):
        put_rhs(lambda q, r, c: _ld(xs, t * T + (q % 2) * HT + r0 + r, 16, (q // 2) * HD + c, 128),
                t * HT + r0, 0, n)

    def prep_wo(k):
        r0, off = (k // 4) * HT + (k % 4) * 16, dz()
        put_rhs(lambda q, r, c: _ld(xq, r0 + (q // 2) * 64, 16, WO0 + (q % 2) * HD + c, 128, off),
                r0, WS0, 16)

    def x_term(i, t):
        if i == 1:
            return _ld(xs, t * T, HT, 0, HD, dz())
        if i == 4:
            return _ld(xs, t * T + HT, HT, HD, HD, dz())
        return _ld(xq, t * HT, HT, RHS_SLOT[i] * HD, HD, dz())

    def project(slot, t, between, out):
        _strassen(lambda i: _dot(_ld(wt[slot], 0, 128, i * HD, HD, dz()), x_term(i, t), NT), between, out)

    st = {}
    wr = wv2[0].astype(f32)
    gw = wv2[1].astype(f32)
    score_rows = jnp.concatenate(
        [jnp.concatenate([jnp.broadcast_to(wr[j:j + 1, :], (8, 128)),
                          jnp.broadcast_to(gw[j:j + 1, :], (8, 128))], axis=0) for j in range(8)],
        axis=1).astype(bf16)

    def score_step(t, j):
        r0, k0 = t * T + (j // 2) * HT, (j % 2) * HD
        d = _dot(score_rows[:, k0:k0 + HD], _ld(xs, r0, HT, k0, HD), NT)
        if j % 2 == 0:
            st['sc'] = d
        else:
            d = d + st.pop('sc')
            rs[:, pl.ds(r0, HT)] = _r16(d[:8])
            gs[pl.ds(r0, HT), :] = _col(jax.nn.sigmoid(d[8:9]))

    def route():
        r = rs[...]
        pos = lax.broadcasted_iota(i32, r.shape, 1)
        best = jnp.max(jnp.where(r == r, r, -jnp.inf))
        idx = jnp.min(jnp.where(r == best, pos, S))
        st['idx'] = idx = jnp.where(idx >= S, 0, idx)
        st['score'] = jnp.sum(jnp.where(pos == idx, r, 0.0)[:1])
        st['blk'] = blk = pl.multiple_of((idx // 16) * 16, 16)
        _st(xsel, 0, _ld(xs, blk, 16))

    def ffn_step(k):
        n, j = divmod(k, 3)
        if j < 2 and n < NF:
            st['f', j] = _dot(_ld(xsel, 0, 16, off=dz()), _ld((wg, wu)[j], 0, D, n * 128, 128), NN)
            if j == 1:
                gt, up = _r16(st.pop(('f', 0))), _r16(st.pop(('f', 1)))
                st['h', n] = (_r16(gt * jax.nn.sigmoid(gt)) * up).astype(bf16)
        if j == 2 and 1 <= n <= NF:
            yk = _dot(st.pop(('h', n - 1)), _ld(wd, (n - 1) * 128, 128), NN)
            st['y'] = yk if n == 1 else st['y'] + yk

    def patch():
        weight = _r16(jax.nn.sigmoid(jnp.full((16, D), st['score'], f32)))
        y = _r16(_r16(st.pop('y')) * weight)
        sel = lax.broadcasted_iota(i32, (16, D), 0) == st['idx'] - st['blk']
        xr = _ld(xs, st['blk'], 16).astype(f32)
        _st(xs, st['blk'], jnp.where(sel, xr + y, xr))

    r80 = lax.broadcasted_iota(i32, (80, 128), 0)
    c80 = lax.broadcasted_iota(i32, (80, 128), 1)
    kv_mask = jnp.where(r80 < 64, r80 // DH, r80 - 64) == c80 // 64
    accs = {}

    def kv_update(pair, is_first, is_last, r):
        phi = _dual_softmax(r[:64])
        d = _dot(r[64:].astype(bf16), phi.astype(bf16), NT)
        accs[pair] = (d, phi) if is_first else (accs[pair][0] + d, accs[pair][1] + phi)
        if is_last:
            d, z = accs.pop(pair)
            z = jnp.sum(z.T, axis=0, keepdims=True)
            kv = jnp.concatenate([d, jnp.broadcast_to(z, (16, 128))], axis=0)
            defer(2, lambda: _st(kvs, pair * 80, jnp.where(kv_mask, kv, 0.0)))

    make_bd(0, 2)
    prep_kv(0)
    prep_kv(1)
    order = [(g, t) for t in range(NTILE) for g in range(2)]
    order += [(g, t) for g in range(2, NG) for t in range(NTILE)]
    for g, t in order:
        if (g, t) == (0, 0):
            wait(x_cps[:1])
            start(x_cps[3:5])
            prep_x(0, 0, HT)
        if (g, t) == (0, 1):
            wait(x_cps[1:3])
            start(x_cps[5:7])
            prep_x(1, 0, HT)
        if (g, t) == (0, 2):
            wait(x_cps[3:4])
            start(x_cps[7:] + second)
        if (g, t) == (0, 3):
            wait(x_cps[4:6])
            start(third)
        if (g, t) == (0, 5):
            wait(x_cps[6:] + second)
            start(fourth)
        if (g, t) == (2, 1):
            wait(third)
        if (g, t) == (4, 0):
            wait(fourth)

        def between(j):
            tick()
            if g == 1 and j in (0, 1, 3, 4):
                score_step(t, (0, 1, 3, 4).index(j))
            if j == 3 and g >= 3:
                feed()
            if j == 3 and g >= 4:
                prep_wo((g - 4) * NTILE + t)
            if g < 2 and 1 < t + 1 < NTILE and g * 7 + j in X_GAPS:
                prep_x(t + 1, X_GAPS.index(g * 7 + j) * 16, 16)
            if (g, t, j) == (0, 5, 0):
                make_bd(2, 6, 2)
            if j == 6 and g >= 1 and t == (6 if g == 1 else 1):
                if g + 1 < NG:
                    prep_kv(g + 1)
                else:
                    prep_q(0)
            if (g, t, j) == (2, 3, 6):
                route()

        def out(q, c):
            defer(KV_LAG[q], functools.partial(
                kv_update, 2 * g + q // 2, t == 0 and q % 2 == 0, t == NTILE - 1 and q % 2 == 1, c))

        project(g, t, between, out)

    pairs = []

    def attend(g, t, u, r):
        phi = _dual_softmax(r).astype(bf16)
        kv = _ld(kvs, (2 * (g + 4 * (u % 2)) + u // 2) * 80, 80, off=dz())
        nd = _dot(kv, phi, NN)
        inv = _recip(nd[64:72] + 1e-6)
        st['o', u] = jnp.concatenate([nd[0:32] * inv[0:1], nd[32:64] * inv[1:2]], axis=0)
        if u < 3:
            return
        lo = jnp.concatenate([st.pop(('o', 0)), st.pop(('o', 2))], axis=0)
        hi = jnp.concatenate([st.pop(('o', 1)), st.pop(('o', 3))], axis=0)
        terms = _lhs_terms(lo[:, :HT], hi[:, :HT], lo[:, HT:], hi[:, HT:])

        def store(i, n):
            v = jnp.concatenate(terms[i:i + n], axis=1).astype(bf16).T
            for k in range(n):
                _st(xq, t * HT, v[k * HT:(k + 1) * HT], OS0 + (i + k) * HD + g * 128)

        for i in range(0, 7, 2):
            defer(O_LAG + i // 2, functools.partial(store, i, min(2, 7 - i)))

    for g in range(NG // 2):
        for t in range(NTILE):
            if (g, t) == (3, 4):
                assert not stream
                wait(ffn_cps)

            def between(j):
                tick()
                if j == 3:
                    feed()
                if j in Q_GAPS and pairs:
                    pairs.pop(0)()
                if (t, j) == (1, 6) and g + 1 < NG // 2:
                    prep_q(g + 1)

            cs = {}
            project(NG + g, t, between, cs.__setitem__)
            lo = jnp.concatenate([cs[0], cs[1]], axis=1)
            hi = jnp.concatenate([cs[2], cs[3]], axis=1)
            for u, r in enumerate((lo[:64], hi[:64], lo[64:], hi[64:])):
                pairs.append(functools.partial(attend, g, t, u, r))

    routed = st['idx'] // T
    tiles = [i + (routed <= i).astype(i32) for i in range(NTILE - 1)] + [routed]
    ffn_gaps = 6 * (NF + 1)
    assert ffn_gaps + 2 < (NTILE - 1) * 28

    def wo_term(k, c):
        r0, c0 = (0, WO0) if k == 1 else (64, WO0 + HD) if k == 4 else (0, WS0 + RHS_SLOT[k] * HD)
        off = dz()
        return jnp.concatenate(
            [_ld(xq, j * HT + r0, 64, c0 + c * 128, 128, off) for j in range(NTILE)], axis=0)

    for i, tile in enumerate(tiles):
        r0 = pl.multiple_of(tile * T, T)
        for c in range(4):
            def between(j):
                tick()
                if j in Q_GAPS and pairs:
                    pairs.pop(0)()
                k = (i * 4 + c) * 7 + j
                if k % 2 == 0 and k < ffn_gaps:
                    ffn_step(k // 2)
                if k == ffn_gaps + 2:
                    patch()

            def mix(q, a):
                rq, cq = r0 + (q // 2) * HT, (q % 2) * HD + c * 128
                gate = gs[pl.ds(pl.multiple_of(rq, HT), HT), :]
                b = _ld(xs, rq, HT, cq, 128).astype(f32)
                _st(ob, rq, b + gate * (a - b), cq)

            _strassen(lambda k: _dot(_ld(xq, 0, HT, OS0 + k * HD, HD, tile * (HT // 2) + dz()),
                                     wo_term(k, c), NN), between, mix)
            n = 1 if i == NTILE - 1 else 4
            if (c + 1) % n == 0:
                for u in range(2):
                    defer(DMA_LAG, out_cp(r0, u * HD + (c + 1 - n) * 128, n * 128).start)
    while delayed:
        tick()
    pltpu.make_async_copy(ob.bitcast(bf16), out_hbm, osem).wait()


@jax.jit
def pallas_gated_mix__linear_kernel_hedgehog__moe_arch_mod__prompt_kernel(A_x, A_wqkv, A_w_phi, A_wo, B_x, B_w_r, B_w_gate, B_w_up, B_w_down, gate_w):
    del B_x
    hbm = pl.BlockSpec(memory_space=pl.ANY)
    out = pl.pallas_call(
        _kernel,
        out_shape=jax.ShapeDtypeStruct((S, D), bf16),
        in_specs=[hbm] * 9,
        out_specs=hbm,
        scratch_shapes=[
            pltpu.VMEM((S // 2, D), i32),
            pltpu.VMEM((S // 4, XQ_COLS), i32),
            pltpu.VMEM((D // 2, 3 * D), i32),
            pltpu.VMEM((H * DH, DH), bf16),
            pltpu.VMEM((2, 8, 128), bf16),
            pltpu.VMEM((D // 2, F), i32),
            pltpu.VMEM((D // 2, F), i32),
            pltpu.VMEM((F // 2, D), i32),
            pltpu.VMEM((NG * 128 // 2, 128), i32),
            pltpu.VMEM((16 * 80 // 2, 128), i32),
            pltpu.VMEM((S, 128), f32),
            pltpu.VMEM((8, S), f32),
            pltpu.VMEM((8, D), i32),
            pltpu.VMEM((S // 2, D), i32),
            pltpu.SemaphoreType.DMA((13,)),
            pltpu.SemaphoreType.DMA,
            pltpu.SemaphoreType.REGULAR,
        ] + [pltpu.VMEM((64, 7 * HD), i32)] * (NG + NG // 2),
        compiler_params=pltpu.CompilerParams(
            vmem_limit_bytes=100 * 1024 * 1024, disable_bounds_checks=True),
    )(A_x.reshape(S, D), A_wqkv, A_w_phi.reshape(H * DH, DH), A_wo,
      B_w_r.reshape(8, 128), B_w_gate, B_w_up, B_w_down, gate_w.reshape(8, 128))
    return out.reshape(1, S, D)
```

```python
import functools
import os
HALF = int(1)

import jax
import jax.numpy as jnp
from jax import lax
import jax.experimental.pallas as pl
import jax.experimental.pallas.tpu as pltpu

S, D, H, DH, F = 2048, 1024, 32, 32, 3584
NG = 8
T = 256
HT = T // 2
HD = D // 2
NTILE = S // T
NF = F // 128
LOG2E = 1.4426950408889634

OS0, WO0, WS0, PIN0, XQ_COLS = 5 * HD, 12 * HD, 14 * HD, 19 * HD, 20 * HD
PIN_LAG = int(os.environ.get('PIN_LAG', 2))

KV_LAG = (3, 5, 3, 6)
X_GAPS = (1, 2, 4, 5, 7, 9, 10, 12)
Q_GAPS = (0, 1, 3, 5)
O_LAG = 3
DMA_LAG = 4

NT = (((1,), (1,)), ((), ()))
NN = (((1,), (0,)), ((), ()))
f32 = jnp.float32
bf16 = jnp.bfloat16
i32 = jnp.int32


def _dot(a, b, dims):
    return lax.dot_general(a, b, dims, preferred_element_type=f32)


def _recip(x):
    r = pl.reciprocal(x, approx=True)
    return r * (2.0 - x * r)


def _r16(x):
    return x.astype(bf16).astype(f32)


def _ld(ref, r0, n, c0=None, nc=None, off=None):
    h0 = r0 // 2 if isinstance(r0, int) else pl.multiple_of(r0 // 2, 8)
    if off is not None:
        h0 = pl.multiple_of(h0 + off, 8)
    cols = slice(None) if c0 is None else pl.ds(c0, nc)
    return pltpu.bitcast(ref[pl.ds(h0, n // 2), cols], bf16)


def _st(ref, r0, val, c0=None):
    h0 = r0 // 2 if isinstance(r0, int) else pl.multiple_of(r0 // 2, 8)
    cols = slice(None) if c0 is None else pl.ds(c0, val.shape[1])
    ref[pl.ds(h0, val.shape[0] // 2), cols] = pltpu.bitcast(val.astype(bf16), i32)


def _dual_softmax(p):
    outs = []
    for h in range(p.shape[0] // DH):
        ph = p[h * DH:(h + 1) * DH]
        mx = jnp.max(ph, axis=0, keepdims=True)
        mn = jnp.min(ph, axis=0, keepdims=True)
        ep = jnp.exp2(ph - mx)
        en = jnp.exp2(mn - ph)
        outs.append(ep * _recip(jnp.sum(ep, axis=0, keepdims=True)))
        outs.append(en * _recip(jnp.sum(en, axis=0, keepdims=True)))
    return jnp.concatenate(outs, axis=0)


def _col(row):
    return jnp.broadcast_to(row, (128, 128)).T


def _lhs_terms(a11, a12, a21, a22):
    return [a11 + a22, a21 + a22, a11, a22, a11 + a12, a21 - a11, a12 - a22]


def _rhs_sums(b11, b12, b21, b22):
    return [b11 + b22, b12 - b22, b21 - b11, b11 + b12, b21 + b22]


RHS_SLOT = {0: 0, 2: 1, 3: 2, 5: 3, 6: 4}


def _strassen(prod, between, out):
    m4 = prod(3)
    between(0)
    m2 = prod(1)
    out(2, m2 + m4)
    between(1)
    c11 = m4 + prod(6)
    between(2)
    m1 = prod(0)
    c11 = c11 + m1
    c22 = m1 - m2
    between(3)
    m5 = prod(4)
    out(0, c11 - m5)
    between(4)
    m3 = prod(2)
    out(1, m3 + m5)
    c22 = c22 + m3
    between(5)
    out(3, c22 + prod(5))
    between(6)


def _kernel(x_hbm, wqkv_hbm, wphi_hbm, wo_hbm, wr_hbm, wg_hbm, wu_hbm, wd_hbm, gw_hbm,
            out_hbm,
            xs, xq, w3, wphi, wv2, wg, wu, wd, bd, kvs, gs, rs, xsel, ob,
            sems, osem, zsem, *wt):
    zero = pl.semaphore_read(zsem)
    uses = [0]

    def dz():
        uses[0] += 1
        return zero * (8 * uses[0])

    delayed = []

    def defer(gaps, fn):
        delayed.append([gaps, fn])

    def tick():
        for item in delayed:
            item[0] -= 1
        due = [item for item in delayed if item[0] <= 0]
        delayed[:] = [item for item in delayed if item[0] > 0]
        for _, fn in due:
            fn()

    def rows_cp(src, dst, r0, n, s):
        return pltpu.make_async_copy(src.at[pl.ds(r0, n)], dst.bitcast(bf16).at[pl.ds(r0, n)], sems.at[s])

    def w3_cp(c0, nc, s):
        return pltpu.make_async_copy(wqkv_hbm.at[:, pl.ds(c0, nc)],
                                     w3.bitcast(bf16).at[:, pl.ds(c0, nc)], sems.at[s])

    def wphi_cp(r0, n, s):
        return pltpu.make_async_copy(wphi_hbm.at[pl.ds(r0, n)], wphi.at[pl.ds(r0, n)], sems.at[s])

    def out_cp(r0, c0, nc):
        return pltpu.make_async_copy(ob.bitcast(bf16).at[pl.ds(r0, T), pl.ds(c0, nc)],
                                     out_hbm.at[pl.ds(r0, T), pl.ds(c0, nc)], osem)

    def start(cps):
        for cp in cps:
            cp.start()

    def wait(cps):
        for cp in cps:
            cp.wait()

    x_cps = [rows_cp(x_hbm, xs, t * T, T, t) for t in range(NTILE)]
    first = [wphi_cp(0, 256, 8), w3_cp(D, 256, 8), w3_cp(2 * D, 256, 8),
             pltpu.make_async_copy(wr_hbm, wv2.at[0], sems.at[8]),
             pltpu.make_async_copy(gw_hbm, wv2.at[1], sems.at[8])]
    second = [w3_cp(D + 256, 128, 9), w3_cp(2 * D + 256, 128, 9), wphi_cp(256, 768, 9)]
    third = [w3_cp(D + 384, 640, 10), w3_cp(2 * D + 384, 640, 10)]
    fourth = [w3_cp(0, D, 11)]
    for j in range(NTILE):
        for u in range(2):
            fourth.append(pltpu.make_async_copy(
                wo_hbm.at[pl.ds(u * HD + j * 64, 64)],
                xq.bitcast(bf16).at[pl.ds(j * HT + u * 64, 64), pl.ds(WO0, D)], sems.at[11]))
    ffn_cps = [rows_cp(src, dst, r, 64, 12)
               for src, dst in ((wg_hbm, wg), (wu_hbm, wu)) for r in range(0, D, 64)]
    ffn_cps += [rows_cp(wd_hbm, wd, r, 128, 12) for r in range(0, F, 128)]
    stream = list(ffn_cps)

    def feed():
        if stream:
            stream.pop(0).start()

    start(first + x_cps[:1])
    row = lax.broadcasted_iota(i32, (128, 128), 0)
    col = lax.broadcasted_iota(i32, (128, 128), 1)
    eye = jnp.where(lax.broadcasted_iota(i32, (128, DH), 0) % DH
                    == lax.broadcasted_iota(i32, (128, DH), 1), 1.0, 0.0).astype(bf16)
    wait(first)
    start(x_cps[1:3])

    def make_bd(g0, n, gaps=0):
        m = _dot(eye, wphi[pl.ds(g0 * 128, n * 128), :], NT)

        def store():
            for g in range(n):
                _st(bd, (g0 + g) * 128, jnp.where(row // DH == col // DH, m[:, g * 128:(g + 1) * 128], 0.0))

        if gaps:
            defer(gaps, store)
        else:
            store()

    def fold(g, c0):
        return _dot(_ld(bd, g * 128, 128), _ld(w3, 0, D, c0, 128), NT) * LOG2E

    def put_lhs(slot, r0, top, bot):
        for i, s in enumerate(_lhs_terms(top[:, :HD], top[:, HD:], bot[:, :HD], bot[:, HD:])):
            _st(wt[slot], r0, s, i * HD)

    def prep_kv(g):
        kt = fold(g, D + g * 128)
        vt = _ld(w3, 0, D, 2 * D + g * 128, 128).T.astype(f32)
        put_lhs(g, 64, vt[:64], vt[64:])
        put_lhs(g, 0, kt[:64], kt[64:])

    def prep_q(g):
        put_lhs(NG + g, 0, fold(g, g * 128), fold(g + 4, (g + 4) * 128))

    def put_rhs(load, rd, cd, n):
        for r in range(0, n, 16):
            for c in range(0, HD, 128):
                for i, s in enumerate(_rhs_sums(*[load(q, r, c).astype(f32) for q in range(4)])):
                    _st(xq, rd + r, s, cd + i * HD + c)

    def prep_x(t, r0, n):
        put_rhs(lambda q, r, c: _ld(xs, t * T + (q % 2) * HT + r0 + r, 16, (q // 2) * HD + c, 128),
                t * HT + r0, 0, n)

    def prep_wo(k):
        r0, off = (k // 4) * HT + (k % 4) * 16, dz()
        put_rhs(lambda q, r, c: _ld(xq, r0 + (q // 2) * 64, 16, WO0 + (q % 2) * HD + c, 128, off),
                r0, WS0, 16)

    def x_term(i, t):
        if i == 1:
            return _ld(xs, t * T, HT, 0, HD, dz())
        if i == 4:
            return _ld(xs, t * T + HT, HT, HD, HD, dz())
        return _ld(xq, t * HT, HT, RHS_SLOT[i] * HD, HD, dz())

    def project(slot, t, between, out):
        _strassen(lambda i: _dot(_ld(wt[slot], 0, 128, i * HD, HD, dz()), x_term(i, t), NT), between, out)

    st = {}
    wr = wv2[0].astype(f32)
    gw = wv2[1].astype(f32)
    upper = lax.broadcasted_iota(i32, (8, 128), 0) < 4
    score_rows = jnp.concatenate(
        [jnp.where(upper, wr[j:j + 1, :], gw[j:j + 1, :]) for j in range(8)], axis=1)

    def score_step(t, j):
        r0, k0 = t * T + (j // 2) * HT, (j % 2) * HD
        d = _dot(score_rows[:, k0:k0 + HD], _ld(xs, r0, HT, k0, HD), NT)
        if j % 2 == 0:
            st['sc'] = d
        else:
            d = d + st.pop('sc')
            rs[:, pl.ds(r0, HT)] = jnp.broadcast_to(_r16(d[:1]), (8, HT))
            gs[pl.ds(r0, HT), :] = _col(jax.nn.sigmoid(d[4:5]))

    def route():
        r = rs[...]
        pos = lax.broadcasted_iota(i32, r.shape, 1)
        best = jnp.max(jnp.where(r == r, r, -jnp.inf))
        idx = jnp.min(jnp.where(r == best, pos, S))
        st['idx'] = idx = jnp.where(idx >= S, 0, idx)
        st['score'] = jnp.sum(jnp.where(pos == idx, r, 0.0)[:1])
        st['blk'] = blk = pl.multiple_of((idx // 16) * 16, 16)
        sel = lax.broadcasted_iota(i32, (16, D), 0) == idx - blk
        xr = jnp.sum(jnp.where(sel, _ld(xs, blk, 16).astype(f32), 0.0), axis=0, keepdims=True)
        xsel[...] = jnp.broadcast_to(xr, (8, D))

    def ffn_step(k):
        n, j = divmod(k, 3)
        if j < 2 and n < NF:
            xr = xsel[pl.ds(pl.multiple_of(dz(), 8), 8), :]
            st['f', j] = _dot(xr, _ld((wg, wu)[j], 0, D, n * 128, 128), NN)
            if j == 1:
                gt, up = _r16(st.pop(('f', 0))), _r16(st.pop(('f', 1)))
                st['h', n] = _r16(_r16(gt * jax.nn.sigmoid(gt)) * up)
        if j == 2 and 1 <= n <= NF:
            yk = _dot(st.pop(('h', n - 1)), _ld(wd, (n - 1) * 128, 128), NN)
            st['y'] = yk if n == 1 else st['y'] + yk

    def pin(v):
        def store():
            xq[pl.ds(0, 8), pl.ds(PIN0, v.shape[1])] = pltpu.bitcast(v, i32)

        defer(PIN_LAG, store)

    def ffn_half(k):
        n, j = divmod(k, 6)
        if j < 4 and n < NF:
            k0 = (j % 2) * HD
            xr = xsel[pl.ds(pl.multiple_of(dz(), 8), 8), pl.ds(k0, HD)]
            st['f', j] = _dot(xr, _ld((wg, wu)[j // 2], k0, HD, n * 128, 128), NN)
            pin(st['f', j])
            if j == 3:
                gt = _r16(st.pop(('f', 0)) + st.pop(('f', 1)))
                up = _r16(st.pop(('f', 2)) + st.pop(('f', 3)))
                st['h', n] = _r16(_r16(gt * jax.nn.sigmoid(gt)) * up)
        if j >= 4 and 1 <= n <= NF:
            yk = _dot(st['h', n - 1], _ld(wd, (n - 1) * 128, 128, (j - 4) * HD, HD), NN)
            pin(yk)
            st['y', j - 4] = yk if n == 1 else st['y', j - 4] + yk
            if n == NF and j == 5:
                st['y'] = jnp.concatenate([st.pop(('y', 0)), st.pop(('y', 1))], axis=1)

    def patch():
        weight = _r16(jax.nn.sigmoid(jnp.full((16, D), st['score'], f32)))
        y = _r16(_r16(st.pop('y')[:1]) * weight)
        sel = lax.broadcasted_iota(i32, (16, D), 0) == st['idx'] - st['blk']
        xr = _ld(xs, st['blk'], 16).astype(f32)
        _st(xs, st['blk'], jnp.where(sel, xr + y, xr))

    r72 = lax.broadcasted_iota(i32, (72, 128), 0)
    c72 = lax.broadcasted_iota(i32, (72, 128), 1)
    kv_mask = jnp.where(r72 < 64, r72 // DH, r72 - 64) == c72 // 64
    accs = {}

    def kv_update(pair, is_first, is_last, r):
        phi = _dual_softmax(r[:64])
        d = _dot(r[64:].astype(bf16), phi.astype(bf16), NT)
        accs[pair] = (d, phi) if is_first else (accs[pair][0] + d, accs[pair][1] + phi)
        if is_last:
            d, z = accs.pop(pair)
            z = jnp.sum(z.T, axis=0, keepdims=True)
            kv = jnp.concatenate([d, jnp.broadcast_to(z, (8, 128))], axis=0)

            def store():
                kvs[pl.ds(pair * 72, 72), :] = jnp.where(kv_mask, _r16(kv), 0.0)

            defer(2, store)

    make_bd(0, 2)
    prep_kv(0)
    prep_kv(1)
    order = [(g, t) for t in range(NTILE) for g in range(2)]
    order += [(g, t) for g in range(2, NG) for t in range(NTILE)]
    for g, t in order:
        if (g, t) == (0, 0):
            wait(x_cps[:1])
            start(x_cps[3:5])
            prep_x(0, 0, HT)
        if (g, t) == (0, 1):
            wait(x_cps[1:3])
            start(x_cps[5:7])
            prep_x(1, 0, HT)
        if (g, t) == (0, 2):
            wait(x_cps[3:4])
            start(x_cps[7:] + second)
        if (g, t) == (0, 3):
            wait(x_cps[4:6])
            start(third)
        if (g, t) == (0, 5):
            wait(x_cps[6:] + second)
            start(fourth)
        if (g, t) == (2, 1):
            wait(third)
        if (g, t) == (4, 0):
            wait(fourth)

        def between(j):
            tick()
            if g == 1 and j in (0, 1, 3, 4):
                score_step(t, (0, 1, 3, 4).index(j))
            if j == 3 and g >= 3:
                feed()
            if j == 3 and g >= 4:
                prep_wo((g - 4) * NTILE + t)
            if g < 2 and 1 < t + 1 < NTILE and g * 7 + j in X_GAPS:
                prep_x(t + 1, X_GAPS.index(g * 7 + j) * 16, 16)
            if (g, t, j) == (0, 5, 0):
                make_bd(2, 6, 2)
            if j == 6 and g >= 1 and t == (6 if g == 1 else 1):
                if g + 1 < NG:
                    prep_kv(g + 1)
                else:
                    prep_q(0)
            if (g, t, j) == (2, 3, 6):
                route()

        def out(q, c):
            defer(KV_LAG[q], functools.partial(
                kv_update, 2 * g + q // 2, t == 0 and q % 2 == 0, t == NTILE - 1 and q % 2 == 1, c))

        project(g, t, between, out)

    pairs = []

    def attend(g, t, u, r):
        phi = _dual_softmax(r).astype(bf16)
        r0 = (2 * (g + 4 * (u % 2)) + u // 2) * 72
        nd = _dot(kvs[pl.ds(pl.multiple_of(r0 + dz(), 8), 72), :], phi, NN)
        inv = _recip(nd[64:72] + 1e-6)
        st['o', u] = jnp.concatenate([nd[0:32] * inv[0:1], nd[32:64] * inv[1:2]], axis=0)
        if u < 3:
            return
        lo = jnp.concatenate([st.pop(('o', 0)), st.pop(('o', 2))], axis=0)
        hi = jnp.concatenate([st.pop(('o', 1)), st.pop(('o', 3))], axis=0)
        terms = _lhs_terms(lo[:, :HT], hi[:, :HT], lo[:, HT:], hi[:, HT:])

        def store(i, n):
            v = jnp.concatenate(terms[i:i + n], axis=1).astype(bf16).T
            for k in range(n):
                _st(xq, t * HT, v[k * HT:(k + 1) * HT], OS0 + (i + k) * HD + g * 128)

        for i in range(0, 7, 2):
            defer(O_LAG + i // 2, functools.partial(store, i, min(2, 7 - i)))

    for g in range(NG // 2):
        for t in range(NTILE):
            if (g, t) == (3, 4):
                assert not stream
                wait(ffn_cps)

            def between(j):
                tick()
                if j == 3:
                    feed()
                if j in Q_GAPS and pairs:
                    pairs.pop(0)()
                if (t, j) == (1, 6) and g + 1 < NG // 2:
                    prep_q(g + 1)

            cs = {}
            project(NG + g, t, between, cs.__setitem__)
            lo = jnp.concatenate([cs[0], cs[1]], axis=1)
            hi = jnp.concatenate([cs[2], cs[3]], axis=1)
            for u, r in enumerate((lo[:64], hi[:64], lo[64:], hi[64:])):
                pairs.append(functools.partial(attend, g, t, u, r))

    routed = st['idx'] // T
    tiles = [i + (routed <= i).astype(i32) for i in range(NTILE - 1)] + [routed]
    ffn_gaps = 6 * (NF + 1)
    assert ffn_gaps + 2 < (NTILE - 1) * 28

    def wo_term(k, c):
        r0, c0 = (0, WO0) if k == 1 else (64, WO0 + HD) if k == 4 else (0, WS0 + RHS_SLOT[k] * HD)
        off = dz()
        return jnp.concatenate(
            [_ld(xq, j * HT + r0, 64, c0 + c * 128, 128, off) for j in range(NTILE)], axis=0)

    for i, tile in enumerate(tiles):
        r0 = pl.multiple_of(tile * T, T)
        for c in range(4):
            def between(j):
                tick()
                if j in Q_GAPS and pairs:
                    pairs.pop(0)()
                k = (i * 4 + c) * 7 + j
                if HALF and k < ffn_gaps:
                    ffn_half(k)
                if not HALF and k % 2 == 0 and k < ffn_gaps:
                    ffn_step(k // 2)
                if k == ffn_gaps + 2:
                    patch()

            def mix(q, a):
                rq, cq = r0 + (q // 2) * HT, (q % 2) * HD + c * 128
                gate = gs[pl.ds(pl.multiple_of(rq, HT), HT), :]
                b = _ld(xs, rq, HT, cq, 128).astype(f32)
                _st(ob, rq, b + gate * (a - b), cq)

            _strassen(lambda k: _dot(_ld(xq, 0, HT, OS0 + k * HD, HD, tile * (HT // 2) + dz()),
                                     wo_term(k, c), NN), between, mix)
            n = 1 if i == NTILE - 1 else 4
            if (c + 1) % n == 0:
                for u in range(2):
                    defer(DMA_LAG, out_cp(r0, u * HD + (c + 1 - n) * 128, n * 128).start)
    while delayed:
        tick()
    pltpu.make_async_copy(ob.bitcast(bf16), out_hbm, osem).wait()


@jax.jit
def pallas_gated_mix__linear_kernel_hedgehog__moe_arch_mod__prompt_kernel(A_x, A_wqkv, A_w_phi, A_wo, B_x, B_w_r, B_w_gate, B_w_up, B_w_down, gate_w):
    del B_x
    hbm = pl.BlockSpec(memory_space=pl.ANY)
    out = pl.pallas_call(
        _kernel,
        out_shape=jax.ShapeDtypeStruct((S, D), bf16),
        in_specs=[hbm] * 9,
        out_specs=hbm,
        scratch_shapes=[
            pltpu.VMEM((S // 2, D), i32),
            pltpu.VMEM((S // 4, XQ_COLS), i32),
            pltpu.VMEM((D // 2, 3 * D), i32),
            pltpu.VMEM((H * DH, DH), bf16),
            pltpu.VMEM((2, 8, 128), bf16),
            pltpu.VMEM((D // 2, F), i32),
            pltpu.VMEM((D // 2, F), i32),
            pltpu.VMEM((F // 2, D), i32),
            pltpu.VMEM((NG * 128 // 2, 128), i32),
            pltpu.VMEM((16 * 72, 128), f32),
            pltpu.VMEM((S, 128), f32),
            pltpu.VMEM((8, S), f32),
            pltpu.VMEM((8, D), f32),
            pltpu.VMEM((S // 2, D), i32),
            pltpu.SemaphoreType.DMA((13,)),
            pltpu.SemaphoreType.DMA,
            pltpu.SemaphoreType.REGULAR,
        ] + [pltpu.VMEM((64, 7 * HD), i32)] * (NG + NG // 2),
        compiler_params=pltpu.CompilerParams(
            vmem_limit_bytes=100 * 1024 * 1024, disable_bounds_checks=True),
    )(A_x.reshape(S, D), A_wqkv, A_w_phi.reshape(H * DH, DH), A_wo,
      B_w_r.reshape(8, 128), B_w_gate, B_w_up, B_w_down, gate_w.reshape(8, 128))
    return out.reshape(1, S, D)
```

```python
import functools
import os
HALF = int(1)

import jax
import jax.numpy as jnp
from jax import lax
import jax.experimental.pallas as pl
import jax.experimental.pallas.tpu as pltpu

S, D, H, DH, F = 2048, 1024, 32, 32, 3584
NG = 8
T = 256
HT = T // 2
HD = D // 2
NTILE = S // T
NF = F // 128
LOG2E = 1.4426950408889634

OS0, WO0, WS0, PIN0, XQ_COLS = 5 * HD, 12 * HD, 14 * HD, 19 * HD, 20 * HD
PIN_LAG = int(os.environ.get('PIN_LAG', 2))

KV_LAG = (3, 5, 3, 6)
X_GAPS = (1, 2, 4, 5, 7, 9, 10, 12)
Q_GAPS = (0, 1, 3, 5)
O_LAG = 3
DMA_LAG = 4

NT = (((1,), (1,)), ((), ()))
NN = (((1,), (0,)), ((), ()))
f32 = jnp.float32
bf16 = jnp.bfloat16
i32 = jnp.int32


def _dot(a, b, dims):
    return lax.dot_general(a, b, dims, preferred_element_type=f32)


def _recip(x):
    r = pl.reciprocal(x, approx=True)
    return r * (2.0 - x * r)


def _r16(x):
    return x.astype(bf16).astype(f32)


def _ld(ref, r0, n, c0=None, nc=None, off=None):
    h0 = r0 // 2 if isinstance(r0, int) else pl.multiple_of(r0 // 2, 8)
    if off is not None:
        h0 = pl.multiple_of(h0 + off, 8)
    cols = slice(None) if c0 is None else pl.ds(c0, nc)
    return pltpu.bitcast(ref[pl.ds(h0, n // 2), cols], bf16)


def _st(ref, r0, val, c0=None):
    h0 = r0 // 2 if isinstance(r0, int) else pl.multiple_of(r0 // 2, 8)
    cols = slice(None) if c0 is None else pl.ds(c0, val.shape[1])
    ref[pl.ds(h0, val.shape[0] // 2), cols] = pltpu.bitcast(val.astype(bf16), i32)


def _dual_softmax(p):
    outs = []
    for h in range(p.shape[0] // DH):
        ph = p[h * DH:(h + 1) * DH]
        mx = jnp.max(ph, axis=0, keepdims=True)
        mn = jnp.min(ph, axis=0, keepdims=True)
        ep = jnp.exp2(ph - mx)
        en = jnp.exp2(mn - ph)
        outs.append(ep * _recip(jnp.sum(ep, axis=0, keepdims=True)))
        outs.append(en * _recip(jnp.sum(en, axis=0, keepdims=True)))
    return jnp.concatenate(outs, axis=0)


def _col(row):
    return jnp.broadcast_to(row, (128, 128)).T


def _lhs_terms(a11, a12, a21, a22):
    return [a11 + a22, a21 + a22, a11, a22, a11 + a12, a21 - a11, a12 - a22]


def _rhs_sums(b11, b12, b21, b22):
    return [b11 + b22, b12 - b22, b21 - b11, b11 + b12, b21 + b22]


RHS_SLOT = {0: 0, 2: 1, 3: 2, 5: 3, 6: 4}


def _strassen(prod, between, out):
    m4 = prod(3)
    between(0)
    m2 = prod(1)
    out(2, m2 + m4)
    between(1)
    c11 = m4 + prod(6)
    between(2)
    m1 = prod(0)
    c11 = c11 + m1
    c22 = m1 - m2
    between(3)
    m5 = prod(4)
    out(0, c11 - m5)
    between(4)
    m3 = prod(2)
    out(1, m3 + m5)
    c22 = c22 + m3
    between(5)
    out(3, c22 + prod(5))
    between(6)


def _kernel(x_hbm, wqkv_hbm, wphi_hbm, wo_hbm, wr_hbm, wg_hbm, wu_hbm, wd_hbm, gw_hbm,
            out_hbm,
            xs, xq, w3, wphi, wv2, wg, wu, wd, bd, kvs, gs, rs, xsel, ob,
            sems, osem, zsem, *wt):
    zero = pl.semaphore_read(zsem)
    uses = [0]

    def dz():
        uses[0] += 1
        return zero * (8 * uses[0])

    delayed = []

    def defer(gaps, fn):
        delayed.append([gaps, fn])

    def tick():
        for item in delayed:
            item[0] -= 1
        due = [item for item in delayed if item[0] <= 0]
        delayed[:] = [item for item in delayed if item[0] > 0]
        for _, fn in due:
            fn()

    def rows_cp(src, dst, r0, n, s):
        return pltpu.make_async_copy(src.at[pl.ds(r0, n)], dst.bitcast(bf16).at[pl.ds(r0, n)], sems.at[s])

    def w3_cp(c0, nc, s):
        return pltpu.make_async_copy(wqkv_hbm.at[:, pl.ds(c0, nc)],
                                     w3.bitcast(bf16).at[:, pl.ds(c0, nc)], sems.at[s])

    def wphi_cp(r0, n, s):
        return pltpu.make_async_copy(wphi_hbm.at[pl.ds(r0, n)], wphi.at[pl.ds(r0, n)], sems.at[s])

    def out_cp(r0, c0, nc):
        return pltpu.make_async_copy(ob.bitcast(bf16).at[pl.ds(r0, T), pl.ds(c0, nc)],
                                     out_hbm.at[pl.ds(r0, T), pl.ds(c0, nc)], osem)

    def start(cps):
        for cp in cps:
            cp.start()

    def wait(cps):
        for cp in cps:
            cp.wait()

    x_cps = [rows_cp(x_hbm, xs, t * T, T, t) for t in range(NTILE)]
    first = [wphi_cp(0, 256, 8), w3_cp(D, 256, 8), w3_cp(2 * D, 256, 8),
             pltpu.make_async_copy(wr_hbm, wv2.at[0], sems.at[8]),
             pltpu.make_async_copy(gw_hbm, wv2.at[1], sems.at[8])]
    second = [w3_cp(D + 256, 128, 9), w3_cp(2 * D + 256, 128, 9), wphi_cp(256, 768, 9)]
    third = [w3_cp(D + 384, 640, 10), w3_cp(2 * D + 384, 640, 10)]
    fourth = [w3_cp(0, D, 11)]
    for j in range(NTILE):
        for u in range(2):
            fourth.append(pltpu.make_async_copy(
                wo_hbm.at[pl.ds(u * HD + j * 64, 64)],
                xq.bitcast(bf16).at[pl.ds(j * HT + u * 64, 64), pl.ds(WO0, D)], sems.at[11]))
    ffn_cps = [rows_cp(src, dst, r, 64, 12)
               for src, dst in ((wg_hbm, wg), (wu_hbm, wu)) for r in range(0, D, 64)]
    ffn_cps += [rows_cp(wd_hbm, wd, r, 128, 12) for r in range(0, F, 128)]
    stream = list(ffn_cps)

    def feed():
        if stream:
            stream.pop(0).start()

    start(first + x_cps[:1])
    row = lax.broadcasted_iota(i32, (128, 128), 0)
    col = lax.broadcasted_iota(i32, (128, 128), 1)
    eye = jnp.where(lax.broadcasted_iota(i32, (128, DH), 0) % DH
                    == lax.broadcasted_iota(i32, (128, DH), 1), 1.0, 0.0).astype(bf16)
    wait(first)
    start(x_cps[1:3])

    def make_bd(g0, n, gaps=0):
        m = _dot(eye, wphi[pl.ds(g0 * 128, n * 128), :], NT)

        def store():
            for g in range(n):
                _st(bd, (g0 + g) * 128, jnp.where(row // DH == col // DH, m[:, g * 128:(g + 1) * 128], 0.0))

        if gaps:
            defer(gaps, store)
        else:
            store()

    def fold(g, c0):
        return _dot(_ld(bd, g * 128, 128), _ld(w3, 0, D, c0, 128), NT) * LOG2E

    def put_lhs(slot, r0, top, bot):
        for i, s in enumerate(_lhs_terms(top[:, :HD], top[:, HD:], bot[:, :HD], bot[:, HD:])):
            _st(wt[slot], r0, s, i * HD)

    def prep_kv(g):
        kt = fold(g, D + g * 128)
        vt = _ld(w3, 0, D, 2 * D + g * 128, 128).T.astype(f32)
        put_lhs(g, 64, vt[:64], vt[64:])
        put_lhs(g, 0, kt[:64], kt[64:])

    def prep_q(g):
        put_lhs(NG + g, 0, fold(g, g * 128), fold(g + 4, (g + 4) * 128))

    def put_rhs(load, rd, cd, n):
        for r in range(0, n, 16):
            for c in range(0, HD, 128):
                for i, s in enumerate(_rhs_sums(*[load(q, r, c).astype(f32) for q in range(4)])):
                    _st(xq, rd + r, s, cd + i * HD + c)

    def prep_x(t, r0, n):
        put_rhs(lambda q, r, c: _ld(xs, t * T + (q % 2) * HT + r0 + r, 16, (q // 2) * HD + c, 128),
                t * HT + r0, 0, n)

    def prep_wo(k):
        r0, off = (k // 4) * HT + (k % 4) * 16, dz()
        put_rhs(lambda q, r, c: _ld(xq, r0 + (q // 2) * 64, 16, WO0 + (q % 2) * HD + c, 128, off),
                r0, WS0, 16)

    def x_term(i, t):
        if i == 1:
            return _ld(xs, t * T, HT, 0, HD, dz())
        if i == 4:
            return _ld(xs, t * T + HT, HT, HD, HD, dz())
        return _ld(xq, t * HT, HT, RHS_SLOT[i] * HD, HD, dz())

    def project(slot, t, between, out):
        _strassen(lambda i: _dot(_ld(wt[slot], 0, 128, i * HD, HD, dz()), x_term(i, t), NT), between, out)

    st = {}
    wr = wv2[0].astype(f32)
    gw = wv2[1].astype(f32)
    upper = lax.broadcasted_iota(i32, (8, 128), 0) < 4
    score_rows = jnp.concatenate(
        [jnp.where(upper, wr[j:j + 1, :], gw[j:j + 1, :]) for j in range(8)], axis=1)

    def score_step(t, j):
        r0, k0 = t * T + (j // 2) * HT, (j % 2) * HD
        d = _dot(score_rows[:, k0:k0 + HD], _ld(xs, r0, HT, k0, HD), NT)
        if j % 2 == 0:
            st['sc'] = d
        else:
            d = d + st.pop('sc')
            rs[:, pl.ds(r0, HT)] = jnp.broadcast_to(_r16(d[:1]), (8, HT))
            gs[pl.ds(r0, HT), :] = _col(jax.nn.sigmoid(d[4:5]))

    def route():
        r = rs[...]
        pos = lax.broadcasted_iota(i32, r.shape, 1)
        best = jnp.max(jnp.where(r == r, r, -jnp.inf))
        idx = jnp.min(jnp.where(r == best, pos, S))
        st['idx'] = idx = jnp.where(idx >= S, 0, idx)
        st['score'] = jnp.sum(jnp.where(pos == idx, r, 0.0)[:1])
        st['blk'] = blk = pl.multiple_of((idx // 16) * 16, 16)
        sel = lax.broadcasted_iota(i32, (16, D), 0) == idx - blk
        xr = jnp.sum(jnp.where(sel, _ld(xs, blk, 16).astype(f32), 0.0), axis=0, keepdims=True)
        xsel[...] = jnp.broadcast_to(xr, (8, D))

    def ffn_step(k):
        n, j = divmod(k, 3)
        if j < 2 and n < NF:
            xr = xsel[pl.ds(pl.multiple_of(dz(), 8), 8), :]
            st['f', j] = _dot(xr, _ld((wg, wu)[j], 0, D, n * 128, 128), NN)
            if j == 1:
                gt, up = _r16(st.pop(('f', 0))), _r16(st.pop(('f', 1)))
                st['h', n] = _r16(_r16(gt * jax.nn.sigmoid(gt)) * up)
        if j == 2 and 1 <= n <= NF:
            yk = _dot(st.pop(('h', n - 1)), _ld(wd, (n - 1) * 128, 128), NN)
            st['y'] = yk if n == 1 else st['y'] + yk

    def pin(v):
        def store():
            xq[pl.ds(0, 8), pl.ds(PIN0, v.shape[1])] = pltpu.bitcast(v, i32)

        defer(PIN_LAG, store)

    def ffn_half(k):
        n, j = divmod(k, 6)
        if j < 4 and n < NF:
            k0 = (j % 2) * HD
            xr = xsel[pl.ds(pl.multiple_of(dz(), 8), 8), pl.ds(k0, HD)]
            st['f', j] = _dot(xr, _ld((wg, wu)[j // 2], k0, HD, n * 128, 128), NN)
            pin(st['f', j])
            if j == 3:
                gt = _r16(st.pop(('f', 0)) + st.pop(('f', 1)))
                up = _r16(st.pop(('f', 2)) + st.pop(('f', 3)))
                st['h', n] = _r16(_r16(gt * jax.nn.sigmoid(gt)) * up)
        if j >= 4 and 1 <= n <= NF:
            yk = _dot(st['h', n - 1], _ld(wd, (n - 1) * 128, 128, (j - 4) * HD, HD), NN)
            pin(yk)
            st['y', j - 4] = yk if n == 1 else st['y', j - 4] + yk
            if n == NF and j == 5:
                st['y'] = jnp.concatenate([st.pop(('y', 0)), st.pop(('y', 1))], axis=1)

    def patch():
        weight = _r16(jax.nn.sigmoid(jnp.full((16, D), st['score'], f32)))
        y = _r16(_r16(st.pop('y')[:1]) * weight)
        sel = lax.broadcasted_iota(i32, (16, D), 0) == st['idx'] - st['blk']
        xr = _ld(xs, st['blk'], 16).astype(f32)
        _st(xs, st['blk'], jnp.where(sel, xr + y, xr))

    r72 = lax.broadcasted_iota(i32, (72, 128), 0)
    c72 = lax.broadcasted_iota(i32, (72, 128), 1)
    kv_mask = jnp.where(r72 < 64, r72 // DH, r72 - 64) == c72 // 64
    accs = {}

    def kv_update(pair, is_first, is_last, r):
        phi = _dual_softmax(r[:64])
        d = _dot(r[64:].astype(bf16), phi.astype(bf16), NT)
        accs[pair] = (d, phi) if is_first else (accs[pair][0] + d, accs[pair][1] + phi)
        if is_last:
            d, z = accs.pop(pair)
            z = jnp.sum(z.T, axis=0, keepdims=True)
            kv = jnp.concatenate([d, jnp.broadcast_to(z, (8, 128))], axis=0)

            def store():
                kvs[pl.ds(pair * 72, 72), :] = jnp.where(kv_mask, _r16(kv), 0.0)

            defer(2, store)

    make_bd(0, 2)
    prep_kv(0)
    prep_kv(1)
    order = [(g, t) for t in range(NTILE) for g in range(2)]
    order += [(g, t) for g in range(2, NG) for t in range(NTILE)]
    for g, t in order:
        if (g, t) == (0, 0):
            wait(x_cps[:1])
            start(x_cps[3:5])
            prep_x(0, 0, HT)
        if (g, t) == (0, 1):
            wait(x_cps[1:3])
            start(x_cps[5:7])
            prep_x(1, 0, HT)
        if (g, t) == (0, 2):
            wait(x_cps[3:4])
            start(x_cps[7:] + second)
        if (g, t) == (0, 3):
            wait(x_cps[4:6])
            start(third)
        if (g, t) == (0, 5):
            wait(x_cps[6:] + second)
            start(fourth)
        if (g, t) == (2, 5):
            wait(third + fourth)

        def between(j):
            tick()
            if g == 1 and j in (0, 1, 3, 4):
                score_step(t, (0, 1, 3, 4).index(j))
            if j == 3 and g >= 3:
                feed()
            if j == 3 and g >= 4:
                prep_wo((g - 4) * NTILE + t)
            if g < 2 and 1 < t + 1 < NTILE and g * 7 + j in X_GAPS:
                prep_x(t + 1, X_GAPS.index(g * 7 + j) * 16, 16)
            if (g, t, j) == (0, 5, 0):
                make_bd(2, 6, 2)
            if j == 6 and g >= 1 and t == (6 if g == 1 else 5 if g == 2 else 1):
                if g + 1 < NG:
                    prep_kv(g + 1)
                else:
                    prep_q(0)
            if (g, t, j) == (2, 3, 6):
                route()

        def out(q, c):
            defer(KV_LAG[q], functools.partial(
                kv_update, 2 * g + q // 2, t == 0 and q % 2 == 0, t == NTILE - 1 and q % 2 == 1, c))

        project(g, t, between, out)

    pairs = []

    def attend(g, t, u, r):
        phi = _dual_softmax(r).astype(bf16)
        r0 = (2 * (g + 4 * (u % 2)) + u // 2) * 72
        nd = _dot(kvs[pl.ds(pl.multiple_of(r0 + dz(), 8), 72), :], phi, NN)
        inv = _recip(nd[64:72] + 1e-6)
        st['o', u] = jnp.concatenate([nd[0:32] * inv[0:1], nd[32:64] * inv[1:2]], axis=0)
        if u < 3:
            return
        lo = jnp.concatenate([st.pop(('o', 0)), st.pop(('o', 2))], axis=0)
        hi = jnp.concatenate([st.pop(('o', 1)), st.pop(('o', 3))], axis=0)
        terms = _lhs_terms(lo[:, :HT], hi[:, :HT], lo[:, HT:], hi[:, HT:])

        def store(i, n):
            v = jnp.concatenate(terms[i:i + n], axis=1).astype(bf16).T
            for k in range(n):
                _st(xq, t * HT, v[k * HT:(k + 1) * HT], OS0 + (i + k) * HD + g * 128)

        for i in range(0, 7, 2):
            defer(O_LAG + i // 2, functools.partial(store, i, min(2, 7 - i)))

    for g in range(NG // 2):
        for t in range(NTILE):
            if (g, t) == (3, 4):
                assert not stream
                wait(ffn_cps)

            def between(j):
                tick()
                if j == 3:
                    feed()
                if j in Q_GAPS and pairs:
                    pairs.pop(0)()
                if (t, j) == (1, 6) and g + 1 < NG // 2:
                    prep_q(g + 1)

            cs = {}
            project(NG + g, t, between, cs.__setitem__)
            lo = jnp.concatenate([cs[0], cs[1]], axis=1)
            hi = jnp.concatenate([cs[2], cs[3]], axis=1)
            for u, r in enumerate((lo[:64], hi[:64], lo[64:], hi[64:])):
                pairs.append(functools.partial(attend, g, t, u, r))

    routed = st['idx'] // T
    tiles = [i + (routed <= i).astype(i32) for i in range(NTILE - 1)] + [routed]
    ffn_gaps = 6 * (NF + 1)
    assert ffn_gaps + 2 < (NTILE - 1) * 28

    def wo_term(k, c):
        r0, c0 = (0, WO0) if k == 1 else (64, WO0 + HD) if k == 4 else (0, WS0 + RHS_SLOT[k] * HD)
        off = dz()
        return jnp.concatenate(
            [_ld(xq, j * HT + r0, 64, c0 + c * 128, 128, off) for j in range(NTILE)], axis=0)

    for i, tile in enumerate(tiles):
        r0 = pl.multiple_of(tile * T, T)
        for c in range(4):
            def between(j):
                tick()
                if j in Q_GAPS and pairs:
                    pairs.pop(0)()
                k = (i * 4 + c) * 7 + j
                if HALF and k < ffn_gaps:
                    ffn_half(k)
                if not HALF and k % 2 == 0 and k < ffn_gaps:
                    ffn_step(k // 2)
                if k == ffn_gaps + 2:
                    patch()

            def mix(q, a):
                rq, cq = r0 + (q // 2) * HT, (q % 2) * HD + c * 128
                gate = gs[pl.ds(pl.multiple_of(rq, HT), HT), :]
                b = _ld(xs, rq, HT, cq, 128).astype(f32)
                _st(ob, rq, b + gate * (a - b), cq)

            _strassen(lambda k: _dot(_ld(xq, 0, HT, OS0 + k * HD, HD, tile * (HT // 2) + dz()),
                                     wo_term(k, c), NN), between, mix)
            n = 1 if i == NTILE - 1 else 4
            if (c + 1) % n == 0:
                for u in range(2):
                    defer(DMA_LAG, out_cp(r0, u * HD + (c + 1 - n) * 128, n * 128).start)
    while delayed:
        tick()
    pltpu.make_async_copy(ob.bitcast(bf16), out_hbm, osem).wait()


@jax.jit
def pallas_gated_mix__linear_kernel_hedgehog__moe_arch_mod__prompt_kernel(A_x, A_wqkv, A_w_phi, A_wo, B_x, B_w_r, B_w_gate, B_w_up, B_w_down, gate_w):
    del B_x
    hbm = pl.BlockSpec(memory_space=pl.ANY)
    out = pl.pallas_call(
        _kernel,
        out_shape=jax.ShapeDtypeStruct((S, D), bf16),
        in_specs=[hbm] * 9,
        out_specs=hbm,
        scratch_shapes=[
            pltpu.VMEM((S // 2, D), i32),
            pltpu.VMEM((S // 4, XQ_COLS), i32),
            pltpu.VMEM((D // 2, 3 * D), i32),
            pltpu.VMEM((H * DH, DH), bf16),
            pltpu.VMEM((2, 8, 128), bf16),
            pltpu.VMEM((D // 2, F), i32),
            pltpu.VMEM((D // 2, F), i32),
            pltpu.VMEM((F // 2, D), i32),
            pltpu.VMEM((NG * 128 // 2, 128), i32),
            pltpu.VMEM((16 * 72, 128), f32),
            pltpu.VMEM((S, 128), f32),
            pltpu.VMEM((8, S), f32),
            pltpu.VMEM((8, D), f32),
            pltpu.VMEM((S // 2, D), i32),
            pltpu.SemaphoreType.DMA((13,)),
            pltpu.SemaphoreType.DMA,
            pltpu.SemaphoreType.REGULAR,
        ] + [pltpu.VMEM((64, 7 * HD), i32)] * (NG + NG // 2),
        compiler_params=pltpu.CompilerParams(
            vmem_limit_bytes=100 * 1024 * 1024, disable_bounds_checks=True),
    )(A_x.reshape(S, D), A_wqkv, A_w_phi.reshape(H * DH, DH), A_wo,
      B_w_r.reshape(8, 128), B_w_gate, B_w_up, B_w_down, gate_w.reshape(8, 128))
    return out.reshape(1, S, D)
```

```python
import functools

import jax
import jax.numpy as jnp
from jax import lax
import jax.experimental.pallas as pl
import jax.experimental.pallas.tpu as pltpu

S, D, H, DH, F = 2048, 1024, 32, 32, 3584
NG = 8
T = 256
HT = T // 2
HD = D // 2
NTILE = S // T
NF = F // 128
LOG2E = 1.4426950408889634

OS0, WO0, WS0, PIN0, XQ_COLS = 5 * HD, 12 * HD, 14 * HD, 19 * HD, 20 * HD

KV_LAG = (3, 5, 3, 6)
X_GAPS = (1, 2, 4, 5, 7, 9, 10, 12)
Q_GAPS = (0, 1, 4, 5)
O_LAG = 3
PIN_LAG = 2
DMA_LAG = 4

NT = (((1,), (1,)), ((), ()))
NN = (((1,), (0,)), ((), ()))
f32 = jnp.float32
bf16 = jnp.bfloat16
i32 = jnp.int32


def _dot(a, b, dims):
    return lax.dot_general(a, b, dims, preferred_element_type=f32)


def _recip(x):
    r = pl.reciprocal(x, approx=True)
    return r * (2.0 - x * r)


def _r16(x):
    return x.astype(bf16).astype(f32)


def _ld(ref, r0, n, c0=None, nc=None, off=None):
    h0 = r0 // 2 if isinstance(r0, int) else pl.multiple_of(r0 // 2, 8)
    if off is not None:
        h0 = pl.multiple_of(h0 + off, 8)
    cols = slice(None) if c0 is None else pl.ds(c0, nc)
    return pltpu.bitcast(ref[pl.ds(h0, n // 2), cols], bf16)


def _st(ref, r0, val, c0=None):
    h0 = r0 // 2 if isinstance(r0, int) else pl.multiple_of(r0 // 2, 8)
    cols = slice(None) if c0 is None else pl.ds(c0, val.shape[1])
    ref[pl.ds(h0, val.shape[0] // 2), cols] = pltpu.bitcast(val.astype(bf16), i32)


def _dual_softmax(p):
    outs = []
    for h in range(p.shape[0] // DH):
        ph = p[h * DH:(h + 1) * DH]
        mx = jnp.max(ph, axis=0, keepdims=True)
        mn = jnp.min(ph, axis=0, keepdims=True)
        ep = jnp.exp2(ph - mx)
        en = jnp.exp2(mn - ph)
        outs.append(ep * _recip(jnp.sum(ep, axis=0, keepdims=True)))
        outs.append(en * _recip(jnp.sum(en, axis=0, keepdims=True)))
    return jnp.concatenate(outs, axis=0)


def _col(row):
    return jnp.broadcast_to(row, (128, 128)).T


def _lhs_terms(a11, a12, a21, a22):
    return [a11 + a22, a21 + a22, a11, a22, a11 + a12, a21 - a11, a12 - a22]


def _rhs_sums(b11, b12, b21, b22):
    return [b11 + b22, b12 - b22, b21 - b11, b11 + b12, b21 + b22]


RHS_SLOT = {0: 0, 2: 1, 3: 2, 5: 3, 6: 4}


def _strassen(prod, between, out):
    m4 = prod(3)
    between(0)
    m2 = prod(1)
    out(2, m2 + m4)
    between(1)
    c11 = m4 + prod(6)
    between(2)
    m1 = prod(0)
    c11 = c11 + m1
    c22 = m1 - m2
    between(3)
    m5 = prod(4)
    out(0, c11 - m5)
    between(4)
    m3 = prod(2)
    out(1, m3 + m5)
    c22 = c22 + m3
    between(5)
    out(3, c22 + prod(5))
    between(6)


def _kernel(x_hbm, wqkv_hbm, wphi_hbm, wo_hbm, wr_hbm, wg_hbm, wu_hbm, wd_hbm, gw_hbm,
            out_hbm,
            xs, xq, w3, wphi, wv2, wg, wu, wd, bd, kvs, gs, rs, xsel, ob,
            sems, osem, zsem, *wt):
    zero = pl.semaphore_read(zsem)
    uses = [0]

    def dz():
        uses[0] += 1
        return zero * (8 * uses[0])

    delayed = []

    def defer(gaps, fn):
        delayed.append([gaps, fn])

    def tick():
        for item in delayed:
            item[0] -= 1
        due = [item for item in delayed if item[0] <= 0]
        delayed[:] = [item for item in delayed if item[0] > 0]
        for _, fn in due:
            fn()

    def rows_cp(src, dst, r0, n, s):
        return pltpu.make_async_copy(src.at[pl.ds(r0, n)], dst.bitcast(bf16).at[pl.ds(r0, n)], sems.at[s])

    def w3_cp(c0, nc, s):
        return pltpu.make_async_copy(wqkv_hbm.at[:, pl.ds(c0, nc)],
                                     w3.bitcast(bf16).at[:, pl.ds(c0, nc)], sems.at[s])

    def wphi_cp(r0, n, s):
        return pltpu.make_async_copy(wphi_hbm.at[pl.ds(r0, n)], wphi.at[pl.ds(r0, n)], sems.at[s])

    def out_cp(r0, c0, nc):
        return pltpu.make_async_copy(ob.bitcast(bf16).at[pl.ds(r0, T), pl.ds(c0, nc)],
                                     out_hbm.at[pl.ds(r0, T), pl.ds(c0, nc)], osem)

    def start(cps):
        for cp in cps:
            cp.start()

    def wait(cps):
        for cp in cps:
            cp.wait()

    x_cps = [rows_cp(x_hbm, xs, t * T, T, t) for t in range(NTILE)]
    first = [wphi_cp(0, 256, 8), w3_cp(D, 256, 8), w3_cp(2 * D, 256, 8),
             pltpu.make_async_copy(wr_hbm, wv2.at[0], sems.at[8]),
             pltpu.make_async_copy(gw_hbm, wv2.at[1], sems.at[8])]
    second = [w3_cp(D + 256, 128, 9), w3_cp(2 * D + 256, 128, 9), wphi_cp(256, 768, 9)]
    third = [w3_cp(D + 384, 640, 10), w3_cp(2 * D + 384, 640, 10)]
    fourth = [w3_cp(0, D, 11)]
    for j in range(NTILE):
        for u in range(2):
            fourth.append(pltpu.make_async_copy(
                wo_hbm.at[pl.ds(u * HD + j * 64, 64)],
                xq.bitcast(bf16).at[pl.ds(j * HT + u * 64, 64), pl.ds(WO0, D)], sems.at[11]))
    ffn_cps = [rows_cp(src, dst, r, 64, 12)
               for src, dst in ((wg_hbm, wg), (wu_hbm, wu)) for r in range(0, D, 64)]
    ffn_cps += [rows_cp(wd_hbm, wd, r, 128, 12) for r in range(0, F, 128)]
    stream = list(ffn_cps)

    def feed():
        if stream:
            stream.pop(0).start()

    start(first + x_cps[:1])
    row = lax.broadcasted_iota(i32, (128, 128), 0)
    col = lax.broadcasted_iota(i32, (128, 128), 1)
    eye = jnp.where(lax.broadcasted_iota(i32, (128, DH), 0) % DH
                    == lax.broadcasted_iota(i32, (128, DH), 1), 1.0, 0.0).astype(bf16)
    wait(first)
    start(x_cps[1:3])

    def make_bd(g0, n, gaps=0):
        m = _dot(eye, wphi[pl.ds(g0 * 128, n * 128), :], NT)

        def store():
            for g in range(n):
                _st(bd, (g0 + g) * 128, jnp.where(row // DH == col // DH, m[:, g * 128:(g + 1) * 128], 0.0))

        if gaps:
            defer(gaps, store)
        else:
            store()

    def fold(g, c0):
        return _dot(_ld(bd, g * 128, 128), _ld(w3, 0, D, c0, 128), NT) * LOG2E

    def put_lhs(slot, r0, top, bot):
        for i, s in enumerate(_lhs_terms(top[:, :HD], top[:, HD:], bot[:, :HD], bot[:, HD:])):
            _st(wt[slot], r0, s, i * HD)

    def prep_kv(g):
        kt = fold(g, D + g * 128)
        vt = _ld(w3, 0, D, 2 * D + g * 128, 128).T.astype(f32)
        put_lhs(g, 64, vt[:64], vt[64:])
        put_lhs(g, 0, kt[:64], kt[64:])

    def prep_q(g):
        put_lhs(NG + g, 0, fold(g, g * 128), fold(g + 4, (g + 4) * 128))

    def put_rhs(load, rd, cd, n):
        for r in range(0, n, 16):
            for c in range(0, HD, 128):
                for i, s in enumerate(_rhs_sums(*[load(q, r, c).astype(f32) for q in range(4)])):
                    _st(xq, rd + r, s, cd + i * HD + c)

    def prep_x(t, r0, n):
        put_rhs(lambda q, r, c: _ld(xs, t * T + (q % 2) * HT + r0 + r, 16, (q // 2) * HD + c, 128),
                t * HT + r0, 0, n)

    def prep_wo(k):
        r0, off = (k // 4) * HT + (k % 4) * 16, dz()
        put_rhs(lambda q, r, c: _ld(xq, r0 + (q // 2) * 64, 16, WO0 + (q % 2) * HD + c, 128, off),
                r0, WS0, 16)

    def x_term(i, t):
        if i == 1:
            return _ld(xs, t * T, HT, 0, HD, dz())
        if i == 4:
            return _ld(xs, t * T + HT, HT, HD, HD, dz())
        return _ld(xq, t * HT, HT, RHS_SLOT[i] * HD, HD, dz())

    def project(slot, t, between, out):
        _strassen(lambda i: _dot(_ld(wt[slot], 0, 128, i * HD, HD, dz()), x_term(i, t), NT), between, out)

    st = {}
    wr = wv2[0].astype(f32)
    gw = wv2[1].astype(f32)
    upper = lax.broadcasted_iota(i32, (8, 128), 0) < 4
    score_rows = jnp.concatenate(
        [jnp.where(upper, wr[j:j + 1, :], gw[j:j + 1, :]) for j in range(8)], axis=1)

    def score_step(t, j):
        r0, k0 = t * T + (j // 2) * HT, (j % 2) * HD
        d = _dot(score_rows[:, k0:k0 + HD], _ld(xs, r0, HT, k0, HD), NT)
        if j % 2 == 0:
            st['sc'] = d
        else:
            d = d + st.pop('sc')
            rs[:, pl.ds(r0, HT)] = jnp.broadcast_to(_r16(d[:1]), (8, HT))
            gs[pl.ds(r0, HT), :] = _col(jax.nn.sigmoid(d[4:5]))

    def route():
        r = rs[...]
        pos = lax.broadcasted_iota(i32, r.shape, 1)
        best = jnp.max(jnp.where(r == r, r, -jnp.inf))
        idx = jnp.min(jnp.where(r == best, pos, S))
        st['idx'] = idx = jnp.where(idx >= S, 0, idx)
        st['score'] = jnp.sum(jnp.where(pos == idx, r, 0.0)[:1])
        st['blk'] = blk = pl.multiple_of((idx // 16) * 16, 16)
        sel = lax.broadcasted_iota(i32, (16, D), 0) == idx - blk
        xr = jnp.sum(jnp.where(sel, _ld(xs, blk, 16).astype(f32), 0.0), axis=0, keepdims=True)
        xsel[...] = jnp.broadcast_to(xr, (8, D))

    def pin(v):
        def store():
            xq[pl.ds(0, 8), pl.ds(PIN0, v.shape[1])] = pltpu.bitcast(v, i32)

        defer(PIN_LAG, store)

    def ffn_step(k):
        n, j = divmod(k, 6)
        if j < 4 and n < NF:
            k0 = (j % 2) * HD
            xr = xsel[pl.ds(pl.multiple_of(dz(), 8), 8), pl.ds(k0, HD)]
            st['f', j] = _dot(xr, _ld((wg, wu)[j // 2], k0, HD, n * 128, 128), NN)
            pin(st['f', j])
            if j == 3:
                gt = _r16(st.pop(('f', 0)) + st.pop(('f', 1)))
                up = _r16(st.pop(('f', 2)) + st.pop(('f', 3)))
                st['h', n] = _r16(_r16(gt * jax.nn.sigmoid(gt)) * up)
        if j >= 4 and 1 <= n <= NF:
            yk = _dot(st['h', n - 1], _ld(wd, (n - 1) * 128, 128, (j - 4) * HD, HD), NN)
            pin(yk)
            st['y', j - 4] = yk if n == 1 else st['y', j - 4] + yk
            if n == NF and j == 5:
                st['y'] = jnp.concatenate([st.pop(('y', 0)), st.pop(('y', 1))], axis=1)

    def patch():
        weight = _r16(jax.nn.sigmoid(jnp.full((16, D), st['score'], f32)))
        y = _r16(_r16(st.pop('y')[:1]) * weight)
        sel = lax.broadcasted_iota(i32, (16, D), 0) == st['idx'] - st['blk']
        xr = _ld(xs, st['blk'], 16).astype(f32)
        _st(xs, st['blk'], jnp.where(sel, xr + y, xr))

    r72 = lax.broadcasted_iota(i32, (72, 128), 0)
    c72 = lax.broadcasted_iota(i32, (72, 128), 1)
    kv_mask = jnp.where(r72 < 64, r72 // DH, r72 - 64) == c72 // 64
    accs = {}

    def kv_update(pair, is_first, is_last, r):
        phi = _dual_softmax(r[:64])
        d = _dot(r[64:].astype(bf16), phi.astype(bf16), NT)
        accs[pair] = (d, phi) if is_first else (accs[pair][0] + d, accs[pair][1] + phi)
        if is_last:
            d, z = accs.pop(pair)
            z = jnp.sum(z.T, axis=0, keepdims=True)
            kv = jnp.concatenate([d, jnp.broadcast_to(z, (8, 128))], axis=0)

            def store():
                kvs[pl.ds(pair * 72, 72), :] = jnp.where(kv_mask, _r16(kv), 0.0)

            defer(2, store)

    make_bd(0, 2)
    prep_kv(0)
    prep_kv(1)
    order = [(g, t) for t in range(NTILE) for g in range(2)]
    order += [(g, t) for g in range(2, NG) for t in range(NTILE)]
    for g, t in order:
        if (g, t) == (0, 0):
            wait(x_cps[:1])
            start(x_cps[3:5])
            prep_x(0, 0, HT)
        if (g, t) == (0, 1):
            wait(x_cps[1:3])
            start(x_cps[5:7])
            prep_x(1, 0, HT)
        if (g, t) == (0, 2):
            wait(x_cps[3:4])
            start(x_cps[7:] + second)
        if (g, t) == (0, 3):
            wait(x_cps[4:6])
            start(third)
        if (g, t) == (0, 5):
            wait(x_cps[6:] + second)
            start(fourth)
        if (g, t) == (2, 5):
            wait(third + fourth)

        def between(j):
            tick()
            if g == 1 and j in (0, 1, 3, 4):
                score_step(t, (0, 1, 3, 4).index(j))
            if j == 3 and g >= 3:
                feed()
            if j == 3 and g >= 4:
                prep_wo((g - 4) * NTILE + t)
            if g < 2 and 1 < t + 1 < NTILE and g * 7 + j in X_GAPS:
                prep_x(t + 1, X_GAPS.index(g * 7 + j) * 16, 16)
            if (g, t, j) == (0, 5, 0):
                make_bd(2, 6, 2)
            if j == 6 and g >= 1 and t == (6 if g == 1 else 5 if g == 2 else 1):
                if g + 1 < NG:
                    prep_kv(g + 1)
                else:
                    prep_q(0)
            if (g, t, j) == (2, 3, 6):
                route()

        def out(q, c):
            defer(KV_LAG[q], functools.partial(
                kv_update, 2 * g + q // 2, t == 0 and q % 2 == 0, t == NTILE - 1 and q % 2 == 1, c))

        project(g, t, between, out)

    pairs = []

    def attend(g, t, u, r):
        phi = _dual_softmax(r).astype(bf16)
        r0 = (2 * (g + 4 * (u % 2)) + u // 2) * 72
        nd = _dot(kvs[pl.ds(pl.multiple_of(r0 + dz(), 8), 72), :], phi, NN)
        inv = _recip(nd[64:72] + 1e-6)
        st['o', u] = jnp.concatenate([nd[0:32] * inv[0:1], nd[32:64] * inv[1:2]], axis=0)
        if u < 3:
            return
        lo = jnp.concatenate([st.pop(('o', 0)), st.pop(('o', 2))], axis=0)
        hi = jnp.concatenate([st.pop(('o', 1)), st.pop(('o', 3))], axis=0)
        terms = _lhs_terms(lo[:, :HT], hi[:, :HT], lo[:, HT:], hi[:, HT:])

        def store(i, n):
            v = jnp.concatenate(terms[i:i + n], axis=1).astype(bf16).T
            for k in range(n):
                _st(xq, t * HT, v[k * HT:(k + 1) * HT], OS0 + (i + k) * HD + g * 128)

        for i in range(0, 7, 2):
            defer(O_LAG + i // 2, functools.partial(store, i, min(2, 7 - i)))

    for g in range(NG // 2):
        for t in range(NTILE):
            if (g, t) == (3, 4):
                assert not stream
                wait(ffn_cps)

            def between(j):
                tick()
                if j == 3:
                    feed()
                if j in Q_GAPS and pairs:
                    pairs.pop(0)()
                if (t, j) == (1, 4) and g + 1 < NG // 2:
                    prep_q(g + 1)

            cs = {}
            project(NG + g, t, between, cs.__setitem__)
            lo = jnp.concatenate([cs[0], cs[1]], axis=1)
            hi = jnp.concatenate([cs[2], cs[3]], axis=1)
            for u, r in enumerate((lo[:64], hi[:64], lo[64:], hi[64:])):
                pairs.append(functools.partial(attend, g, t, u, r))

    routed = st['idx'] // T
    tiles = [i + (routed <= i).astype(i32) for i in range(NTILE - 1)] + [routed]
    ffn_gaps = 6 * (NF + 1)
    assert ffn_gaps + 2 < (NTILE - 1) * 28

    def wo_term(k, c):
        r0, c0 = (0, WO0) if k == 1 else (64, WO0 + HD) if k == 4 else (0, WS0 + RHS_SLOT[k] * HD)
        off = dz()
        return jnp.concatenate(
            [_ld(xq, j * HT + r0, 64, c0 + c * 128, 128, off) for j in range(NTILE)], axis=0)

    for i, tile in enumerate(tiles):
        r0 = pl.multiple_of(tile * T, T)
        for c in range(4):
            def between(j):
                tick()
                if j in Q_GAPS and pairs:
                    pairs.pop(0)()
                k = (i * 4 + c) * 7 + j
                if k < ffn_gaps:
                    ffn_step(k)
                if k == ffn_gaps + 2:
                    patch()

            def mix(q, a):
                rq, cq = r0 + (q // 2) * HT, (q % 2) * HD + c * 128
                gate = gs[pl.ds(pl.multiple_of(rq, HT), HT), :]
                b = _ld(xs, rq, HT, cq, 128).astype(f32)
                _st(ob, rq, b + gate * (a - b), cq)

            _strassen(lambda k: _dot(_ld(xq, 0, HT, OS0 + k * HD, HD, tile * (HT // 2) + dz()),
                                     wo_term(k, c), NN), between, mix)
            n = 1 if i == NTILE - 1 else 4
            if (c + 1) % n == 0:
                for u in range(2):
                    defer(DMA_LAG, out_cp(r0, u * HD + (c + 1 - n) * 128, n * 128).start)
    while delayed:
        tick()
    pltpu.make_async_copy(ob.bitcast(bf16), out_hbm, osem).wait()


@jax.jit
def pallas_gated_mix__linear_kernel_hedgehog__moe_arch_mod__prompt_kernel(A_x, A_wqkv, A_w_phi, A_wo, B_x, B_w_r, B_w_gate, B_w_up, B_w_down, gate_w):
    del B_x
    hbm = pl.BlockSpec(memory_space=pl.ANY)
    out = pl.pallas_call(
        _kernel,
        out_shape=jax.ShapeDtypeStruct((S, D), bf16),
        in_specs=[hbm] * 9,
        out_specs=hbm,
        scratch_shapes=[
            pltpu.VMEM((S // 2, D), i32),
            pltpu.VMEM((S // 4, XQ_COLS), i32),
            pltpu.VMEM((D // 2, 3 * D), i32),
            pltpu.VMEM((H * DH, DH), bf16),
            pltpu.VMEM((2, 8, 128), bf16),
            pltpu.VMEM((D // 2, F), i32),
            pltpu.VMEM((D // 2, F), i32),
            pltpu.VMEM((F // 2, D), i32),
            pltpu.VMEM((NG * 128 // 2, 128), i32),
            pltpu.VMEM((16 * 72, 128), f32),
            pltpu.VMEM((S, 128), f32),
            pltpu.VMEM((8, S), f32),
            pltpu.VMEM((8, D), f32),
            pltpu.VMEM((S // 2, D), i32),
            pltpu.SemaphoreType.DMA((13,)),
            pltpu.SemaphoreType.DMA,
            pltpu.SemaphoreType.REGULAR,
        ] + [pltpu.VMEM((64, 7 * HD), i32)] * (NG + NG // 2),
        compiler_params=pltpu.CompilerParams(
            vmem_limit_bytes=100 * 1024 * 1024, disable_bounds_checks=True),
    )(A_x.reshape(S, D), A_wqkv, A_w_phi.reshape(H * DH, DH), A_wo,
      B_w_r.reshape(8, 128), B_w_gate, B_w_up, B_w_down, gate_w.reshape(8, 128))
    return out.reshape(1, S, D)
```

```python
import functools

import jax
import jax.numpy as jnp
from jax import lax
import jax.experimental.pallas as pl
import jax.experimental.pallas.tpu as pltpu

S, D, H, DH, F = 2048, 1024, 32, 32, 3584
NG = 8
T = 256
HT = T // 2
HD = D // 2
NTILE = S // T
NF = F // 128
LOG2E = 1.4426950408889634

OS0, WO0, WS0, PIN0, XQ_COLS = 5 * HD, 12 * HD, 14 * HD, 19 * HD, 20 * HD + 128

KV_LAG = (3, 5, 3, 6)
X_GAPS = (1, 2, 4, 5, 7, 9, 10, 12)
Q_GAPS = (0, 1, 4, 5)
O_LAG = 3
PIN_LAG = 2
DMA_LAG = 4

NT = (((1,), (1,)), ((), ()))
NN = (((1,), (0,)), ((), ()))
f32 = jnp.float32
bf16 = jnp.bfloat16
i32 = jnp.int32


def _dot(a, b, dims):
    return lax.dot_general(a, b, dims, preferred_element_type=f32)


def _recip(x):
    r = pl.reciprocal(x, approx=True)
    return r * (2.0 - x * r)


def _r16(x):
    return x.astype(bf16).astype(f32)


def _ld(ref, r0, n, c0=None, nc=None, off=None):
    h0 = r0 // 2 if isinstance(r0, int) else pl.multiple_of(r0 // 2, 8)
    if off is not None:
        h0 = pl.multiple_of(h0 + off, 8)
    cols = slice(None) if c0 is None else pl.ds(c0, nc)
    return pltpu.bitcast(ref[pl.ds(h0, n // 2), cols], bf16)


def _st(ref, r0, val, c0=None):
    h0 = r0 // 2 if isinstance(r0, int) else pl.multiple_of(r0 // 2, 8)
    cols = slice(None) if c0 is None else pl.ds(c0, val.shape[1])
    ref[pl.ds(h0, val.shape[0] // 2), cols] = pltpu.bitcast(val.astype(bf16), i32)


def _dual_softmax(p):
    outs = []
    for h in range(p.shape[0] // DH):
        ph = p[h * DH:(h + 1) * DH]
        mx = jnp.max(ph, axis=0, keepdims=True)
        mn = jnp.min(ph, axis=0, keepdims=True)
        ep = jnp.exp2(ph - mx)
        en = jnp.exp2(mn - ph)
        outs.append(ep * _recip(jnp.sum(ep, axis=0, keepdims=True)))
        outs.append(en * _recip(jnp.sum(en, axis=0, keepdims=True)))
    return jnp.concatenate(outs, axis=0)


def _col(row):
    return jnp.broadcast_to(row, (128, 128)).T


def _lhs_terms(a11, a12, a21, a22):
    return [a11 + a22, a21 + a22, a11, a22, a11 + a12, a21 - a11, a12 - a22]


def _rhs_sums(b11, b12, b21, b22):
    return [b11 + b22, b12 - b22, b21 - b11, b11 + b12, b21 + b22]


RHS_SLOT = {0: 0, 2: 1, 3: 2, 5: 3, 6: 4}


def _strassen(prod, between, out):
    m4 = prod(3)
    between(0)
    m2 = prod(1)
    out(2, m2 + m4)
    between(1)
    c11 = m4 + prod(6)
    between(2)
    m1 = prod(0)
    c11 = c11 + m1
    c22 = m1 - m2
    between(3)
    m5 = prod(4)
    out(0, c11 - m5)
    between(4)
    m3 = prod(2)
    out(1, m3 + m5)
    c22 = c22 + m3
    between(5)
    out(3, c22 + prod(5))
    between(6)


def _kernel(x_hbm, wqkv_hbm, wphi_hbm, wo_hbm, wr_hbm, wg_hbm, wu_hbm, wd_hbm, gw_hbm,
            out_hbm,
            xs, xq, w3, wphi, wv2, wg, wu, wd, bd, kvs, gs, rs, xsel, ob,
            sems, osem, zsem, *wt):
    zero = pl.semaphore_read(zsem)
    uses = [0]

    def dz():
        uses[0] += 1
        return zero * (8 * uses[0])

    delayed = []

    def defer(gaps, fn):
        delayed.append([gaps, fn])

    def tick():
        for item in delayed:
            item[0] -= 1
        due = [item for item in delayed if item[0] <= 0]
        delayed[:] = [item for item in delayed if item[0] > 0]
        for _, fn in due:
            fn()

    def rows_cp(src, dst, r0, n, s):
        return pltpu.make_async_copy(src.at[pl.ds(r0, n)], dst.bitcast(bf16).at[pl.ds(r0, n)], sems.at[s])

    def w3_cp(c0, nc, s):
        return pltpu.make_async_copy(wqkv_hbm.at[:, pl.ds(c0, nc)],
                                     w3.bitcast(bf16).at[:, pl.ds(c0, nc)], sems.at[s])

    def wphi_cp(r0, n, s):
        return pltpu.make_async_copy(wphi_hbm.at[pl.ds(r0, n)], wphi.at[pl.ds(r0, n)], sems.at[s])

    def out_cp(r0, c0, nc):
        return pltpu.make_async_copy(ob.bitcast(bf16).at[pl.ds(r0, T), pl.ds(c0, nc)],
                                     out_hbm.at[pl.ds(r0, T), pl.ds(c0, nc)], osem)

    def start(cps):
        for cp in cps:
            cp.start()

    def wait(cps):
        for cp in cps:
            cp.wait()

    x_cps = [rows_cp(x_hbm, xs, t * T, T, t) for t in range(NTILE)]
    first = [wphi_cp(0, 256, 8), w3_cp(D, 256, 8), w3_cp(2 * D, 256, 8),
             pltpu.make_async_copy(wr_hbm, wv2.at[0], sems.at[8]),
             pltpu.make_async_copy(gw_hbm, wv2.at[1], sems.at[8])]
    second = [w3_cp(D + 256, 128, 9), w3_cp(2 * D + 256, 128, 9), wphi_cp(256, 768, 9)]
    third = [w3_cp(D + 384, 640, 10), w3_cp(2 * D + 384, 640, 10)]
    fourth = [w3_cp(0, D, 11)]
    for j in range(NTILE):
        for u in range(2):
            fourth.append(pltpu.make_async_copy(
                wo_hbm.at[pl.ds(u * HD + j * 64, 64)],
                xq.bitcast(bf16).at[pl.ds(j * HT + u * 64, 64), pl.ds(WO0, D)], sems.at[11]))
    ffn_cps = [rows_cp(src, dst, r, 64, 12)
               for src, dst in ((wg_hbm, wg), (wu_hbm, wu)) for r in range(0, D, 64)]
    ffn_cps += [rows_cp(wd_hbm, wd, r, 128, 12) for r in range(0, F, 128)]
    stream = list(ffn_cps)

    def feed():
        if stream:
            stream.pop(0).start()

    start(first + x_cps[:1])
    row = lax.broadcasted_iota(i32, (128, 128), 0)
    col = lax.broadcasted_iota(i32, (128, 128), 1)
    eye = jnp.where(lax.broadcasted_iota(i32, (128, DH), 0) % DH
                    == lax.broadcasted_iota(i32, (128, DH), 1), 1.0, 0.0).astype(bf16)
    wait(first)
    start(x_cps[1:3])

    def make_bd(g0, n, gaps=0):
        m = _dot(eye, wphi[pl.ds(g0 * 128, n * 128), :], NT)

        def store():
            for g in range(n):
                _st(bd, (g0 + g) * 128, jnp.where(row // DH == col // DH, m[:, g * 128:(g + 1) * 128], 0.0))

        if gaps:
            defer(gaps, store)
        else:
            store()

    def fold(g, c0):
        return _dot(_ld(bd, g * 128, 128), _ld(w3, 0, D, c0, 128), NT) * LOG2E

    def put_lhs(slot, r0, top, bot):
        for i, s in enumerate(_lhs_terms(top[:, :HD], top[:, HD:], bot[:, :HD], bot[:, HD:])):
            _st(wt[slot], r0, s, i * HD)

    def prep_kv(g):
        kt = fold(g, D + g * 128)
        vt = _ld(w3, 0, D, 2 * D + g * 128, 128).T.astype(f32)
        put_lhs(g, 64, vt[:64], vt[64:])
        put_lhs(g, 0, kt[:64], kt[64:])

    def prep_q(g):
        put_lhs(NG + g, 0, fold(g, g * 128), fold(g + 4, (g + 4) * 128))

    def put_rhs(load, rd, cd, n):
        for r in range(0, n, 16):
            for c in range(0, HD, 128):
                for i, s in enumerate(_rhs_sums(*[load(q, r, c).astype(f32) for q in range(4)])):
                    _st(xq, rd + r, s, cd + i * HD + c)

    def prep_x(t, r0, n):
        put_rhs(lambda q, r, c: _ld(xs, t * T + (q % 2) * HT + r0 + r, 16, (q // 2) * HD + c, 128),
                t * HT + r0, 0, n)

    def prep_wo(k):
        r0, off = (k // 4) * HT + (k % 4) * 16, dz()
        put_rhs(lambda q, r, c: _ld(xq, r0 + (q // 2) * 64, 16, WO0 + (q % 2) * HD + c, 128, off),
                r0, WS0, 16)

    def x_term(i, t):
        if i == 1:
            return _ld(xs, t * T, HT, 0, HD, dz())
        if i == 4:
            return _ld(xs, t * T + HT, HT, HD, HD, dz())
        return _ld(xq, t * HT, HT, RHS_SLOT[i] * HD, HD, dz())

    def project(slot, t, between, out):
        _strassen(lambda i: _dot(_ld(wt[slot], 0, 128, i * HD, HD, dz()), x_term(i, t), NT), between, out)

    st = {}
    wr = wv2[0].astype(f32)
    gw = wv2[1].astype(f32)
    upper = lax.broadcasted_iota(i32, (8, 128), 0) < 4
    score_rows = jnp.concatenate(
        [jnp.where(upper, wr[j:j + 1, :], gw[j:j + 1, :]) for j in range(8)], axis=1)

    def score_step(t, j):
        r0, k0 = t * T + (j // 2) * HT, (j % 2) * HD
        d = _dot(score_rows[:, k0:k0 + HD], _ld(xs, r0, HT, k0, HD), NT)
        if j % 2 == 0:
            st['sc'] = d
        else:
            d = d + st.pop('sc')
            rs[:, pl.ds(r0, HT)] = jnp.broadcast_to(_r16(d[:1]), (8, HT))
            gs[pl.ds(r0, HT), :] = _col(jax.nn.sigmoid(d[4:5]))

    def route():
        r = rs[...]
        pos = lax.broadcasted_iota(i32, r.shape, 1)
        best = jnp.max(jnp.where(r == r, r, -jnp.inf))
        idx = jnp.min(jnp.where(r == best, pos, S))
        st['idx'] = idx = jnp.where(idx >= S, 0, idx)
        st['score'] = jnp.sum(jnp.where(pos == idx, r, 0.0)[:1])
        st['blk'] = blk = pl.multiple_of((idx // 16) * 16, 16)
        sel = lax.broadcasted_iota(i32, (16, D), 0) == idx - blk
        xr = jnp.sum(jnp.where(sel, _ld(xs, blk, 16).astype(f32), 0.0), axis=0, keepdims=True)
        xsel[...] = jnp.broadcast_to(xr, (8, D))

    def pin(v):
        def store():
            xq[pl.ds(0, 8), pl.ds(PIN0, v.shape[1])] = pltpu.bitcast(v, i32)

        defer(PIN_LAG, store)

    def ffn_step(k):
        n, j = divmod(k, 6)
        if j < 4 and n < NF:
            k0 = (j % 2) * HD
            xr = xsel[pl.ds(pl.multiple_of(dz(), 8), 8), pl.ds(k0, HD)]
            st['f', j] = _dot(xr, _ld((wg, wu)[j // 2], k0, HD, n * 128, 128), NN)
            pin(st['f', j])
            if j == 3:
                gt = _r16(st.pop(('f', 0)) + st.pop(('f', 1)))
                up = _r16(st.pop(('f', 2)) + st.pop(('f', 3)))
                st['h', n] = _r16(_r16(gt * jax.nn.sigmoid(gt)) * up)
        if j >= 4 and 1 <= n <= NF:
            yk = _dot(st['h', n - 1], _ld(wd, (n - 1) * 128, 128, (j - 4) * HD, HD), NN)
            pin(yk)
            st['y', j - 4] = yk if n == 1 else st['y', j - 4] + yk
            if n == NF and j == 5:
                st['y'] = jnp.concatenate([st.pop(('y', 0)), st.pop(('y', 1))], axis=1)

    def patch():
        weight = _r16(jax.nn.sigmoid(jnp.full((16, D), st['score'], f32)))
        y = _r16(_r16(st.pop('y')[:1]) * weight)
        sel = lax.broadcasted_iota(i32, (16, D), 0) == st['idx'] - st['blk']
        xr = _ld(xs, st['blk'], 16).astype(f32)
        _st(xs, st['blk'], jnp.where(sel, xr + y, xr))

    r72 = lax.broadcasted_iota(i32, (72, 128), 0)
    c72 = lax.broadcasted_iota(i32, (72, 128), 1)
    kv_mask = jnp.where(r72 < 64, r72 // DH, r72 - 64) == c72 // 64
    accs = {}

    def kv_update(pair, is_first, is_last, r):
        phi = _dual_softmax(r[:64])
        d = _dot(r[64:].astype(bf16), phi.astype(bf16), NT)
        accs[pair] = (d, phi) if is_first else (accs[pair][0] + d, accs[pair][1] + phi)
        if is_last:
            d, z = accs.pop(pair)
            z = jnp.sum(z.T, axis=0, keepdims=True)
            kv = jnp.concatenate([d, jnp.broadcast_to(z, (8, 128))], axis=0)

            def store():
                kvs[pl.ds(pair * 72, 72), :] = jnp.where(kv_mask, _r16(kv), 0.0)

            defer(2, store)

    make_bd(0, 2)
    prep_kv(0)
    prep_kv(1)
    order = [(g, t) for t in range(NTILE) for g in range(2)]
    order += [(g, t) for g in range(2, NG) for t in range(NTILE)]
    for g, t in order:
        if (g, t) == (0, 0):
            wait(x_cps[:1])
            start(x_cps[3:5])
            prep_x(0, 0, HT)
        if (g, t) == (0, 1):
            wait(x_cps[1:3])
            start(x_cps[5:7])
            prep_x(1, 0, HT)
        if (g, t) == (0, 2):
            wait(x_cps[3:4])
            start(x_cps[7:] + second)
        if (g, t) == (0, 3):
            wait(x_cps[4:6])
            start(third)
        if (g, t) == (0, 5):
            wait(x_cps[6:] + second)
            start(fourth)
        if (g, t) == (2, 5):
            wait(third + fourth)

        def between(j):
            tick()
            if g == 1 and j in (0, 1, 3, 4):
                score_step(t, (0, 1, 3, 4).index(j))
            if j == 3 and g >= 3:
                feed()
            if j == 3 and g >= 4:
                prep_wo((g - 4) * NTILE + t)
            if g < 2 and 1 < t + 1 < NTILE and g * 7 + j in X_GAPS:
                prep_x(t + 1, X_GAPS.index(g * 7 + j) * 16, 16)
            if (g, t, j) == (0, 5, 0):
                make_bd(2, 6, 2)
            if j == 6 and g >= 1 and t == (6 if g == 1 else 5 if g == 2 else 1):
                if g + 1 < NG:
                    prep_kv(g + 1)
                else:
                    prep_q(0)
            if (g, t, j) == (2, 3, 6):
                route()

        def out(q, c):
            defer(KV_LAG[q], functools.partial(
                kv_update, 2 * g + q // 2, t == 0 and q % 2 == 0, t == NTILE - 1 and q % 2 == 1, c))

        project(g, t, between, out)

    pairs = []

    def attend(g, t, u, r):
        phi = _dual_softmax(r).astype(bf16)
        r0 = (2 * (g + 4 * (u % 2)) + u // 2) * 72
        nd = _dot(kvs[pl.ds(pl.multiple_of(r0 + dz(), 8), 72), :], phi, NN)
        inv = _recip(nd[64:72] + 1e-6)
        st['o', u] = jnp.concatenate([nd[0:32] * inv[0:1], nd[32:64] * inv[1:2]], axis=0)
        if u < 3:
            return
        lo = jnp.concatenate([st.pop(('o', 0)), st.pop(('o', 2))], axis=0)
        hi = jnp.concatenate([st.pop(('o', 1)), st.pop(('o', 3))], axis=0)
        terms = _lhs_terms(lo[:, :HT], hi[:, :HT], lo[:, HT:], hi[:, HT:])

        def store(i, n):
            v = jnp.concatenate(terms[i:i + n], axis=1).astype(bf16).T
            for k in range(n):
                _st(xq, t * HT, v[k * HT:(k + 1) * HT], OS0 + (i + k) * HD + g * 128)

        for i in range(0, 7, 2):
            defer(O_LAG + i // 2, functools.partial(store, i, min(2, 7 - i)))

    for g in range(NG // 2):
        for t in range(NTILE):
            if (g, t) == (3, 4):
                assert not stream
                wait(ffn_cps)

            def between(j):
                tick()
                if j == 3:
                    feed()
                if j in Q_GAPS and pairs:
                    pairs.pop(0)()
                if (t, j) == (1, 4) and g + 1 < NG // 2:
                    prep_q(g + 1)

            cs = {}
            project(NG + g, t, between, cs.__setitem__)
            lo = jnp.concatenate([cs[0], cs[1]], axis=1)
            hi = jnp.concatenate([cs[2], cs[3]], axis=1)
            for u, r in enumerate((lo[:64], hi[:64], lo[64:], hi[64:])):
                pairs.append(functools.partial(attend, g, t, u, r))

    routed = st['idx'] // T
    tiles = [i + (routed <= i).astype(i32) for i in range(NTILE - 1)] + [routed]
    ffn_gaps = 6 * (NF + 1)
    assert ffn_gaps + 2 < (NTILE - 1) * 28

    def wo_term(k, c):
        r0, c0 = (0, WO0) if k == 1 else (64, WO0 + HD) if k == 4 else (0, WS0 + RHS_SLOT[k] * HD)
        off = dz()
        return jnp.concatenate(
            [_ld(xq, j * HT + r0, 64, c0 + c * 128, 128, off) for j in range(NTILE)], axis=0)

    for i, tile in enumerate(tiles):
        r0 = pl.multiple_of(tile * T, T)
        for c in range(4):
            def between(j):
                tick()
                if j in Q_GAPS and pairs:
                    pairs.pop(0)()
                k = (i * 4 + c) * 7 + j
                if k < ffn_gaps:
                    ffn_step(k)
                if k == ffn_gaps + 2:
                    patch()

            def mix(q, a):
                rq, cq = r0 + (q // 2) * HT, (q % 2) * HD + c * 128
                gate = gs[pl.ds(pl.multiple_of(rq, HT), HT), :]
                b = _ld(xs, rq, HT, cq, 128).astype(f32)
                _st(ob, rq, b + gate * (a - b), cq)

            _strassen(lambda k: _dot(_ld(xq, 0, HT, OS0 + k * HD, HD, tile * (HT // 2) + dz()),
                                     wo_term(k, c), NN), between, mix)
            n = 1 if i == NTILE - 1 else 4
            if (c + 1) % n == 0:
                for u in range(2):
                    defer(DMA_LAG, out_cp(r0, u * HD + (c + 1 - n) * 128, n * 128).start)
    while delayed:
        tick()
    pltpu.make_async_copy(ob.bitcast(bf16), out_hbm, osem).wait()


@jax.jit
def pallas_gated_mix__linear_kernel_hedgehog__moe_arch_mod__prompt_kernel(A_x, A_wqkv, A_w_phi, A_wo, B_x, B_w_r, B_w_gate, B_w_up, B_w_down, gate_w):
    del B_x
    hbm = pl.BlockSpec(memory_space=pl.ANY)
    out = pl.pallas_call(
        _kernel,
        out_shape=jax.ShapeDtypeStruct((S, D), bf16),
        in_specs=[hbm] * 9,
        out_specs=hbm,
        scratch_shapes=[
            pltpu.VMEM((S // 2, D), i32),
            pltpu.VMEM((S // 4, XQ_COLS), i32),
            pltpu.VMEM((D // 2, 3 * D), i32),
            pltpu.VMEM((H * DH, DH), bf16),
            pltpu.VMEM((2, 8, 128), bf16),
            pltpu.VMEM((D // 2, F), i32),
            pltpu.VMEM((D // 2, F), i32),
            pltpu.VMEM((F // 2, D), i32),
            pltpu.VMEM((NG * 128 // 2, 128), i32),
            pltpu.VMEM((16 * 72, 128), f32),
            pltpu.VMEM((S, 128), f32),
            pltpu.VMEM((8, S), f32),
            pltpu.VMEM((8, D), f32),
            pltpu.VMEM((S // 2, D), i32),
            pltpu.SemaphoreType.DMA((13,)),
            pltpu.SemaphoreType.DMA,
            pltpu.SemaphoreType.REGULAR,
        ] + [pltpu.VMEM((64, 7 * HD + 128), i32)] * (NG + NG // 2),
        compiler_params=pltpu.CompilerParams(vmem_limit_bytes=100 * 1024 * 1024),
    )(A_x.reshape(S, D), A_wqkv, A_w_phi.reshape(H * DH, DH), A_wo,
      B_w_r.reshape(8, 128), B_w_gate, B_w_up, B_w_down, gate_w.reshape(8, 128))
    return out.reshape(1, S, D)
```

```python
import functools

import jax
import jax.numpy as jnp
from jax import lax
import jax.experimental.pallas as pl
import jax.experimental.pallas.tpu as pltpu

S, D, H, DH, F = 2048, 1024, 32, 32, 3584
NG = 8
T = 256
HT = T // 2
HD = D // 2
NTILE = S // T
NF = F // 128
LOG2E = 1.4426950408889634

OS0, WO0, WS0, PIN0, XQ_COLS = 5 * HD, 12 * HD, 14 * HD, 19 * HD, 20 * HD + 128

KV_LAG = (3, 5, 3, 6)
X_GAPS = (1, 2, 4, 5, 7, 9, 10, 12)
Q_GAPS = (0, 1, 4, 5)
O_LAG = 3
PIN_LAG = 2
DMA_LAG = 4

NT = (((1,), (1,)), ((), ()))
NN = (((1,), (0,)), ((), ()))
f32 = jnp.float32
bf16 = jnp.bfloat16
i32 = jnp.int32


def _dot(a, b, dims):
    return lax.dot_general(a, b, dims, preferred_element_type=f32)


def _recip(x):
    r = pl.reciprocal(x, approx=True)
    return r * (2.0 - x * r)


def _r16(x):
    return x.astype(bf16).astype(f32)


def _ld(ref, r0, n, c0=None, nc=None, off=None):
    h0 = r0 // 2 if isinstance(r0, int) else pl.multiple_of(r0 // 2, 8)
    if off is not None:
        h0 = pl.multiple_of(h0 + off, 8)
    cols = slice(None) if c0 is None else pl.ds(c0, nc)
    return pltpu.bitcast(ref[pl.ds(h0, n // 2), cols], bf16)


def _st(ref, r0, val, c0=None):
    h0 = r0 // 2 if isinstance(r0, int) else pl.multiple_of(r0 // 2, 8)
    cols = slice(None) if c0 is None else pl.ds(c0, val.shape[1])
    ref[pl.ds(h0, val.shape[0] // 2), cols] = pltpu.bitcast(val.astype(bf16), i32)


def _dual_softmax(p):
    outs = []
    for h in range(p.shape[0] // DH):
        ph = p[h * DH:(h + 1) * DH]
        mx = jnp.max(ph, axis=0, keepdims=True)
        mn = jnp.min(ph, axis=0, keepdims=True)
        ep = jnp.exp2(ph - mx)
        en = jnp.exp2(mn - ph)
        outs.append(ep * _recip(jnp.sum(ep, axis=0, keepdims=True)))
        outs.append(en * _recip(jnp.sum(en, axis=0, keepdims=True)))
    return jnp.concatenate(outs, axis=0)


def _col(row):
    return jnp.broadcast_to(row, (128, 128)).T


def _lhs_terms(a11, a12, a21, a22):
    return [a11 + a22, a21 + a22, a11, a22, a11 + a12, a21 - a11, a12 - a22]


def _rhs_sums(b11, b12, b21, b22):
    return [b11 + b22, b12 - b22, b21 - b11, b11 + b12, b21 + b22]


RHS_SLOT = {0: 0, 2: 1, 3: 2, 5: 3, 6: 4}


def _strassen(prod, between, out):
    m4 = prod(3)
    between(0)
    m2 = prod(1)
    out(2, m2 + m4)
    between(1)
    c11 = m4 + prod(6)
    between(2)
    m1 = prod(0)
    c11 = c11 + m1
    c22 = m1 - m2
    between(3)
    m5 = prod(4)
    out(0, c11 - m5)
    between(4)
    m3 = prod(2)
    out(1, m3 + m5)
    c22 = c22 + m3
    between(5)
    out(3, c22 + prod(5))
    between(6)


def _kernel(x_hbm, wqkv_hbm, wphi_hbm, wo_hbm, wr_hbm, wg_hbm, wu_hbm, wd_hbm, gw_hbm,
            out_hbm,
            xs, xq, w3, wphi, wv2, wg, wu, wd, bd, kvs, gs, rs, xsel, ob,
            sems, osem, zsem, *wt):
    zero = pl.semaphore_read(zsem)
    uses = [0]

    def dz():
        uses[0] += 1
        return zero * (8 * uses[0])

    delayed = []

    def defer(gaps, fn):
        delayed.append([gaps, fn])

    def tick():
        for item in delayed:
            item[0] -= 1
        due = [item for item in delayed if item[0] <= 0]
        delayed[:] = [item for item in delayed if item[0] > 0]
        for _, fn in due:
            fn()

    def rows_cp(src, dst, r0, n, s):
        return pltpu.make_async_copy(src.at[pl.ds(r0, n)], dst.bitcast(bf16).at[pl.ds(r0, n)], sems.at[s])

    def w3_cp(c0, nc, s):
        return pltpu.make_async_copy(wqkv_hbm.at[:, pl.ds(c0, nc)],
                                     w3.bitcast(bf16).at[:, pl.ds(c0, nc)], sems.at[s])

    def wphi_cp(r0, n, s):
        return pltpu.make_async_copy(wphi_hbm.at[pl.ds(r0, n)], wphi.at[pl.ds(r0, n)], sems.at[s])

    def out_cp(r0, c0, nc):
        return pltpu.make_async_copy(ob.bitcast(bf16).at[pl.ds(r0, T), pl.ds(c0, nc)],
                                     out_hbm.at[pl.ds(r0, T), pl.ds(c0, nc)], osem)

    def start(cps):
        for cp in cps:
            cp.start()

    def wait(cps):
        for cp in cps:
            cp.wait()

    x_cps = [rows_cp(x_hbm, xs, t * T, T, t) for t in range(NTILE)]
    first = [wphi_cp(0, 256, 8), w3_cp(D, 256, 8), w3_cp(2 * D, 256, 8),
             pltpu.make_async_copy(wr_hbm, wv2.at[0], sems.at[8]),
             pltpu.make_async_copy(gw_hbm, wv2.at[1], sems.at[8])]
    second = [w3_cp(D + 256, 128, 9), w3_cp(2 * D + 256, 128, 9), wphi_cp(256, 768, 9)]
    third = [w3_cp(D + 384, 640, 10), w3_cp(2 * D + 384, 640, 10)]
    fourth = [w3_cp(0, D, 11)]
    for j in range(NTILE):
        for u in range(2):
            fourth.append(pltpu.make_async_copy(
                wo_hbm.at[pl.ds(u * HD + j * 64, 64)],
                xq.bitcast(bf16).at[pl.ds(j * HT + u * 64, 64), pl.ds(WO0, D)], sems.at[11]))
    ffn_cps = [rows_cp(src, dst, r, 64, 12)
               for src, dst in ((wg_hbm, wg), (wu_hbm, wu)) for r in range(0, D, 64)]
    ffn_cps += [rows_cp(wd_hbm, wd, r, 128, 12) for r in range(0, F, 128)]
    stream = list(ffn_cps)

    def feed():
        if stream:
            stream.pop(0).start()

    start(first + x_cps[:1])
    row = lax.broadcasted_iota(i32, (128, 128), 0)
    col = lax.broadcasted_iota(i32, (128, 128), 1)
    eye = jnp.where(lax.broadcasted_iota(i32, (128, DH), 0) % DH
                    == lax.broadcasted_iota(i32, (128, DH), 1), 1.0, 0.0).astype(bf16)
    wait(first)
    start(x_cps[1:3])

    def make_bd(g0, n, gaps=0):
        m = _dot(eye, wphi[pl.ds(g0 * 128, n * 128), :], NT)

        def store():
            for g in range(n):
                _st(bd, (g0 + g) * 128, jnp.where(row // DH == col // DH, m[:, g * 128:(g + 1) * 128], 0.0))

        if gaps:
            defer(gaps, store)
        else:
            store()

    def fold(g, c0):
        return _dot(_ld(bd, g * 128, 128), _ld(w3, 0, D, c0, 128), NT) * LOG2E

    def put_lhs(slot, r0, top, bot):
        for i, s in enumerate(_lhs_terms(top[:, :HD], top[:, HD:], bot[:, :HD], bot[:, HD:])):
            _st(wt[slot], r0, s, i * HD)

    def prep_kv(g):
        kt = fold(g, D + g * 128)
        vt = _ld(w3, 0, D, 2 * D + g * 128, 128).T.astype(f32)
        put_lhs(g, 64, vt[:64], vt[64:])
        put_lhs(g, 0, kt[:64], kt[64:])

    def prep_q(g):
        put_lhs(NG + g, 0, fold(g, g * 128), fold(g + 4, (g + 4) * 128))

    def put_rhs(load, rd, cd, n):
        for r in range(0, n, 16):
            for c in range(0, HD, 128):
                for i, s in enumerate(_rhs_sums(*[load(q, r, c).astype(f32) for q in range(4)])):
                    _st(xq, rd + r, s, cd + i * HD + c)

    def prep_x(t, r0, n):
        put_rhs(lambda q, r, c: _ld(xs, t * T + (q % 2) * HT + r0 + r, 16, (q // 2) * HD + c, 128),
                t * HT + r0, 0, n)

    def prep_wo(k):
        r0, off = (k // 4) * HT + (k % 4) * 16, dz()
        put_rhs(lambda q, r, c: _ld(xq, r0 + (q // 2) * 64, 16, WO0 + (q % 2) * HD + c, 128, off),
                r0, WS0, 16)

    def x_term(i, t):
        if i == 1:
            return _ld(xs, t * T, HT, 0, HD, dz())
        if i == 4:
            return _ld(xs, t * T + HT, HT, HD, HD, dz())
        return _ld(xq, t * HT, HT, RHS_SLOT[i] * HD, HD, dz())

    def project(slot, t, between, out):
        _strassen(lambda i: _dot(_ld(wt[slot], 0, 128, i * HD, HD, dz()), x_term(i, t), NT), between, out)

    st = {}
    wr = wv2[0].astype(f32)
    gw = wv2[1].astype(f32)
    upper = lax.broadcasted_iota(i32, (8, 128), 0) < 4
    score_rows = jnp.concatenate(
        [jnp.where(upper, wr[j:j + 1, :], gw[j:j + 1, :]) for j in range(8)], axis=1)

    def score_step(t, j):
        r0, k0 = t * T + (j // 2) * HT, (j % 2) * HD
        d = _dot(score_rows[:, k0:k0 + HD], _ld(xs, r0, HT, k0, HD), NT)
        if j % 2 == 0:
            st['sc'] = d
        else:
            d = d + st.pop('sc')
            rs[:, pl.ds(r0, HT)] = jnp.broadcast_to(_r16(d[:1]), (8, HT))
            gs[pl.ds(r0, HT), :] = _col(jax.nn.sigmoid(d[4:5]))

    def route():
        r = rs[...]
        pos = lax.broadcasted_iota(i32, r.shape, 1)
        best = jnp.max(jnp.where(r == r, r, -jnp.inf))
        idx = jnp.min(jnp.where(r == best, pos, S))
        st['idx'] = idx = jnp.where(idx >= S, 0, idx)
        st['score'] = jnp.sum(jnp.where(pos == idx, r, 0.0)[:1])
        st['blk'] = blk = pl.multiple_of((idx // 16) * 16, 16)
        sel = lax.broadcasted_iota(i32, (16, D), 0) == idx - blk
        xr = jnp.sum(jnp.where(sel, _ld(xs, blk, 16).astype(f32), 0.0), axis=0, keepdims=True)
        xsel[...] = jnp.broadcast_to(xr, (8, D))

    def pin(v):
        def store():
            xq[pl.ds(0, 8), pl.ds(PIN0, v.shape[1])] = pltpu.bitcast(v, i32)

        defer(PIN_LAG, store)

    def ffn_step(k):
        n, j = divmod(k, 6)
        if j < 4 and n < NF:
            k0 = (j % 2) * HD
            xr = xsel[pl.ds(pl.multiple_of(dz(), 8), 8), pl.ds(k0, HD)]
            st['f', j] = _dot(xr, _ld((wg, wu)[j // 2], k0, HD, n * 128, 128), NN)
            pin(st['f', j])
            if j == 3:
                gt = _r16(st.pop(('f', 0)) + st.pop(('f', 1)))
                up = _r16(st.pop(('f', 2)) + st.pop(('f', 3)))
                st['h', n] = _r16(_r16(gt * jax.nn.sigmoid(gt)) * up)
        if j >= 4 and 1 <= n <= NF:
            yk = _dot(st['h', n - 1], _ld(wd, (n - 1) * 128, 128, (j - 4) * HD, HD), NN)
            pin(yk)
            st['y', j - 4] = yk if n == 1 else st['y', j - 4] + yk
            if n == NF and j == 5:
                st['y'] = jnp.concatenate([st.pop(('y', 0)), st.pop(('y', 1))], axis=1)

    def patch():
        weight = _r16(jax.nn.sigmoid(jnp.full((16, D), st['score'], f32)))
        y = _r16(_r16(st.pop('y')[:1]) * weight)
        sel = lax.broadcasted_iota(i32, (16, D), 0) == st['idx'] - st['blk']
        xr = _ld(xs, st['blk'], 16).astype(f32)
        _st(xs, st['blk'], jnp.where(sel, xr + y, xr))

    r72 = lax.broadcasted_iota(i32, (72, 128), 0)
    c72 = lax.broadcasted_iota(i32, (72, 128), 1)
    kv_mask = jnp.where(r72 < 64, r72 // DH, r72 - 64) == c72 // 64
    accs = {}

    def kv_update(pair, is_first, is_last, r):
        phi = _dual_softmax(r[:64])
        d = _dot(r[64:].astype(bf16), phi.astype(bf16), NT)
        accs[pair] = (d, phi) if is_first else (accs[pair][0] + d, accs[pair][1] + phi)
        if is_last:
            d, z = accs.pop(pair)
            z = jnp.sum(z.T, axis=0, keepdims=True)
            kv = jnp.concatenate([d, jnp.broadcast_to(z, (8, 128))], axis=0)

            def store():
                kvs[pl.ds(pair * 72, 72), :] = jnp.where(kv_mask, _r16(kv), 0.0)

            defer(2, store)

    make_bd(0, 2)
    prep_kv(0)
    prep_kv(1)
    order = [(g, t) for t in range(NTILE) for g in range(2)]
    order += [(g, t) for g in range(2, NG) for t in range(NTILE)]
    for g, t in order:
        if (g, t) == (0, 0):
            wait(x_cps[:1])
            start(x_cps[3:5])
            prep_x(0, 0, HT)
        if (g, t) == (0, 1):
            wait(x_cps[1:3])
            start(x_cps[5:7])
            prep_x(1, 0, HT)
        if (g, t) == (0, 2):
            wait(x_cps[3:4])
            start(x_cps[7:] + second)
        if (g, t) == (0, 3):
            wait(x_cps[4:6])
            start(third)
        if (g, t) == (0, 5):
            wait(x_cps[6:] + second)
            start(fourth)
        if (g, t) == (2, 5):
            wait(third + fourth)

        def between(j):
            tick()
            if g == 1 and j in (0, 1, 3, 4):
                score_step(t, (0, 1, 3, 4).index(j))
            if j == 3 and g >= 3:
                feed()
            if j == 3 and g >= 4:
                prep_wo((g - 4) * NTILE + t)
            if g < 2 and 1 < t + 1 < NTILE and g * 7 + j in X_GAPS:
                prep_x(t + 1, X_GAPS.index(g * 7 + j) * 16, 16)
            if (g, t, j) == (0, 5, 0):
                make_bd(2, 6, 2)
            if j == 6 and g >= 1 and t == (6 if g == 1 else 5 if g == 2 else 1):
                if g + 1 < NG:
                    prep_kv(g + 1)
                else:
                    prep_q(0)
            if (g, t, j) == (2, 3, 6):
                route()

        def out(q, c):
            defer(KV_LAG[q], functools.partial(
                kv_update, 2 * g + q // 2, t == 0 and q % 2 == 0, t == NTILE - 1 and q % 2 == 1, c))

        project(g, t, between, out)

    pairs = []

    def attend(g, t, u, r):
        phi = _dual_softmax(r).astype(bf16)
        r0 = (2 * (g + 4 * (u % 2)) + u // 2) * 72
        nd = _dot(kvs[pl.ds(pl.multiple_of(r0 + dz(), 8), 72), :], phi, NN)
        inv = _recip(nd[64:72] + 1e-6)
        st['o', u] = jnp.concatenate([nd[0:32] * inv[0:1], nd[32:64] * inv[1:2]], axis=0)
        if u < 3:
            return
        lo = jnp.concatenate([st.pop(('o', 0)), st.pop(('o', 2))], axis=0)
        hi = jnp.concatenate([st.pop(('o', 1)), st.pop(('o', 3))], axis=0)
        terms = _lhs_terms(lo[:, :HT], hi[:, :HT], lo[:, HT:], hi[:, HT:])

        def store(i, n):
            v = jnp.concatenate(terms[i:i + n], axis=1).astype(bf16).T
            for k in range(n):
                _st(xq, t * HT, v[k * HT:(k + 1) * HT], OS0 + (i + k) * HD + g * 128)

        for i in range(0, 7, 2):
            defer(O_LAG + i // 2, functools.partial(store, i, min(2, 7 - i)))

    for g in range(NG // 2):
        for t in range(NTILE):
            if (g, t) == (3, 4):
                assert not stream
                wait(ffn_cps)

            def between(j):
                tick()
                if j == 3:
                    feed()
                if j in Q_GAPS and pairs:
                    pairs.pop(0)()
                if (t, j) == (1, 4) and g + 1 < NG // 2:
                    prep_q(g + 1)

            cs = {}
            project(NG + g, t, between, cs.__setitem__)
            lo = jnp.concatenate([cs[0], cs[1]], axis=1)
            hi = jnp.concatenate([cs[2], cs[3]], axis=1)
            for u, r in enumerate((lo[:64], hi[:64], lo[64:], hi[64:])):
                pairs.append(functools.partial(attend, g, t, u, r))

    routed = st['idx'] // T
    tiles = [i + (routed <= i).astype(i32) for i in range(NTILE - 1)] + [routed]
    ffn_gaps = 6 * (NF + 1)
    assert ffn_gaps + 2 < (NTILE - 1) * 28

    def wo_term(k, c):
        r0, c0 = (0, WO0) if k == 1 else (64, WO0 + HD) if k == 4 else (0, WS0 + RHS_SLOT[k] * HD)
        off = dz()
        return jnp.concatenate(
            [_ld(xq, j * HT + r0, 64, c0 + c * 128, 128, off) for j in range(NTILE)], axis=0)

    for i, tile in enumerate(tiles):
        r0 = pl.multiple_of(tile * T, T)
        for c in range(4):
            def between(j):
                tick()
                if j in Q_GAPS and pairs:
                    pairs.pop(0)()
                k = (i * 4 + c) * 7 + j
                if k < ffn_gaps:
                    ffn_step(k)
                if k == ffn_gaps + 2:
                    patch()

            def mix(q, a):
                rq, cq = r0 + (q // 2) * HT, (q % 2) * HD + c * 128
                gate = gs[pl.ds(pl.multiple_of(rq, HT), HT), :]
                b = _ld(xs, rq, HT, cq, 128).astype(f32)
                _st(ob, rq, b + gate * (a - b), cq)

            _strassen(lambda k: _dot(_ld(xq, 0, HT, OS0 + k * HD, HD, tile * (HT // 2) + dz()),
                                     wo_term(k, c), NN), between, mix)
            for u in range(2):
                defer(DMA_LAG, out_cp(r0, u * HD + c * 128, 128).start)
    while delayed:
        tick()
    pltpu.make_async_copy(ob.bitcast(bf16), out_hbm, osem).wait()


@jax.jit
def pallas_gated_mix__linear_kernel_hedgehog__moe_arch_mod__prompt_kernel(A_x, A_wqkv, A_w_phi, A_wo, B_x, B_w_r, B_w_gate, B_w_up, B_w_down, gate_w):
    del B_x
    hbm = pl.BlockSpec(memory_space=pl.ANY)
    out = pl.pallas_call(
        _kernel,
        out_shape=jax.ShapeDtypeStruct((S, D), bf16),
        in_specs=[hbm] * 9,
        out_specs=hbm,
        scratch_shapes=[
            pltpu.VMEM((S // 2, D), i32),
            pltpu.VMEM((S // 4, XQ_COLS), i32),
            pltpu.VMEM((D // 2, 3 * D), i32),
            pltpu.VMEM((H * DH, DH), bf16),
            pltpu.VMEM((2, 8, 128), bf16),
            pltpu.VMEM((D // 2, F), i32),
            pltpu.VMEM((D // 2, F), i32),
            pltpu.VMEM((F // 2, D), i32),
            pltpu.VMEM((NG * 128 // 2, 128), i32),
            pltpu.VMEM((16 * 72, 128), f32),
            pltpu.VMEM((S, 128), f32),
            pltpu.VMEM((8, S), f32),
            pltpu.VMEM((8, D), f32),
            pltpu.VMEM((S // 2, D), i32),
            pltpu.SemaphoreType.DMA((13,)),
            pltpu.SemaphoreType.DMA,
            pltpu.SemaphoreType.REGULAR,
        ] + [pltpu.VMEM((64, 7 * HD + 128), i32)] * (NG + NG // 2),
        compiler_params=pltpu.CompilerParams(vmem_limit_bytes=100 * 1024 * 1024),
    )(A_x.reshape(S, D), A_wqkv, A_w_phi.reshape(H * DH, DH), A_wo,
      B_w_r.reshape(8, 128), B_w_gate, B_w_up, B_w_down, gate_w.reshape(8, 128))
    return out.reshape(1, S, D)
```
